```python
import jax
import jax.numpy as jnp

def _softmax(x, axis=-1):
    return jax.nn.softmax(x, axis=axis)
def _gelu(x):
    return jax.nn.gelu(x, approximate=True)
def _silu(x):
    return jax.nn.silu(x)
def _sigmoid(x):
    return jax.nn.sigmoid(x)
def _layernorm(x, axis=-1, eps=1e-5):
    m = jnp.mean(x, axis=axis, keepdims=True)
    v = jnp.var(x, axis=axis, keepdims=True)
    return (x - m) / jnp.sqrt(v + eps)
def _scatter_add(tgt, idx, src, axis=0):
    return tgt.at[idx].add(src)
def _segment_sum(src, seg, n):
    return jax.ops.segment_sum(src, seg, n)
class _Rng:
    def __init__(self, key):
        self._k = key
    def _next(self):
        self._k, sub = jax.random.split(self._k)
        return sub
    def normal(self, shape):
        return jax.random.normal(self._next(), shape, dtype=jnp.bfloat16)
    def randint(self, lo, hi, shape):
        return jax.random.randint(self._next(), shape, lo, hi, dtype=jnp.int32)
    def uniform(self, shape, lo=0.0, hi=1.0):
        return jax.random.uniform(self._next(), shape, jnp.bfloat16, lo, hi)
    def permutation(self, n):
        return jax.random.permutation(self._next(), n)


kernel_name = 'interleave_layers__sliding_block__moe_arch_mod__prompt'

def setup_inputs():
    _rng = _Rng(jax.random.key(int.from_bytes(__import__("os").urandom(4), "little")))
    _w = (lambda a: (lambda t: t.astype(jnp.bfloat16) if jnp.issubdtype(t.dtype, jnp.floating) else t)(jnp.asarray(a)))
    def _A_setup():
        B, S, D = 1, 2048, 1024
        return {
            "x": _w((lambda *s: _rng.normal(s) * 0.05)(B, S, D)),
            "wqkv": _w((lambda *s: _rng.normal(s) * 0.05)(D, 3 * D)),
            "wo": _w((lambda *s: _rng.normal(s) * 0.05)(D, D)),
        }
    _A_in = _A_setup()

    def _B_setup():
        B, S, D, F, C = 1, 2048, 1024, 3584, 1
        return {
            "x": _w((lambda *s: _rng.normal(s) * 0.05)(B, S, D)),
            "w_r": _w((lambda *s: _rng.normal(s) * 0.05)(D)),
            "w_gate": _w((lambda *s: _rng.normal(s) * 0.05)(D, F)),
            "w_up": _w((lambda *s: _rng.normal(s) * 0.05)(D, F)),
            "w_down": _w((lambda *s: _rng.normal(s) * 0.05)(F, D)),
        }
    _B_in = _B_setup()

    return {
        "A_x": _A_in["x"],
        "A_wqkv": _A_in["wqkv"],
        "A_wo": _A_in["wo"],
        "B_x": _B_in["x"],
        "B_w_r": _B_in["w_r"],
        "B_w_gate": _B_in["w_gate"],
        "B_w_up": _B_in["w_up"],
        "B_w_down": _B_in["w_down"],
    }

def reference(A_x, A_wqkv, A_wo, B_x, B_w_r, B_w_gate, B_w_up, B_w_down):
    def _A_ref(x, wqkv, wo):
        B, S, D = x.shape
        H = 32; Dh = D // H; W = 256
        qkv = (lambda x, *d: x.transpose(*d))((x @ wqkv).reshape(B, S, 3, H, Dh), 2, 0, 3, 1, 4)
        q, k, v = qkv[0], qkv[1], qkv[2]
        scores = jnp.einsum("bhqd,bhkd->bhqk", q, k) * (Dh ** -0.5)
        idx = jnp.arange(S)
        mask = (idx[:, None] - idx[None, :] >= 0) & (idx[:, None] - idx[None, :] < W)
        scores = jnp.where(mask[None, None], scores, -1e9)
        p = _softmax(scores, axis=-1)
        o = jnp.einsum("bhqk,bhkd->bhqd", p, v)
        return (lambda x, *d: x.transpose(*d))(o, 0, 2, 1, 3).reshape(B, S, D) @ wo

    def _B_ref(x, w_r, w_gate, w_up, w_down):
        B, S, D = x.shape
        C = 1
        r = x @ w_r
        idx = jnp.argsort(-r, axis=-1)[:, :C]
        idx_e = jnp.repeat(idx.reshape(B, C, 1), D, axis=2)
        x_sel = jnp.take_along_axis(x, idx_e, axis=1)
        g = _silu(x_sel @ w_gate)
        u = x_sel @ w_up
        y = (g * u) @ w_down
        r_sel = _sigmoid(jnp.take_along_axis(r, idx, axis=1))
        y = y * r_sel.reshape(B, C, 1)
        b_off = (jnp.arange(B) * S).reshape(B, 1)
        flat_idx = (idx + b_off).reshape(B * C)
        zero = (x * 0.0).reshape(B * S, D)
        upd = _scatter_add(zero, flat_idx, y.reshape(B * C, D), axis=0)
        return x + upd.reshape(B, S, D)

    x = A_x
    x = x + _A_ref(_layernorm(x, axis=-1), A_wqkv, A_wo)
    x = x + _B_ref(_layernorm(x, axis=-1), B_w_r, B_w_gate, B_w_up, B_w_down)
    x = x + _A_ref(_layernorm(x, axis=-1), A_wqkv, A_wo)
    x = x + _B_ref(_layernorm(x, axis=-1), B_w_r, B_w_gate, B_w_up, B_w_down)
    return x
```

```python
import math

import jax
import jax.numpy as jnp
from jax import lax
import jax.experimental.pallas as pl
import jax.experimental.pallas.tpu as pltpu

S = 2048
D = 1024
DH = 32
F = 3584
TB = 256
NTB = S // TB
QB = 128
NQB = S // QB
NG = D // 128
NC = 512
NNC = 3 * D // NC
EPS = 1e-5
QSCALE = (DH ** -0.5) * math.log2(math.e)

BF = jnp.bfloat16
F32 = jnp.float32
I32 = jnp.int32
NT = (((1,), (1,)), ((), ()))


def _pack(v):
    return pltpu.bitcast(v.astype(BF), I32)


def _unpack(v):
    return pltpu.bitcast(v, BF)


def _layernorm(x):
    m = jnp.sum(x, axis=-1, keepdims=True) * (1.0 / D)
    xc = x - m
    v = jnp.sum(xc * xc, axis=-1, keepdims=True) * (1.0 / D)
    return xc * lax.rsqrt(v + EPS)


def _kernel(x_hbm, wqkv_hbm, wo_hbm, wr_ref, wg_hbm, wu_hbm, wd_hbm, out_hbm,
            xio, xf, n1, xn, wqkv, wo, wg, wu, wd, q_s, k_s, vt_s, o_s, r_s,
            x_sem, w_sem, o_sem):

    def x_copy(i):
        rows = pl.ds(pl.multiple_of(i * TB, TB), TB)
        return pltpu.make_async_copy(x_hbm.at[0, rows], xio.at[rows], x_sem.at[i])

    def out_copy(i):
        rows = pl.ds(pl.multiple_of(i * TB, TB), TB)
        return pltpu.make_async_copy(xio.at[rows], out_hbm.at[0, rows], o_sem.at[i])

    def wqkv_copy(j):
        return pltpu.make_async_copy(
            wqkv_hbm.at[:, pl.ds(j * NC, NC)], wqkv.at[j], w_sem.at[j])

    wo_copy = pltpu.make_async_copy(wo_hbm, wo, w_sem.at[NNC])

    def ffn_copies():
        cs = []
        for j in range(F // 128):
            cs.append(pltpu.make_async_copy(
                wg_hbm.at[:, pl.ds(j * 128, 128)], wg.at[j], w_sem.at[NNC + 1]))
            cs.append(pltpu.make_async_copy(
                wu_hbm.at[:, pl.ds(j * 128, 128)], wu.at[j], w_sem.at[NNC + 1]))
        for j in range(D // 128):
            cs.append(pltpu.make_async_copy(
                wd_hbm.at[:, pl.ds(j * 128, 128)], wd.at[j], w_sem.at[NNC + 1]))
        return cs

    x_copy(0).start()
    for j in range(NNC):
        wqkv_copy(j).start()
    for i in range(1, NTB):
        x_copy(i).start()
    wo_copy.start()
    for c in ffn_copies():
        c.start()

    def load_x(i):
        x_copy(i).wait()
        rows = pl.ds(pl.multiple_of(i * TB, TB), TB)
        xf[rows, :] = xio[rows, :].astype(F32)

    def ln_block(i):
        rows = pl.ds(pl.multiple_of(i * TB, TB), TB)
        half = pl.ds(pl.multiple_of(i * (TB // 2), TB // 2), TB // 2)
        xn[half, :] = _pack(_layernorm(xf[rows, :]))

    def qkv_block(i, first):
        half = pl.ds(pl.multiple_of(i * (TB // 2), TB // 2), TB // 2)
        for j in range(NNC):
            @pl.when(first)
            def _():
                wqkv_copy(j).wait()
            y = jnp.dot(_unpack(xn[half, :]), wqkv[j], preferred_element_type=F32)
            kind, c0 = divmod(j * NC, D)
            for c in range(NC // 128):
                g = c0 // 128 + c
                yc = y[:, c * 128:(c + 1) * 128]
                if kind == 0:
                    q_s[g, half, :] = _pack(yc * QSCALE)
                elif kind == 1:
                    k_s[g, half, :] = _pack(yc)
                else:
                    for t in range(TB // QB):
                        vt_s[i * (TB // QB) + t, g * 64:(g + 1) * 64, :] = _pack(
                            yc[t * QB:(t + 1) * QB, :].T)

    def attn_block(qb, nk):
        lane = lax.broadcasted_iota(I32, (QB // 2, 128), 1)
        kk = lax.broadcasted_iota(I32, (QB, QB), 0)
        qq = lax.broadcasted_iota(I32, (QB, QB), 1)
        newest = kk <= qq
        every = jnp.full((QB, QB), -1, I32)
        bits_new = _pack(jnp.where(newest, pltpu.bitcast(every, F32), 0.0)) if False else None
        del every, bits_new
        k2 = lax.broadcasted_iota(I32, (QB // 2, QB), 0) * 2
        q2 = lax.broadcasted_iota(I32, (QB // 2, QB), 1)
        bits_new = jnp.where(k2 <= q2, 0xFFFF, 0) | jnp.where(k2 + 1 <= q2, -65536, 0)
        bits_old = ~bits_new
        qrows = pl.ds(pl.multiple_of(qb * (QB // 2), QB // 2), QB // 2)
        krows = pl.ds(pl.multiple_of((qb - nk + 1) * (QB // 2), QB // 2), nk * QB // 2)
        for g in range(NG):
            qg = q_s[g, qrows, :]
            q4 = jnp.concatenate(
                [jnp.where((lane >= h * DH) & (lane < (h + 1) * DH), qg, 0) for h in range(4)],
                axis=0)
            st = lax.dot_general(_unpack(k_s[g, krows, :]), _unpack(q4), NT,
                                 preferred_element_type=F32)
            outs = []
            for h in range(4):
                sh = st[:, h * QB:(h + 1) * QB]
                s_new = sh[(nk - 1) * QB:]
                s_old = sh[:QB] if nk == 3 else -1e30
                tiles = [jnp.where(newest, s_new, s_old)]
                if nk >= 2:
                    tiles.append(sh[(nk - 2) * QB:(nk - 1) * QB])
                m = tiles[0] if nk == 1 else jnp.maximum(tiles[0], tiles[1])
                m = jnp.max(m, axis=0, keepdims=True)
                ps = [jnp.exp2(t - m) for t in tiles]
                l = ps[0] if nk == 1 else ps[0] + ps[1]
                l = jnp.sum(l, axis=0, keepdims=True)
                pk = [_pack(p) for p in ps]
                if nk == 3:
                    pt = [pk[0] & bits_old, pk[1], pk[0] & bits_new]
                elif nk == 2:
                    pt = [pk[1], pk[0]]
                else:
                    pt = [pk[0]]
                r0 = (g * 4 + h) * (DH // 2)
                vt = jnp.concatenate(
                    [vt_s[qb - nk + 1 + t, r0:r0 + DH // 2, :] for t in range(nk)], axis=1)
                ot = jnp.dot(_unpack(vt), _unpack(jnp.concatenate(pt, axis=0)),
                             preferred_element_type=F32)
                outs.append(ot * (1.0 / l))
            o_s[qrows, g * 128:(g + 1) * 128] = _pack(jnp.concatenate(outs, axis=0).T)

    def out_block(i, last):
        rows = pl.ds(pl.multiple_of(i * TB, TB), TB)
        half = pl.ds(pl.multiple_of(i * (TB // 2), TB // 2), TB // 2)
        x1 = xf[rows, :] + jnp.dot(_unpack(o_s[half, :]), wo[...], preferred_element_type=F32)
        n = _layernorm(x1)
        n1[rows, :] = n
        wr = wr_ref[...].astype(F32).reshape(1, D)
        r_s[rows, :] = jnp.broadcast_to(jnp.sum(n * wr, axis=-1, keepdims=True), (TB, 128))
        x2 = x1 + n
        xf[rows, :] = x2

        @pl.when(last)
        def _():
            xio[rows, :] = xf[rows, :].astype(BF)
            out_copy(i).start()

    def ffn(first, last):
        r = r_s[...]
        rmax = jnp.max(r, axis=0, keepdims=True)
        tok = lax.broadcasted_iota(I32, (S, 128), 0)
        idx = jnp.min(jnp.where(r == rmax, tok, S - 1))
        idx = jnp.clip(idx, 0, S - 1)

        @pl.when(first)
        def _():
            for c in ffn_copies():
                c.wait()

        xs = jnp.broadcast_to(n1[pl.ds(idx, 1), :], (16, D)).astype(BF)
        hs = []
        for j in range(F // 128):
            gj = jnp.dot(xs, wg[j], preferred_element_type=F32)
            uj = jnp.dot(xs, wu[j], preferred_element_type=F32)
            hs.append((gj * jax.nn.sigmoid(gj) * uj).astype(BF))
        hid = jnp.concatenate(hs, axis=1)
        y = jnp.concatenate(
            [jnp.dot(hid, wd[j], preferred_element_type=F32) for j in range(D // 128)], axis=1)
        gate = jax.nn.sigmoid(rmax[:, 0:1])
        xf[pl.ds(idx, 1), :] = xf[pl.ds(idx, 1), :] + y[0:1, :] * gate

        @pl.when(last)
        def _():
            for i in range(NTB):
                out_copy(i).wait()
            rows = pl.ds(pl.multiple_of((idx // 16) * 16, 16), 16)
            xio[rows, :] = xf[rows, :].astype(BF)
            fix = pltpu.make_async_copy(xio.at[rows], out_hbm.at[0, rows], o_sem.at[0])
            fix.start()
            fix.wait()

    def layer(l, carry):
        first = l == 0
        last = l == 1

        def qkv_body(i, c):
            @pl.when(first)
            def _():
                load_x(i)
            ln_block(i)
            qkv_block(i, first & (i == 0))
            return c
        lax.fori_loop(0, NTB, qkv_body, 0)

        attn_block(0, 1)
        attn_block(1, 2)

        def attn_body(qb, c):
            attn_block(qb, 3)
            return c
        lax.fori_loop(2, NQB, attn_body, 0)

        @pl.when(first)
        def _():
            wo_copy.wait()

        def out_body(i, c):
            out_block(i, last)
            return c
        lax.fori_loop(0, NTB, out_body, 0)

        ffn(first, last)
        return carry

    lax.fori_loop(0, 2, layer, 0)


@jax.jit
def pallas_interleave_layers__sliding_block__moe_arch_mod__prompt_kernel(
    A_x: jax.Array,
    A_wqkv: jax.Array,
    A_wo: jax.Array,
    B_x: jax.Array,
    B_w_r: jax.Array,
    B_w_gate: jax.Array,
    B_w_up: jax.Array,
    B_w_down: jax.Array,
):
    del B_x
    hbm = pl.BlockSpec(memory_space=pl.ANY)
    return pl.pallas_call(
        _kernel,
        in_specs=[hbm, hbm, hbm, pl.BlockSpec(memory_space=pltpu.VMEM), hbm, hbm, hbm],
        out_specs=hbm,
        out_shape=jax.ShapeDtypeStruct((1, S, D), BF),
        scratch_shapes=[
            pltpu.VMEM((S, D), BF),
            pltpu.VMEM((S, D), F32),
            pltpu.VMEM((S, D), F32),
            pltpu.VMEM((S // 2, D), I32),
            pltpu.VMEM((NNC, D, NC), BF),
            pltpu.VMEM((D, D), BF),
            pltpu.VMEM((F // 128, D, 128), BF),
            pltpu.VMEM((F // 128, D, 128), BF),
            pltpu.VMEM((D // 128, F, 128), BF),
            pltpu.VMEM((NG, S // 2, 128), I32),
            pltpu.VMEM((NG, S // 2, 128), I32),
            pltpu.VMEM((NQB, D // 2, QB), I32),
            pltpu.VMEM((S // 2, D), I32),
            pltpu.VMEM((S, 128), F32),
            pltpu.SemaphoreType.DMA((NTB,)),
            pltpu.SemaphoreType.DMA((NNC + 2,)),
            pltpu.SemaphoreType.DMA((NTB,)),
        ],
        compiler_params=pltpu.CompilerParams(vmem_limit_bytes=100 * 1024 * 1024),
        name="mod_swa",
    )(A_x, A_wqkv, A_wo, B_w_r, B_w_gate, B_w_up, B_w_down)
```

```python
import math

import jax
import jax.numpy as jnp
from jax import lax
import jax.experimental.pallas as pl
import jax.experimental.pallas.tpu as pltpu

S = 2048
D = 1024
DH = 32
F = 3584
TB = 256
NTB = S // TB
QB = 128
NQB = S // QB
NG = D // 128
NC = 512
NNC = 3 * D // NC
EPS = 1e-5
QSCALE = (DH ** -0.5) * math.log2(math.e)

BF = jnp.bfloat16
F32 = jnp.float32
I32 = jnp.int32
NT = (((1,), (1,)), ((), ()))


def _pack(v):
    return pltpu.bitcast(v.astype(BF), I32)


def _unpack(v):
    return pltpu.bitcast(v, BF)


def _layernorm(x):
    m = jnp.sum(x, axis=-1, keepdims=True) * (1.0 / D)
    xc = x - m
    v = jnp.sum(xc * xc, axis=-1, keepdims=True) * (1.0 / D)
    return xc * lax.rsqrt(v + EPS)


def _kernel(x_hbm, wqkv_hbm, wo_hbm, wr_ref, wg_hbm, wu_hbm, wd_hbm, out_hbm,
            xio, xf, n1, xn, wqkv, wo, wg, wu, wd, q_s, k_s, vt_s, o_s, r_s, s_s, m_s,
            x_sem, w_sem, o_sem):

    def x_copy(i):
        rows = pl.ds(pl.multiple_of(i * TB, TB), TB)
        return pltpu.make_async_copy(x_hbm.at[0, rows], xio.at[rows], x_sem.at[i])

    def out_copy(i):
        rows = pl.ds(pl.multiple_of(i * TB, TB), TB)
        return pltpu.make_async_copy(xio.at[rows], out_hbm.at[0, rows], o_sem.at[i])

    def wqkv_copy(j):
        return pltpu.make_async_copy(
            wqkv_hbm.at[:, pl.ds(j * NC, NC)], wqkv.at[j], w_sem.at[j])

    wo_copy = pltpu.make_async_copy(wo_hbm, wo, w_sem.at[NNC])

    def ffn_copies():
        cs = []
        for j in range(F // 128):
            cs.append(pltpu.make_async_copy(
                wg_hbm.at[:, pl.ds(j * 128, 128)], wg.at[j], w_sem.at[NNC + 1]))
            cs.append(pltpu.make_async_copy(
                wu_hbm.at[:, pl.ds(j * 128, 128)], wu.at[j], w_sem.at[NNC + 1]))
        for j in range(D // 128):
            cs.append(pltpu.make_async_copy(
                wd_hbm.at[:, pl.ds(j * 128, 128)], wd.at[j], w_sem.at[NNC + 1]))
        return cs

    x_copy(0).start()
    for j in range(NNC):
        wqkv_copy(j).start()
    for i in range(1, NTB):
        x_copy(i).start()
    wo_copy.start()

    def load_x(i):
        x_copy(i).wait()
        rows = pl.ds(pl.multiple_of(i * TB, TB), TB)
        xf[rows, :] = xio[rows, :].astype(F32)

    def ln_block(i):
        rows = pl.ds(pl.multiple_of(i * TB, TB), TB)
        half = pl.ds(pl.multiple_of(i * (TB // 2), TB // 2), TB // 2)
        xn[half, :] = _pack(_layernorm(xf[rows, :]))

    def qkv_block(i, first):
        half = pl.ds(pl.multiple_of(i * (TB // 2), TB // 2), TB // 2)
        for j in range(NNC):
            @pl.when(first)
            def _():
                wqkv_copy(j).wait()
            y = jnp.dot(_unpack(xn[half, :]), wqkv[j], preferred_element_type=F32)
            kind, c0 = divmod(j * NC, D)
            for c in range(NC // 128):
                g = c0 // 128 + c
                yc = y[:, c * 128:(c + 1) * 128]
                if kind == 0:
                    q_s[g, half, :] = _pack(yc * QSCALE)
                elif kind == 1:
                    k_s[g, half, :] = _pack(yc)
                else:
                    for t in range(TB // QB):
                        vt_s[i * (TB // QB) + t, g * 64:(g + 1) * 64, :] = _pack(
                            yc[t * QB:(t + 1) * QB, :].T)

    def tri():
        kk = lax.broadcasted_iota(I32, (QB, QB), 0)
        qq = lax.broadcasted_iota(I32, (QB, QB), 1)
        return kk <= qq

    def scores(qb, g, nk, slot):
        lane = lax.broadcasted_iota(I32, (QB // 2, 128), 1)
        newest = tri()
        qrows = pl.ds(pl.multiple_of(qb * (QB // 2), QB // 2), QB // 2)
        qg = q_s[g, qrows, :]
        q4 = jnp.concatenate(
            [jnp.where((lane >= h * DH) & (lane < (h + 1) * DH), qg, 0) for h in range(4)],
            axis=0)
        order = [0, 2, 1][:nk] if nk == 3 else [0, 1][:nk]
        pieces = []
        for c in range(QB // 16):
            for back in order:
                r0 = pl.multiple_of((qb - back) * (QB // 2) + c * 8, 8)
                pieces.append(k_s[g, pl.ds(r0, 8), :])
        st = lax.dot_general(_unpack(jnp.concatenate(pieces, axis=0)), _unpack(q4), NT,
                             preferred_element_type=F32)
        ms = [None] * 4
        for c in range(QB // 16):
            base = c * 16 * nk
            for h in range(4):
                cols = slice(h * QB, (h + 1) * QB)
                s_new = st[base:base + 16, cols]
                s_old = st[base + 16:base + 32, cols] if nk == 3 else -1e30
                t = jnp.where(newest[c * 16:(c + 1) * 16], s_new, s_old)
                s_s[slot, h, c * 16:(c + 1) * 16, :] = t
                if nk >= 2:
                    u = st[base + 16 * (nk - 1):base + 16 * nk, cols]
                    s_s[slot, h, QB + c * 16:QB + (c + 1) * 16, :] = u
                    t = jnp.maximum(t, u)
                t = jnp.maximum(t[:8], t[8:])
                ms[h] = t if ms[h] is None else jnp.maximum(ms[h], t)
        for h in range(4):
            m_s[slot, h] = jnp.broadcast_to(jnp.max(ms[h], axis=0, keepdims=True), (8, QB))

    def softmax_pv(qb, g, nk, slot):
        newest = tri()
        qrows = pl.ds(pl.multiple_of(qb * (QB // 2), QB // 2), QB // 2)
        outs = []
        for h in range(4):
            m = m_s[slot, h][0:1]
            p0 = jnp.exp2(s_s[slot, h, 0:QB, :] - m)
            l = p0
            if nk == 3:
                pt = [jnp.where(newest, p0, 0.0), jnp.where(newest, 0.0, p0)]
                backs = [0, 2, 1]
            else:
                pt = [p0]
                backs = [0, 1][:nk]
            if nk >= 2:
                p1 = jnp.exp2(s_s[slot, h, QB:2 * QB, :] - m)
                l = l + p1
                pt.append(p1)
            l = jnp.sum(l, axis=0, keepdims=True)
            r0 = (g * 4 + h) * (DH // 2)
            vt = jnp.concatenate([vt_s[qb - b, r0:r0 + DH // 2, :] for b in backs], axis=1)
            ot = jnp.dot(_unpack(vt), jnp.concatenate(pt, axis=0).astype(BF),
                         preferred_element_type=F32)
            outs.append(ot * (1.0 / l))
        o_s[qrows, g * 128:(g + 1) * 128] = _pack(jnp.concatenate(outs, axis=0).T)

    def attn_block(qb, nk, nxt, nk_nxt):
        for g in range(NG):
            if g + 1 < NG:
                scores(qb, g + 1, nk, (g + 1) % 2)
            else:
                scores(nxt, 0, nk_nxt, 0)
            softmax_pv(qb, g, nk, g % 2)

    def out_block(i, last):
        rows = pl.ds(pl.multiple_of(i * TB, TB), TB)
        half = pl.ds(pl.multiple_of(i * (TB // 2), TB // 2), TB // 2)
        x1 = xf[rows, :] + jnp.dot(_unpack(o_s[half, :]), wo[...], preferred_element_type=F32)
        n = _layernorm(x1)
        n1[rows, :] = n
        wr = wr_ref[...].astype(F32).reshape(1, D)
        r_s[rows, :] = jnp.broadcast_to(jnp.sum(n * wr, axis=-1, keepdims=True), (TB, 128))
        x2 = x1 + n
        xf[rows, :] = x2

        @pl.when(last)
        def _():
            xio[rows, :] = xf[rows, :].astype(BF)
            out_copy(i).start()

    def ffn(first, last):
        r = r_s[...]
        rmax = jnp.max(r, axis=0, keepdims=True)
        tok = lax.broadcasted_iota(I32, (S, 128), 0)
        idx = jnp.min(jnp.where(r == rmax, tok, S - 1))
        idx = jnp.clip(idx, 0, S - 1)

        @pl.when(first)
        def _():
            for c in ffn_copies():
                c.wait()

        xs = jnp.broadcast_to(n1[pl.ds(idx, 1), :], (16, D)).astype(BF)
        hs = []
        for j in range(F // 128):
            gj = jnp.dot(xs, wg[j], preferred_element_type=F32)
            uj = jnp.dot(xs, wu[j], preferred_element_type=F32)
            hs.append((gj * jax.nn.sigmoid(gj) * uj).astype(BF))
        hid = jnp.concatenate(hs, axis=1)
        y = jnp.concatenate(
            [jnp.dot(hid, wd[j], preferred_element_type=F32) for j in range(D // 128)], axis=1)
        gate = jax.nn.sigmoid(rmax[:, 0:1])
        xf[pl.ds(idx, 1), :] = xf[pl.ds(idx, 1), :] + y[0:1, :] * gate

        @pl.when(last)
        def _():
            for i in range(NTB):
                out_copy(i).wait()
            rows = pl.ds(pl.multiple_of((idx // 16) * 16, 16), 16)
            xio[rows, :] = xf[rows, :].astype(BF)
            fix = pltpu.make_async_copy(xio.at[rows], out_hbm.at[0, rows], o_sem.at[0])
            fix.start()
            fix.wait()

    def layer(l, carry):
        first = l == 0
        last = l == 1

        def qkv_body(i, c):
            @pl.when(first)
            def _():
                load_x(i)
            ln_block(i)
            qkv_block(i, first & (i == 0))
            return c
        lax.fori_loop(0, NTB, qkv_body, 0)

        @pl.when(first)
        def _():
            for c in ffn_copies():
                c.start()

        scores(0, 0, 1, 0)
        attn_block(0, 1, 1, 2)
        attn_block(1, 2, 2, 3)

        def attn_body(qb, c):
            attn_block(qb, 3, jnp.minimum(qb + 1, NQB - 1), 3)
            return c
        lax.fori_loop(2, NQB, attn_body, 0)

        @pl.when(first)
        def _():
            wo_copy.wait()

        def out_body(i, c):
            out_block(i, last)
            return c
        lax.fori_loop(0, NTB, out_body, 0)

        ffn(first, last)
        return carry

    lax.fori_loop(0, 2, layer, 0)


@jax.jit
def pallas_interleave_layers__sliding_block__moe_arch_mod__prompt_kernel(
    A_x: jax.Array,
    A_wqkv: jax.Array,
    A_wo: jax.Array,
    B_x: jax.Array,
    B_w_r: jax.Array,
    B_w_gate: jax.Array,
    B_w_up: jax.Array,
    B_w_down: jax.Array,
):
    del B_x
    hbm = pl.BlockSpec(memory_space=pl.ANY)
    return pl.pallas_call(
        _kernel,
        in_specs=[hbm, hbm, hbm, pl.BlockSpec(memory_space=pltpu.VMEM), hbm, hbm, hbm],
        out_specs=hbm,
        out_shape=jax.ShapeDtypeStruct((1, S, D), BF),
        scratch_shapes=[
            pltpu.VMEM((S, D), BF),
            pltpu.VMEM((S, D), F32),
            pltpu.VMEM((S, D), F32),
            pltpu.VMEM((S // 2, D), I32),
            pltpu.VMEM((NNC, D, NC), BF),
            pltpu.VMEM((D, D), BF),
            pltpu.VMEM((F // 128, D, 128), BF),
            pltpu.VMEM((F // 128, D, 128), BF),
            pltpu.VMEM((D // 128, F, 128), BF),
            pltpu.VMEM((NG, S // 2, 128), I32),
            pltpu.VMEM((NG, S // 2, 128), I32),
            pltpu.VMEM((NQB, D // 2, QB), I32),
            pltpu.VMEM((S // 2, D), I32),
            pltpu.VMEM((S, 128), F32),
            pltpu.VMEM((2, 4, 2 * QB, QB), F32),
            pltpu.VMEM((2, 4, 8, QB), F32),
            pltpu.SemaphoreType.DMA((NTB,)),
            pltpu.SemaphoreType.DMA((NNC + 2,)),
            pltpu.SemaphoreType.DMA((NTB,)),
        ],
        compiler_params=pltpu.CompilerParams(vmem_limit_bytes=100 * 1024 * 1024),
        name="mod_swa",
    )(A_x, A_wqkv, A_wo, B_w_r, B_w_gate, B_w_up, B_w_down)
```

```python
import math

import jax
import jax.numpy as jnp
from jax import lax
import jax.experimental.pallas as pl
import jax.experimental.pallas.tpu as pltpu

S = 2048
D = 1024
DH = 32
F = 3584
TB = 256
NTB = S // TB
QB = 128
NQB = S // QB
NG = D // 128
NC = 512
NNC = 3 * D // NC
EPS = 1e-5
QSCALE = (DH ** -0.5) * math.log2(math.e)

BF = jnp.bfloat16
F32 = jnp.float32
I32 = jnp.int32
NT = (((1,), (1,)), ((), ()))


def _pack(v):
    return pltpu.bitcast(v.astype(BF), I32)


def _unpack(v):
    return pltpu.bitcast(v, BF)


def _layernorm(x):
    m = jnp.sum(x, axis=-1, keepdims=True) * (1.0 / D)
    xc = x - m
    v = jnp.sum(xc * xc, axis=-1, keepdims=True) * (1.0 / D)
    return xc * lax.rsqrt(v + EPS)


def _rows(i, n):
    return pl.ds(i * n if isinstance(i, int) else pl.multiple_of(i * n, n), n)


def _kernel(x_hbm, wqkv_hbm, wo_hbm, wr_ref, wg_hbm, wu_hbm, wd_hbm, out_hbm,
            x_s, n_s, xn, wqkv, wo, wg, wu, wd, q_s, k_s, vt_s, o_s, ot_s, r_s, s_s, m_s,
            x_sem, w_sem, o_sem):

    def x_copy(i):
        return pltpu.make_async_copy(x_hbm.at[0, _rows(i, TB)], x_s.at[_rows(i, TB)],
                                     x_sem.at[i])

    def out_copy(i):
        return pltpu.make_async_copy(x_s.at[_rows(i, QB)], out_hbm.at[0, _rows(i, QB)],
                                     o_sem.at[i])

    def wqkv_copy(j):
        return pltpu.make_async_copy(
            wqkv_hbm.at[:, pl.ds(j * NC, NC)], wqkv.at[j], w_sem.at[j])

    wo_copy = pltpu.make_async_copy(wo_hbm, wo, w_sem.at[NNC])

    def ffn_copies():
        cs = []
        for j in range(F // 128):
            cs.append(pltpu.make_async_copy(
                wg_hbm.at[:, pl.ds(j * 128, 128)], wg.at[j], w_sem.at[NNC + 1]))
            cs.append(pltpu.make_async_copy(
                wu_hbm.at[:, pl.ds(j * 128, 128)], wu.at[j], w_sem.at[NNC + 1]))
        for j in range(D // 128):
            cs.append(pltpu.make_async_copy(
                wd_hbm.at[:, pl.ds(j * 128, 128)], wd.at[j], w_sem.at[NNC + 1]))
        return cs

    def ln_rows(r0, n):
        x = x_s[pl.ds(pl.multiple_of(r0, n), n), :].astype(F32)
        xn[pl.ds(pl.multiple_of(r0 // 2, n // 2), n // 2), :] = _pack(_layernorm(x))

    def qkv_block(i, nxt, startup):
        half = _rows(i, TB // 2)
        for j in range(NNC):
            if startup:
                wqkv_copy(j).wait()
                if j + 2 < NNC:
                    wqkv_copy(j + 2).start()
                elif j + 2 == NNC:
                    x_copy(1).start()
                else:
                    for b in range(2, NTB):
                        x_copy(b).start()
                    wo_copy.start()
            y = jnp.dot(_unpack(xn[half, :]), wqkv[j], preferred_element_type=F32)
            kind, c0 = divmod(j * NC, D)
            for c in range(NC // 128):
                g = c0 // 128 + c
                yc = y[:, c * 128:(c + 1) * 128]
                if kind == 0:
                    q_s[g, half, :] = _pack(yc * QSCALE)
                elif kind == 1:
                    k_s[g, half, :] = _pack(yc)
                else:
                    for t in range(TB // QB):
                        vt_s[i * (TB // QB) + t, g * 64:(g + 1) * 64, :] = _pack(
                            yc[t * QB:(t + 1) * QB, :].T)
            if startup:
                if j == NNC - 2:
                    x_copy(1).wait()
                    ln_rows(nxt * TB, TB)
            elif j < 4:
                ln_rows(nxt * TB + j * (TB // 4), TB // 4)

    def tri():
        kk = lax.broadcasted_iota(I32, (QB, QB), 0)
        qq = lax.broadcasted_iota(I32, (QB, QB), 1)
        return kk <= qq

    def scores(qb, g, nk, slot):
        lane = lax.broadcasted_iota(I32, (QB // 2, 128), 1)
        newest = tri()
        qg = q_s[g, _rows(qb, QB // 2), :]
        q4 = jnp.concatenate(
            [jnp.where((lane >= h * DH) & (lane < (h + 1) * DH), qg, 0) for h in range(4)],
            axis=0)
        order = [0, 2, 1] if nk == 3 else [0, 1][:nk]
        tiles = {b: k_s[g, _rows(qb - b, QB // 2), :] for b in order}
        pieces = [tiles[b][c * 8:(c + 1) * 8] for c in range(QB // 16) for b in order]
        st = lax.dot_general(_unpack(jnp.concatenate(pieces, axis=0)), _unpack(q4), NT,
                             preferred_element_type=F32)
        ms = [None] * 4
        for c in range(QB // 16):
            base = c * 16 * nk
            for h in range(4):
                cols = slice(h * QB, (h + 1) * QB)
                s_new = st[base:base + 16, cols]
                s_old = st[base + 16:base + 32, cols] if nk == 3 else -1e30
                t = jnp.where(newest[c * 16:(c + 1) * 16], s_new, s_old)
                s_s[slot, h, c * 16:(c + 1) * 16, :] = t
                if nk >= 2:
                    u = st[base + 16 * (nk - 1):base + 16 * nk, cols]
                    s_s[slot, h, QB + c * 16:QB + (c + 1) * 16, :] = u
                    t = jnp.maximum(t, u)
                t = jnp.maximum(t[:8], t[8:])
                ms[h] = t if ms[h] is None else jnp.maximum(ms[h], t)
        for h in range(4):
            m_s[slot, h] = ms[h]

    def softmax_pv(qb, g, nk, slot):
        newest = tri()
        outs = []
        for h in range(4):
            m = jnp.max(m_s[slot, h], axis=0, keepdims=True)
            p0 = jnp.exp2(s_s[slot, h, 0:QB, :] - m)
            l = p0
            if nk == 3:
                pt = [jnp.where(newest, p0, 0.0), jnp.where(newest, 0.0, p0)]
                backs = [0, 2, 1]
            else:
                pt = [p0]
                backs = [0, 1][:nk]
            if nk >= 2:
                p1 = jnp.exp2(s_s[slot, h, QB:2 * QB, :] - m)
                l = l + p1
                pt.append(p1)
            l = jnp.sum(l, axis=0, keepdims=True)
            r0 = (g * 4 + h) * (DH // 2)
            vt = jnp.concatenate([vt_s[qb - b, r0:r0 + DH // 2, :] for b in backs], axis=1)
            ot = jnp.dot(_unpack(vt), jnp.concatenate(pt, axis=0).astype(BF),
                         preferred_element_type=F32)
            outs.append(ot * (1.0 / l))
        ot = jnp.concatenate(outs, axis=0)
        if g + 1 < NG:
            o_s[_rows(qb, QB // 2), g * 128:(g + 1) * 128] = _pack(ot.T)
        else:
            ot_s[...] = ot

    def out_block(i):
        rows = _rows(i, QB)
        o = jnp.concatenate(
            [o_s[_rows(i, QB // 2), 0:D - 128], _pack(ot_s[...].T)], axis=1)
        x1 = x_s[rows, :].astype(F32) + jnp.dot(_unpack(o), wo[...],
                                                preferred_element_type=F32)
        n = _layernorm(x1)
        n_s[rows, :] = n
        wr = wr_ref[...].astype(F32).reshape(1, D)
        r_s[rows, :] = jnp.broadcast_to(jnp.sum(n * wr, axis=-1, keepdims=True), (QB, 128))
        x_s[rows, :] = (x1 + n).astype(BF)

    def attn_block(qb, nk, nxt, nk_nxt):
        for g in range(NG):
            if g + 1 < NG:
                scores(qb, g + 1, nk, (g + 1) % 2)
            else:
                scores(nxt, 0, nk_nxt, 0)
            softmax_pv(qb, g, nk, g % 2)
            if g == 0 and nk > 1:
                out_block(qb - 1)

    def ffn(first, last):
        r = r_s[...]
        rmax = jnp.max(r, axis=0, keepdims=True)
        tok = lax.broadcasted_iota(I32, (S, 128), 0)
        idx = jnp.min(jnp.where(r == rmax, tok, S - 1))
        idx = jnp.clip(idx, 0, S - 1)

        @pl.when(first)
        def _():
            for c in ffn_copies():
                c.wait()

        xs = jnp.broadcast_to(n_s[pl.ds(idx, 1), :], (16, D)).astype(BF)
        hs = []
        for j in range(F // 128):
            gj = jnp.dot(xs, wg[j], preferred_element_type=F32)
            uj = jnp.dot(xs, wu[j], preferred_element_type=F32)
            hs.append((gj * jax.nn.sigmoid(gj) * uj).astype(BF))
        hid = jnp.concatenate(hs, axis=1)
        y = jnp.concatenate(
            [jnp.dot(hid, wd[j], preferred_element_type=F32) for j in range(D // 128)], axis=1)
        y = y * jax.nn.sigmoid(rmax[:, 0:1])

        @pl.when(last)
        def _():
            for i in range(NQB):
                out_copy(i).wait()

        rows = _rows(idx // 16, 16)
        x = x_s[rows, :].astype(F32)
        sel = lax.broadcasted_iota(I32, (16, D), 0) == idx % 16
        x_s[rows, :] = jnp.where(sel, x + y, x).astype(BF)

        @pl.when(last)
        def _():
            fix = pltpu.make_async_copy(x_s.at[rows], out_hbm.at[0, rows], o_sem.at[0])
            fix.start()
            fix.wait()

    x_copy(0).start()
    wqkv_copy(0).start()
    wqkv_copy(1).start()
    x_copy(0).wait()
    ln_rows(0, TB)
    qkv_block(0, 1, True)

    def layer(l, carry):
        first = l == 0
        last = l == 1

        @pl.when(last)
        def _():
            ln_rows(0, TB)

        def qkv_body(i, c):
            @pl.when(first & (i + 1 < NTB))
            def _():
                x_copy(i + 1).wait()
            qkv_block(i, (i + 1) % NTB, False)
            return c
        lax.fori_loop(1 - l, NTB, qkv_body, 0)

        @pl.when(first)
        def _():
            for c in ffn_copies():
                c.start()
            wo_copy.wait()

        scores(0, 0, 1, 0)
        attn_block(0, 1, 1, 2)
        attn_block(1, 2, 2, 3)

        def attn_body(qb, c):
            @pl.when(last)
            def _():
                out_copy(qb - 2).start()
            attn_block(qb, 3, jnp.minimum(qb + 1, NQB - 1), 3)
            return c
        lax.fori_loop(2, NQB, attn_body, 0)

        @pl.when(last)
        def _():
            out_copy(NQB - 2).start()
        out_block(NQB - 1)

        @pl.when(last)
        def _():
            out_copy(NQB - 1).start()

        ffn(first, last)
        return carry

    lax.fori_loop(0, 2, layer, 0)


@jax.jit
def pallas_interleave_layers__sliding_block__moe_arch_mod__prompt_kernel(
    A_x: jax.Array,
    A_wqkv: jax.Array,
    A_wo: jax.Array,
    B_x: jax.Array,
    B_w_r: jax.Array,
    B_w_gate: jax.Array,
    B_w_up: jax.Array,
    B_w_down: jax.Array,
):
    del B_x
    hbm = pl.BlockSpec(memory_space=pl.ANY)
    return pl.pallas_call(
        _kernel,
        in_specs=[hbm, hbm, hbm, pl.BlockSpec(memory_space=pltpu.VMEM), hbm, hbm, hbm],
        out_specs=hbm,
        out_shape=jax.ShapeDtypeStruct((1, S, D), BF),
        scratch_shapes=[
            pltpu.VMEM((S, D), BF),
            pltpu.VMEM((S, D), F32),
            pltpu.VMEM((S // 2, D), I32),
            pltpu.VMEM((NNC, D, NC), BF),
            pltpu.VMEM((D, D), BF),
            pltpu.VMEM((F // 128, D, 128), BF),
            pltpu.VMEM((F // 128, D, 128), BF),
            pltpu.VMEM((D // 128, F, 128), BF),
            pltpu.VMEM((NG, S // 2, 128), I32),
            pltpu.VMEM((NG, S // 2, 128), I32),
            pltpu.VMEM((NQB, D // 2, QB), I32),
            pltpu.VMEM((S // 2, D), I32),
            pltpu.VMEM((128, QB), F32),
            pltpu.VMEM((S, 128), F32),
            pltpu.VMEM((2, 4, 2 * QB, QB), F32),
            pltpu.VMEM((2, 4, 8, QB), F32),
            pltpu.SemaphoreType.DMA((NTB,)),
            pltpu.SemaphoreType.DMA((NNC + 2,)),
            pltpu.SemaphoreType.DMA((NQB,)),
        ],
        compiler_params=pltpu.CompilerParams(vmem_limit_bytes=100 * 1024 * 1024),
        name="mod_swa",
    )(A_x, A_wqkv, A_wo, B_w_r, B_w_gate, B_w_up, B_w_down)
```

```python
import math

import jax
import jax.numpy as jnp
from jax import lax
import jax.experimental.pallas as pl
import jax.experimental.pallas.tpu as pltpu

S = 2048
D = 1024
DH = 32
F = 3584
TB = 256
NTB = S // TB
QB = 128
NQB = S // QB
NG = D // 128
NC = 512
NNC = 3 * D // NC
CHUNKS = [4, 5, 2, 3, 0, 1]
SUB = 32
EPS = 1e-5
QSCALE = (DH ** -0.5) * math.log2(math.e)

BF = jnp.bfloat16
F32 = jnp.float32
I32 = jnp.int32
NT = (((1,), (1,)), ((), ()))


def _pack(v):
    return pltpu.bitcast(v.astype(BF), I32)


def _unpack(v):
    return pltpu.bitcast(v, BF)


def _layernorm(x):
    m = jnp.sum(x, axis=-1, keepdims=True) * (1.0 / D)
    xc = x - m
    v = jnp.sum(xc * xc, axis=-1, keepdims=True) * (1.0 / D)
    return xc * lax.rsqrt(v + EPS)


def _rows(i, n):
    return pl.ds(i * n if isinstance(i, int) else pl.multiple_of(i * n, n), n)


def _kernel(x_hbm, wqkv_hbm, wo_hbm, wr_ref, wg_hbm, wu_hbm, wd_hbm, out_hbm,
            x_s, n_s, xn, wqkv, wo, wg, wu, wd, q_s, k_s, vt_s, o_s, ot_s, y_s, r_s, s_s, m_s,
            x_sem, w_sem, o_sem):

    def x_copy(i):
        return pltpu.make_async_copy(x_hbm.at[0, _rows(i, TB)], x_s.at[_rows(i, TB)],
                                     x_sem.at[i])

    def out_copy(i):
        return pltpu.make_async_copy(x_s.at[_rows(i, QB)], out_hbm.at[0, _rows(i, QB)],
                                     o_sem.at[i])

    def wqkv_copy(j):
        return pltpu.make_async_copy(
            wqkv_hbm.at[:, pl.ds(j * NC, NC)], wqkv.at[j], w_sem.at[j])

    wo_copy = pltpu.make_async_copy(wo_hbm, wo, w_sem.at[NNC])

    def ffn_copies():
        cs = []
        for j in range(F // 128):
            cs.append(pltpu.make_async_copy(
                wg_hbm.at[:, pl.ds(j * 128, 128)], wg.at[j], w_sem.at[NNC + 1]))
            cs.append(pltpu.make_async_copy(
                wu_hbm.at[:, pl.ds(j * 128, 128)], wu.at[j], w_sem.at[NNC + 1]))
        for j in range(D // 128):
            cs.append(pltpu.make_async_copy(
                wd_hbm.at[:, pl.ds(j * 128, 128)], wd.at[j], w_sem.at[NNC + 1]))
        return cs

    def ln_rows(i, r0, n):
        x = x_s[pl.ds(pl.multiple_of(i * TB + r0, n), n), :].astype(F32)
        xn[0, r0 // 2:(r0 + n) // 2, :] = _pack(_layernorm(x))

    def lane_group(n):
        return lax.broadcasted_iota(I32, (n, 128), 1) // DH

    def store_q(i, g, q):
        grp = lane_group(SUB // 2)
        rolled = [q] + [pltpu.roll(q, DH * t, 1) for t in range(1, 4)]
        for h in range(4):
            parts = []
            for c in range(TB // SUB):
                b = c % 4
                rows = slice(c * SUB // 2, (c + 1) * SUB // 2)
                parts.append(jnp.where(grp == b, rolled[(b - h) % 4][rows], 0))
            q_s[g * 4 + h, _rows(i, TB // 2), :] = jnp.concatenate(parts, axis=0)

    def store_k(i, g, k):
        grp = lane_group(TB // 2)
        even = grp % 2 == 0
        low = grp < 2
        pairs = [jnp.where(even, k, pltpu.roll(k, DH, 1)),
                 jnp.where(even, pltpu.roll(k, 3 * DH, 1), k)]
        for h in range(2):
            swapped = pltpu.roll(pairs[h], 2 * DH, 1)
            k_s[g * 4 + h, _rows(i, TB // 2), :] = jnp.where(low, pairs[h], swapped)
            k_s[g * 4 + h + 2, _rows(i, TB // 2), :] = jnp.where(low, swapped, pairs[h])

    def qkv_block(i, nxt, startup):
        for jj, j in enumerate(CHUNKS):
            if startup:
                wqkv_copy(j).wait()
                if jj + 2 < NNC:
                    wqkv_copy(CHUNKS[jj + 2]).start()
                elif jj + 2 == NNC:
                    x_copy(1).start()
                else:
                    x_copy(1).wait()
                    for b in range(2, NTB):
                        x_copy(b).start()
                    wo_copy.start()
            y = jnp.dot(_unpack(xn[min(jj, 1)]), wqkv[j], preferred_element_type=F32)
            if jj == 0:
                xn[1] = xn[0]
            kind, c0 = divmod(j * NC, D)
            for c in range(NC // 128):
                g = c0 // 128 + c
                yc = y[:, c * 128:(c + 1) * 128]
                if kind == 0:
                    store_q(i, g, _pack(yc * QSCALE))
                elif kind == 1:
                    store_k(i, g, _pack(yc))
                else:
                    for t in range(TB // QB):
                        vt_s[i * (TB // QB) + t, g * 64:(g + 1) * 64, :] = _pack(
                            yc[t * QB:(t + 1) * QB, :].T)
            if startup:
                if jj == NNC - 1:
                    for c in range(8):
                        ln_rows(nxt, c * (TB // 8), TB // 8)
            elif 1 <= jj < 5:
                for c in range(2 * jj - 2, 2 * jj):
                    ln_rows(nxt, c * (TB // 8), TB // 8)

    def tri():
        kk = lax.broadcasted_iota(I32, (QB, QB), 0)
        qq = lax.broadcasted_iota(I32, (QB, QB), 1)
        return kk <= qq

    def scores(qb, g, nk, slot):
        kk = lax.broadcasted_iota(I32, (QB, QB), 0)
        qq = lax.broadcasted_iota(I32, (QB, QB), 1)
        grp = lane_group(SUB // 2)
        n = SUB // 2
        for h in range(4):
            hd = g * 4 + h
            tiles = [k_s[hd, _rows(qb - b, QB // 2), :] for b in range(nk)]
            if nk == 3:
                new, mid, old = tiles
                diag = jnp.where(grp >= 2,
                                 jnp.where(grp >= 3, old[3 * n:], old[2 * n:3 * n]),
                                 jnp.where(grp >= 1, old[n:2 * n], old[:n]))
                lhs = [diag, new[:n]] + [
                    jnp.where(grp >= c, new[c * n:(c + 1) * n], old[c * n:(c + 1) * n])
                    for c in range(1, 4)] + [mid]
            else:
                lhs = tiles
            st = lax.dot_general(_unpack(jnp.concatenate(lhs, axis=0)),
                                 _unpack(q_s[hd, _rows(qb, QB // 2), :]), NT,
                                 preferred_element_type=F32)
            if nk == 3:
                t = jnp.where((kk > qq) & (kk // SUB == qq // SUB),
                              jnp.concatenate([st[:SUB]] * 4, axis=0), st[SUB:SUB + QB])
                st = st[SUB:]
            else:
                t = jnp.where(kk <= qq, st[:QB], -1e30)
            s_s[slot, h, 0:QB, :] = t
            if nk >= 2:
                s_s[slot, h, QB:2 * QB, :] = st[QB:]
                t = jnp.maximum(t, st[QB:])
            m_s[slot, h] = jnp.max(t.reshape(QB // 8, 8, QB), axis=0)

    def softmax_pv(qb, g, nk, slot):
        newest = tri()
        outs = []
        for h in range(4):
            m = jnp.max(m_s[slot, h], axis=0, keepdims=True)
            p0 = jnp.exp2(s_s[slot, h, 0:QB, :] - m)
            l = p0
            if nk == 3:
                pt = [jnp.where(newest, p0, 0.0), jnp.where(newest, 0.0, p0)]
                backs = [0, 2, 1]
            else:
                pt = [p0]
                backs = [0, 1][:nk]
            if nk >= 2:
                p1 = jnp.exp2(s_s[slot, h, QB:2 * QB, :] - m)
                l = l + p1
                pt.append(p1)
            l = jnp.sum(l, axis=0, keepdims=True)
            r0 = (g * 4 + h) * (DH // 2)
            vt = jnp.concatenate([vt_s[qb - b, r0:r0 + DH // 2, :] for b in backs], axis=1)
            ot = jnp.dot(_unpack(vt), jnp.concatenate(pt, axis=0).astype(BF),
                         preferred_element_type=F32)
            outs.append(ot * (1.0 / l))
        ot = jnp.concatenate(outs, axis=0)
        if g + 1 < NG:
            o_s[:, g * 128:(g + 1) * 128] = _pack(ot.T)
        else:
            ot_s[...] = ot

    def out_proj(i):
        o = jnp.concatenate([o_s[...], _pack(ot_s[...].T)], axis=1)
        y_s[...] = x_s[_rows(i, QB), :].astype(F32) + jnp.dot(
            _unpack(o), wo[...], preferred_element_type=F32)

    def router(i):
        wr = wr_ref[...].astype(F32).reshape(1, D)
        n = QB // 4
        for c in range(4):
            rows = _rows(i * 4 + c, n)
            x1 = y_s[c * n:(c + 1) * n, :]
            xn1 = _layernorm(x1)
            n_s[rows, :] = xn1
            r_s[rows, :] = jnp.broadcast_to(jnp.sum(xn1 * wr, axis=-1, keepdims=True), (n, 128))
            x_s[rows, :] = (x1 + xn1).astype(BF)

    def attn_block(qb, nk, nxt, nk_nxt):
        for g in range(NG):
            if g + 1 < NG:
                scores(qb, g + 1, nk, (g + 1) % 2)
            else:
                scores(nxt, 0, nk_nxt, 0)
            if g == 0 and nk > 2:
                router(qb - 2)
            if g == 0 and nk > 1:
                out_proj(qb - 1)
            softmax_pv(qb, g, nk, g % 2)

    def ffn(first, last):
        r = r_s[...]
        rmax = jnp.max(r, axis=0, keepdims=True)
        tok = lax.broadcasted_iota(I32, (S, 128), 0)
        idx = jnp.min(jnp.where(r == rmax, tok, S - 1))
        idx = jnp.clip(idx, 0, S - 1)

        @pl.when(first)
        def _():
            for c in ffn_copies():
                c.wait()

        xs = jnp.broadcast_to(n_s[pl.ds(idx, 1), :], (16, D)).astype(BF)
        hs = []
        for j in range(F // 128):
            gj = jnp.dot(xs, wg[j], preferred_element_type=F32)
            uj = jnp.dot(xs, wu[j], preferred_element_type=F32)
            hs.append((gj * jax.nn.sigmoid(gj) * uj).astype(BF))
        hid = jnp.concatenate(hs, axis=1)
        y = jnp.concatenate(
            [jnp.dot(hid, wd[j], preferred_element_type=F32) for j in range(D // 128)], axis=1)
        y = y * jax.nn.sigmoid(rmax[:, 0:1])

        @pl.when(last)
        def _():
            for i in range(NQB):
                out_copy(i).wait()

        rows = _rows(idx // 16, 16)
        x = x_s[rows, :].astype(F32)
        sel = lax.broadcasted_iota(I32, (16, D), 0) == idx % 16
        x_s[rows, :] = jnp.where(sel, x + y, x).astype(BF)

        @pl.when(last)
        def _():
            fix = pltpu.make_async_copy(x_s.at[rows], out_hbm.at[0, rows], o_sem.at[0])
            fix.start()
            fix.wait()

    x_copy(0).start()
    wqkv_copy(CHUNKS[0]).start()
    wqkv_copy(CHUNKS[1]).start()
    x_copy(0).wait()
    ln_rows(0, 0, TB)
    qkv_block(0, 1, True)

    def layer(l, carry):
        first = l == 0
        last = l == 1

        @pl.when(last)
        def _():
            ln_rows(0, 0, TB)

        def qkv_body(i, c):
            @pl.when(first & (i + 1 < NTB))
            def _():
                x_copy(i + 1).wait()
            qkv_block(i, (i + 1) % NTB, False)
            return c
        lax.fori_loop(1 - l, NTB, qkv_body, 0)

        @pl.when(first)
        def _():
            for c in ffn_copies():
                c.start()
            wo_copy.wait()

        scores(0, 0, 1, 0)
        attn_block(0, 1, 1, 2)
        attn_block(1, 2, 2, 3)

        def attn_body(qb, c):
            @pl.when(last & (qb > 2))
            def _():
                out_copy(qb - 3).start()
            attn_block(qb, 3, jnp.minimum(qb + 1, NQB - 1), 3)
            return c
        lax.fori_loop(2, NQB, attn_body, 0)

        router(NQB - 2)
        out_proj(NQB - 1)
        router(NQB - 1)

        @pl.when(last)
        def _():
            for i in range(NQB - 3, NQB):
                out_copy(i).start()

        ffn(first, last)
        return carry

    lax.fori_loop(0, 2, layer, 0)


@jax.jit
def pallas_interleave_layers__sliding_block__moe_arch_mod__prompt_kernel(
    A_x: jax.Array,
    A_wqkv: jax.Array,
    A_wo: jax.Array,
    B_x: jax.Array,
    B_w_r: jax.Array,
    B_w_gate: jax.Array,
    B_w_up: jax.Array,
    B_w_down: jax.Array,
):
    del B_x
    hbm = pl.BlockSpec(memory_space=pl.ANY)
    return pl.pallas_call(
        _kernel,
        in_specs=[hbm, hbm, hbm, pl.BlockSpec(memory_space=pltpu.VMEM), hbm, hbm, hbm],
        out_specs=hbm,
        out_shape=jax.ShapeDtypeStruct((1, S, D), BF),
        scratch_shapes=[
            pltpu.VMEM((S, D), BF),
            pltpu.VMEM((S, D), F32),
            pltpu.VMEM((2, TB // 2, D), I32),
            pltpu.VMEM((NNC, D, NC), BF),
            pltpu.VMEM((D, D), BF),
            pltpu.VMEM((F // 128, D, 128), BF),
            pltpu.VMEM((F // 128, D, 128), BF),
            pltpu.VMEM((D // 128, F, 128), BF),
            pltpu.VMEM((4 * NG, S // 2, 128), I32),
            pltpu.VMEM((4 * NG, S // 2, 128), I32),
            pltpu.VMEM((NQB, D // 2, QB), I32),
            pltpu.VMEM((QB // 2, D - 128), I32),
            pltpu.VMEM((128, QB), F32),
            pltpu.VMEM((QB, D), F32),
            pltpu.VMEM((S, 128), F32),
            pltpu.VMEM((2, 4, 2 * QB, QB), F32),
            pltpu.VMEM((2, 4, 8, QB), F32),
            pltpu.SemaphoreType.DMA((NTB,)),
            pltpu.SemaphoreType.DMA((NNC + 2,)),
            pltpu.SemaphoreType.DMA((NQB,)),
        ],
        compiler_params=pltpu.CompilerParams(vmem_limit_bytes=100 * 1024 * 1024),
        name="mod_swa",
    )(A_x, A_wqkv, A_wo, B_w_r, B_w_gate, B_w_up, B_w_down)
```

```python
import math

import jax
import jax.numpy as jnp
from jax import lax
import jax.experimental.pallas as pl
import jax.experimental.pallas.tpu as pltpu

S = 2048
D = 1024
DH = 32
F = 3584
TB = 256
NTB = S // TB
QB = 128
NQB = S // QB
NG = D // 128
NC = 512
NNC = 3 * D // NC
CHUNKS = [4, 5, 2, 3, 0, 1]
RC = 32
SUB = 32
EPS = 1e-5
QSCALE = (DH ** -0.5) * math.log2(math.e)

BF = jnp.bfloat16
F32 = jnp.float32
I32 = jnp.int32
NT = (((1,), (1,)), ((), ()))


def _pack(v):
    return pltpu.bitcast(v.astype(BF), I32)


def _unpack(v):
    return pltpu.bitcast(v, BF)


def _layernorm(x):
    m = jnp.sum(x, axis=-1, keepdims=True) * (1.0 / D)
    xc = x - m
    v = jnp.sum(xc * xc, axis=-1, keepdims=True) * (1.0 / D)
    return xc * lax.rsqrt(v + EPS)


def _rows(i, n):
    return pl.ds(i * n if isinstance(i, int) else pl.multiple_of(i * n, n), n)


def _kernel(x_hbm, wqkv_hbm, wo_hbm, wr_ref, wg_hbm, wu_hbm, wd_hbm, out_hbm,
            x_s, n_s, xn, wqkv, wo, wg, wu, wd, q_s, k_s, vt_s, o_s, ot_s, y_s, best_s, arg_s,
            s_s, m_s,
            x_sem, w_sem, o_sem):

    def x_copy(i):
        return pltpu.make_async_copy(x_hbm.at[0, _rows(i, TB)], x_s.at[_rows(i, TB)],
                                     x_sem.at[i])

    def out_copy(i):
        return pltpu.make_async_copy(x_s.at[_rows(i, TB)], out_hbm.at[0, _rows(i, TB)],
                                     o_sem.at[i])

    def wqkv_copy(j):
        return pltpu.make_async_copy(
            wqkv_hbm.at[:, pl.ds(j * NC, NC)], wqkv.at[j], w_sem.at[j])

    wo_copy = pltpu.make_async_copy(wo_hbm, wo, w_sem.at[NNC])

    def ffn_copies():
        cs = []
        for j in range(F // 128):
            cs.append(pltpu.make_async_copy(
                wg_hbm.at[:, pl.ds(j * 128, 128)], wg.at[j], w_sem.at[NNC + 1]))
            cs.append(pltpu.make_async_copy(
                wu_hbm.at[:, pl.ds(j * 128, 128)], wu.at[j], w_sem.at[NNC + 1]))
        for j in range(D // 128):
            cs.append(pltpu.make_async_copy(
                wd_hbm.at[:, pl.ds(j * 128, 128)], wd.at[j], w_sem.at[NNC + 1]))
        return cs

    def ln_rows(i, r0, n):
        x = x_s[pl.ds(pl.multiple_of(i * TB + r0, n), n), :].astype(F32)
        xn[0, r0 // 2:(r0 + n) // 2, :] = _pack(_layernorm(x))

    def lane_group(n):
        return lax.broadcasted_iota(I32, (n, 128), 1) // DH

    def store_q(i, g, q):
        grp = lane_group(SUB // 2)
        rolled = [q] + [pltpu.roll(q, DH * t, 1) for t in range(1, 4)]
        for h in range(4):
            parts = []
            for c in range(TB // SUB):
                b = c % 4
                rows = slice(c * SUB // 2, (c + 1) * SUB // 2)
                parts.append(jnp.where(grp == b, rolled[(b - h) % 4][rows], 0))
            q_s[g * 4 + h, _rows(i, TB // 2), :] = jnp.concatenate(parts, axis=0)

    def store_k(i, g, k):
        grp = lane_group(TB // 2)
        even = grp % 2 == 0
        low = grp < 2
        pairs = [jnp.where(even, k, pltpu.roll(k, DH, 1)),
                 jnp.where(even, pltpu.roll(k, 3 * DH, 1), k)]
        for h in range(2):
            swapped = pltpu.roll(pairs[h], 2 * DH, 1)
            k_s[g * 4 + h, _rows(i, TB // 2), :] = jnp.where(low, pairs[h], swapped)
            k_s[g * 4 + h + 2, _rows(i, TB // 2), :] = jnp.where(low, swapped, pairs[h])

    def qkv_block(i, nxt, startup):
        for jj, j in enumerate(CHUNKS):
            if startup:
                wqkv_copy(j).wait()
                if jj + 2 < NNC:
                    wqkv_copy(CHUNKS[jj + 2]).start()
                elif jj + 2 == NNC:
                    x_copy(1).start()
                else:
                    x_copy(1).wait()
                    for b in range(2, NTB):
                        x_copy(b).start()
                    wo_copy.start()
            y = jnp.dot(_unpack(xn[min(jj, 1)]), wqkv[j], preferred_element_type=F32)
            if jj == 0:
                xn[1] = xn[0]
            kind, c0 = divmod(j * NC, D)
            for c in range(NC // 128):
                g = c0 // 128 + c
                yc = y[:, c * 128:(c + 1) * 128]
                if kind == 0:
                    store_q(i, g, _pack(yc * QSCALE))
                elif kind == 1:
                    store_k(i, g, _pack(yc))
                else:
                    for t in range(TB // QB):
                        vt_s[i * (TB // QB) + t, g * 64:(g + 1) * 64, :] = _pack(
                            yc[t * QB:(t + 1) * QB, :].T)
            if startup:
                if jj == NNC - 1:
                    for c in range(8):
                        ln_rows(nxt, c * (TB // 8), TB // 8)
            elif 1 <= jj < 5:
                for c in range(2 * jj - 2, 2 * jj):
                    ln_rows(nxt, c * (TB // 8), TB // 8)

    def tri():
        kk = lax.broadcasted_iota(I32, (QB, QB), 0)
        qq = lax.broadcasted_iota(I32, (QB, QB), 1)
        return kk <= qq

    def scores(qb, g, nk, slot):
        kk = lax.broadcasted_iota(I32, (QB, QB), 0)
        qq = lax.broadcasted_iota(I32, (QB, QB), 1)
        grp = lane_group(SUB // 2)
        n = SUB // 2
        for h in range(4):
            hd = g * 4 + h
            tiles = [k_s[hd, _rows(qb - b, QB // 2), :] for b in range(nk)]
            if nk == 3:
                new, mid, old = tiles
                diag = jnp.where(grp >= 2,
                                 jnp.where(grp >= 3, old[3 * n:], old[2 * n:3 * n]),
                                 jnp.where(grp >= 1, old[n:2 * n], old[:n]))
                lhs = [diag, new[:n]] + [
                    jnp.where(grp >= c, new[c * n:(c + 1) * n], old[c * n:(c + 1) * n])
                    for c in range(1, 4)] + [mid]
            else:
                lhs = tiles
            st = lax.dot_general(_unpack(jnp.concatenate(lhs, axis=0)),
                                 _unpack(q_s[hd, _rows(qb, QB // 2), :]), NT,
                                 preferred_element_type=F32)
            if nk == 3:
                t = jnp.where((kk > qq) & (kk // SUB == qq // SUB),
                              jnp.concatenate([st[:SUB]] * 4, axis=0), st[SUB:SUB + QB])
                st = st[SUB:]
            else:
                t = jnp.where(kk <= qq, st[:QB], -1e30)
            s_s[slot, h, 0:QB, :] = t
            if nk >= 2:
                s_s[slot, h, QB:2 * QB, :] = st[QB:]
                t = jnp.maximum(t, st[QB:])
            m_s[slot, h] = jnp.max(t.reshape(QB // 8, 8, QB), axis=0)

    def softmax_pv(qb, g, nk, slot, odd):
        newest = tri()
        outs = []
        for h in range(4):
            m = jnp.max(m_s[slot, h], axis=0, keepdims=True)
            p0 = jnp.exp2(s_s[slot, h, 0:QB, :] - m)
            l = p0
            if nk == 3:
                pt = [jnp.where(newest, p0, 0.0), jnp.where(newest, 0.0, p0)]
                backs = [0, 2, 1]
            else:
                pt = [p0]
                backs = [0, 1][:nk]
            if nk >= 2:
                p1 = jnp.exp2(s_s[slot, h, QB:2 * QB, :] - m)
                l = l + p1
                pt.append(p1)
            l = jnp.sum(l, axis=0, keepdims=True)
            r0 = (g * 4 + h) * (DH // 2)
            vt = jnp.concatenate([vt_s[qb - b, r0:r0 + DH // 2, :] for b in backs], axis=1)
            ot = jnp.dot(_unpack(vt), jnp.concatenate(pt, axis=0).astype(BF),
                         preferred_element_type=F32)
            outs.append(ot * (1.0 / l))
        ot = jnp.concatenate(outs, axis=0)
        if odd and g + 1 == NG:
            ot_s[...] = ot
        else:
            o_s[_rows(odd, QB // 2), g * 128:(g + 1) * 128] = _pack(ot.T)

    def out_proj():
        o_s[QB // 2:, D - 128:] = _pack(ot_s[...].T)
        y_s[1] = jnp.dot(_unpack(o_s[...]), wo[...], preferred_element_type=F32)

    def router(i, slot):
        wr = wr_ref[...].astype(F32).reshape(1, D)
        tok = lax.broadcasted_iota(I32, (8, 128), 0) + i * TB
        best, arg = best_s[...], arg_s[...]
        for c in range(TB // RC):
            rows = _rows(i * (TB // RC) + c, RC)
            x1 = x_s[rows, :].astype(F32) + y_s[slot, c * RC:(c + 1) * RC, :]
            xn1 = _layernorm(x1)
            n_s[rows, :] = xn1
            r = jnp.broadcast_to(jnp.sum(xn1 * wr, axis=-1, keepdims=True), (RC, 128))
            x_s[rows, :] = (x1 + xn1).astype(BF)
            for t in range(RC // 8):
                rt = r[t * 8:(t + 1) * 8]
                arg = jnp.where(rt > best, tok + (c * RC + t * 8), arg)
                best = jnp.where(rt > best, rt, best)
        best_s[...] = jnp.where(i < NTB, best, -jnp.inf)
        arg_s[...] = arg

    def attn_pair(i, nks, nxt):
        for odd in range(2):
            qb = 2 * i + odd
            for g in range(NG):
                if g + 1 < NG:
                    scores(qb, g + 1, nks[odd], (g + 1) % 2)
                elif odd:
                    scores(nxt, 0, 3, 0)
                else:
                    scores(qb + 1, 0, nks[1], 0)
                if nks[0] == 3 and g == 0:
                    if odd:
                        y_s[0] = y_s[1]
                    else:
                        router(jnp.where(i >= 2, i - 2, NTB), 0)
                        out_proj()
                softmax_pv(qb, g, nks[odd], g % 2, odd)

    def ffn(first, last):
        best = best_s[...]
        rmax = jnp.max(best, axis=0, keepdims=True)
        idx = jnp.min(jnp.where(best == rmax, arg_s[...], S - 1))
        idx = jnp.clip(idx, 0, S - 1)

        @pl.when(first)
        def _():
            for c in ffn_copies():
                c.wait()

        xs = jnp.broadcast_to(n_s[pl.ds(idx, 1), :], (16, D)).astype(BF)
        hs = []
        for j in range(F // 128):
            gj = jnp.dot(xs, wg[j], preferred_element_type=F32)
            uj = jnp.dot(xs, wu[j], preferred_element_type=F32)
            hs.append((gj * jax.nn.sigmoid(gj) * uj).astype(BF))
        hid = jnp.concatenate(hs, axis=1)
        y = jnp.concatenate(
            [jnp.dot(hid, wd[j], preferred_element_type=F32) for j in range(D // 128)], axis=1)
        y = y * jax.nn.sigmoid(rmax[:, 0:1])

        @pl.when(last)
        def _():
            for i in range(NTB):
                out_copy(i).wait()

        rows = _rows(idx // 16, 16)
        x = x_s[rows, :].astype(F32)
        sel = lax.broadcasted_iota(I32, (16, D), 0) == idx % 16
        x_s[rows, :] = jnp.where(sel, x + y, x).astype(BF)

        @pl.when(last)
        def _():
            fix = pltpu.make_async_copy(x_s.at[rows], out_hbm.at[0, rows], o_sem.at[0])
            fix.start()
            fix.wait()

    x_copy(0).start()
    wqkv_copy(CHUNKS[0]).start()
    wqkv_copy(CHUNKS[1]).start()
    x_s[_rows(NTB, TB), :] = jnp.zeros((TB, D), BF)
    y_s[0] = jnp.zeros((TB, D), F32)
    best_s[...] = jnp.zeros((8, 128), F32)
    arg_s[...] = jnp.zeros((8, 128), I32)
    x_copy(0).wait()
    ln_rows(0, 0, TB)
    qkv_block(0, 1, True)

    def layer(l, carry):
        first = l == 0
        last = l == 1

        @pl.when(last)
        def _():
            ln_rows(0, 0, TB)

        def qkv_body(i, c):
            @pl.when(first & (i + 1 < NTB))
            def _():
                x_copy(i + 1).wait()
            qkv_block(i, (i + 1) % NTB, False)
            return c
        lax.fori_loop(1 - l, NTB, qkv_body, 0)

        @pl.when(first)
        def _():
            for c in ffn_copies():
                c.start()
            wo_copy.wait()

        scores(0, 0, 1, 0)
        attn_pair(0, (1, 2), 2)

        def attn_body(i, c):
            @pl.when(last & (i > 2))
            def _():
                out_copy(i - 3).start()
            attn_pair(i, (3, 3), jnp.minimum(2 * i + 2, NQB - 1))
            return c
        lax.fori_loop(1, NTB, attn_body, 0)

        router(NTB - 2, 0)
        out_proj()
        router(NTB - 1, 1)

        @pl.when(last)
        def _():
            for i in range(NTB - 3, NTB):
                out_copy(i).start()

        ffn(first, last)
        return carry

    lax.fori_loop(0, 2, layer, 0)


@jax.jit
def pallas_interleave_layers__sliding_block__moe_arch_mod__prompt_kernel(
    A_x: jax.Array,
    A_wqkv: jax.Array,
    A_wo: jax.Array,
    B_x: jax.Array,
    B_w_r: jax.Array,
    B_w_gate: jax.Array,
    B_w_up: jax.Array,
    B_w_down: jax.Array,
):
    del B_x
    hbm = pl.BlockSpec(memory_space=pl.ANY)
    return pl.pallas_call(
        _kernel,
        in_specs=[hbm, hbm, hbm, pl.BlockSpec(memory_space=pltpu.VMEM), hbm, hbm, hbm],
        out_specs=hbm,
        out_shape=jax.ShapeDtypeStruct((1, S, D), BF),
        scratch_shapes=[
            pltpu.VMEM((S + TB, D), BF),
            pltpu.VMEM((S + TB, D), F32),
            pltpu.VMEM((2, TB // 2, D), I32),
            pltpu.VMEM((NNC, D, NC), BF),
            pltpu.VMEM((D, D), BF),
            pltpu.VMEM((F // 128, D, 128), BF),
            pltpu.VMEM((F // 128, D, 128), BF),
            pltpu.VMEM((D // 128, F, 128), BF),
            pltpu.VMEM((4 * NG, S // 2, 128), I32),
            pltpu.VMEM((4 * NG, S // 2, 128), I32),
            pltpu.VMEM((NQB, D // 2, QB), I32),
            pltpu.VMEM((TB // 2, D), I32),
            pltpu.VMEM((128, QB), F32),
            pltpu.VMEM((2, TB, D), F32),
            pltpu.VMEM((8, 128), F32),
            pltpu.VMEM((8, 128), I32),
            pltpu.VMEM((2, 4, 2 * QB, QB), F32),
            pltpu.VMEM((2, 4, 8, QB), F32),
            pltpu.SemaphoreType.DMA((NTB,)),
            pltpu.SemaphoreType.DMA((NNC + 2,)),
            pltpu.SemaphoreType.DMA((NTB,)),
        ],
        compiler_params=pltpu.CompilerParams(vmem_limit_bytes=100 * 1024 * 1024),
        name="mod_swa",
    )(A_x, A_wqkv, A_wo, B_w_r, B_w_gate, B_w_up, B_w_down)
```

```python
import math

import jax
import jax.numpy as jnp
from jax import lax
import jax.experimental.pallas as pl
import jax.experimental.pallas.tpu as pltpu

S = 2048
D = 1024
DH = 32
F = 3584
TB = 256
NTB = S // TB
QB = 128
NQB = S // QB
NG = D // 128
NC = 512
NNC = 3 * D // NC
CHUNKS = [4, 5, 2, 3, 0, 1]
RC = 32
SUB = 32
EPS = 1e-5
QSCALE = (DH ** -0.5) * math.log2(math.e)

BF = jnp.bfloat16
F32 = jnp.float32
I32 = jnp.int32
NT = (((1,), (1,)), ((), ()))


def _pack(v):
    return pltpu.bitcast(v.astype(BF), I32)


def _unpack(v):
    return pltpu.bitcast(v, BF)


def _layernorm(x):
    m = jnp.sum(x, axis=-1, keepdims=True) * (1.0 / D)
    xc = x - m
    v = jnp.sum(xc * xc, axis=-1, keepdims=True) * (1.0 / D)
    return xc * lax.rsqrt(v + EPS)


def _rows(i, n):
    return pl.ds(i * n if isinstance(i, int) else pl.multiple_of(i * n, n), n)


def _kernel(x_hbm, wqkv_hbm, wo_hbm, wr_ref, wg_hbm, wu_hbm, wd_hbm, out_hbm,
            x_s, n_s, xn, wqkv, wo, wg, wu, wd, q_s, k_s, vt_s, o_s, ot_s, y_s, best_s, arg_s,
            s_s, m_s,
            x_sem, w_sem, o_sem):

    def x_copy(i):
        return pltpu.make_async_copy(x_hbm.at[0, _rows(i, TB)], x_s.at[_rows(i, TB)],
                                     x_sem.at[i])

    def out_copy(i):
        return pltpu.make_async_copy(x_s.at[_rows(i, TB)], out_hbm.at[0, _rows(i, TB)],
                                     o_sem.at[i])

    def wqkv_copy(j):
        return pltpu.make_async_copy(
            wqkv_hbm.at[:, pl.ds(j * NC, NC)], wqkv.at[j], w_sem.at[j])

    wo_copy = pltpu.make_async_copy(wo_hbm, wo, w_sem.at[NNC])

    def ffn_copies():
        cs = []
        for j in range(F // 128):
            cs.append(pltpu.make_async_copy(
                wg_hbm.at[:, pl.ds(j * 128, 128)], wg.at[j], w_sem.at[NNC + 1]))
            cs.append(pltpu.make_async_copy(
                wu_hbm.at[:, pl.ds(j * 128, 128)], wu.at[j], w_sem.at[NNC + 1]))
        for j in range(D // 128):
            cs.append(pltpu.make_async_copy(
                wd_hbm.at[:, pl.ds(j * 128, 128)], wd.at[j], w_sem.at[NNC + 1]))
        return cs

    def ln_rows(i, r0, n):
        x = x_s[pl.ds(pl.multiple_of(i * TB + r0, n), n), :].astype(F32)
        xn[0, r0 // 2:(r0 + n) // 2, :] = _pack(_layernorm(x))

    def lane_group(n):
        return lax.broadcasted_iota(I32, (n, 128), 1) // DH

    def store_q(i, g, q):
        grp = lane_group(SUB // 2)
        rolled = [q] + [pltpu.roll(q, DH * t, 1) for t in range(1, 4)]
        for h in range(4):
            parts = []
            for c in range(TB // SUB):
                b = c % 4
                rows = slice(c * SUB // 2, (c + 1) * SUB // 2)
                parts.append(jnp.where(grp == b, rolled[(b - h) % 4][rows], 0))
            q_s[g * 4 + h, _rows(i, TB // 2), :] = jnp.concatenate(parts, axis=0)

    def store_k(i, g, k):
        grp = lane_group(TB // 2)
        even = grp % 2 == 0
        low = grp < 2
        pairs = [jnp.where(even, k, pltpu.roll(k, DH, 1)),
                 jnp.where(even, pltpu.roll(k, 3 * DH, 1), k)]
        for h in range(2):
            swapped = pltpu.roll(pairs[h], 2 * DH, 1)
            k_s[g * 4 + h, _rows(i, TB // 2), :] = jnp.where(low, pairs[h], swapped)
            k_s[g * 4 + h + 2, _rows(i, TB // 2), :] = jnp.where(low, swapped, pairs[h])

    def qkv_block(i, nxt, startup):
        for jj, j in enumerate(CHUNKS):
            if startup:
                wqkv_copy(j).wait()
                if jj + 2 < NNC:
                    wqkv_copy(CHUNKS[jj + 2]).start()
                elif jj + 2 == NNC:
                    x_copy(1).start()
                else:
                    x_copy(1).wait()
                    for b in range(2, NTB):
                        x_copy(b).start()
                    wo_copy.start()
            y = jnp.dot(_unpack(xn[min(jj, 1)]), wqkv[j], preferred_element_type=F32)
            if jj == 0:
                xn[1] = xn[0]
            kind, c0 = divmod(j * NC, D)
            for c in range(NC // 128):
                g = c0 // 128 + c
                yc = y[:, c * 128:(c + 1) * 128]
                if kind == 0:
                    store_q(i, g, _pack(yc * QSCALE))
                elif kind == 1:
                    store_k(i, g, _pack(yc))
                else:
                    for t in range(TB // QB):
                        vt_s[i * (TB // QB) + t, g * 64:(g + 1) * 64, :] = _pack(
                            yc[t * QB:(t + 1) * QB, :].T)
            if startup:
                if jj == NNC - 1:
                    for c in range(8):
                        ln_rows(nxt, c * (TB // 8), TB // 8)
            elif 1 <= jj < 5:
                for c in range(2 * jj - 2, 2 * jj):
                    ln_rows(nxt, c * (TB // 8), TB // 8)

    def tri():
        kk = lax.broadcasted_iota(I32, (QB, QB), 0)
        qq = lax.broadcasted_iota(I32, (QB, QB), 1)
        return kk <= qq

    def scores(qb, g, nk, slot):
        kk = lax.broadcasted_iota(I32, (QB, QB), 0)
        qq = lax.broadcasted_iota(I32, (QB, QB), 1)
        grp = lane_group(SUB // 2)
        n = SUB // 2
        for h in range(4):
            hd = g * 4 + h
            tiles = [k_s[hd, _rows(qb - b, QB // 2), :] for b in range(nk)]
            if nk == 3:
                new, mid, old = tiles
                diag = jnp.where(grp >= 2,
                                 jnp.where(grp >= 3, old[3 * n:], old[2 * n:3 * n]),
                                 jnp.where(grp >= 1, old[n:2 * n], old[:n]))
                lhs = [diag, new[:n]] + [
                    jnp.where(grp >= c, new[c * n:(c + 1) * n], old[c * n:(c + 1) * n])
                    for c in range(1, 4)] + [mid]
            else:
                lhs = tiles
            st = lax.dot_general(_unpack(jnp.concatenate(lhs, axis=0)),
                                 _unpack(q_s[hd, _rows(qb, QB // 2), :]), NT,
                                 preferred_element_type=F32)
            if nk == 3:
                t = jnp.where((kk > qq) & (kk // SUB == qq // SUB),
                              jnp.concatenate([st[:SUB]] * 4, axis=0), st[SUB:SUB + QB])
                st = st[SUB:]
            else:
                t = jnp.where(kk <= qq, st[:QB], -1e30)
            s_s[slot, h, 0:QB, :] = t
            if nk >= 2:
                s_s[slot, h, QB:2 * QB, :] = st[QB:]
                t = jnp.maximum(t, st[QB:])
            m_s[slot, h] = jnp.max(t.reshape(QB // 8, 8, QB), axis=0)

    def softmax_pv(qb, g, nk, slot, odd):
        newest = tri()
        outs = []
        for h in range(4):
            m = jnp.max(m_s[slot, h], axis=0, keepdims=True)
            p0 = jnp.exp2(s_s[slot, h, 0:QB, :] - m)
            l = p0
            if nk == 3:
                pt = [jnp.where(newest, p0, 0.0), jnp.where(newest, 0.0, p0)]
                backs = [0, 2, 1]
            else:
                pt = [p0]
                backs = [0, 1][:nk]
            if nk >= 2:
                p1 = jnp.exp2(s_s[slot, h, QB:2 * QB, :] - m)
                l = l + p1
                pt.append(p1)
            l = jnp.sum(l, axis=0, keepdims=True)
            r0 = (g * 4 + h) * (DH // 2)
            vt = jnp.concatenate([vt_s[qb - b, r0:r0 + DH // 2, :] for b in backs], axis=1)
            ot = jnp.dot(_unpack(vt), jnp.concatenate(pt, axis=0).astype(BF),
                         preferred_element_type=F32)
            outs.append(ot * (1.0 / l))
        ot = jnp.concatenate(outs, axis=0)
        if odd and g + 1 == NG:
            ot_s[...] = ot
        else:
            o_s[_rows(odd, QB // 2), g * 128:(g + 1) * 128] = _pack(ot.T)

    def router(i, slot, c):
        wr = wr_ref[...].astype(F32).reshape(1, D)
        tok = lax.broadcasted_iota(I32, (8, 128), 0) + i * TB
        best, arg = best_s[...], arg_s[...]
        rows = _rows(i * (TB // RC) + c, RC)
        x1 = x_s[rows, :].astype(F32) + y_s[slot, c * RC:(c + 1) * RC, :]
        xn1 = _layernorm(x1)
        n_s[rows, :] = xn1
        r = jnp.broadcast_to(jnp.sum(xn1 * wr, axis=-1, keepdims=True), (RC, 128))
        x_s[rows, :] = (x1 + xn1).astype(BF)
        for t in range(RC // 8):
            rt = r[t * 8:(t + 1) * 8]
            arg = jnp.where(rt > best, tok + (c * RC + t * 8), arg)
            best = jnp.where(rt > best, rt, best)
        best_s[...] = jnp.where(i < NTB, best, -jnp.inf)
        arg_s[...] = arg

    def out_proj(slot, prev):
        o_s[QB // 2:, D - 128:] = _pack(ot_s[...].T)
        for j in range(D // 128):
            for c in range(j * TB // RC // 8, (j + 1) * TB // RC // 8):
                router(prev, 1 - slot, c)
            cols = slice(j * 128, (j + 1) * 128)
            y_s[slot, :, cols] = jnp.dot(_unpack(o_s[...]), wo[:, cols],
                                         preferred_element_type=F32)

    def attn_pair(i, nks, nxt):
        for odd in range(2):
            qb = 2 * i + odd
            for g in range(NG):
                if g + 1 < NG:
                    scores(qb, g + 1, nks[odd], (g + 1) % 2)
                elif odd:
                    scores(nxt, 0, 3, 0)
                else:
                    scores(qb + 1, 0, nks[1], 0)
                if nks[0] == 3 and g == 0 and not odd:
                    out_proj(i % 2, jnp.where(i >= 2, i - 2, NTB))
                softmax_pv(qb, g, nks[odd], g % 2, odd)

    def ffn(first, last):
        best = best_s[...]
        rmax = jnp.max(best, axis=0, keepdims=True)
        idx = jnp.min(jnp.where(best == rmax, arg_s[...], S - 1))
        idx = jnp.clip(idx, 0, S - 1)

        @pl.when(first)
        def _():
            for c in ffn_copies():
                c.wait()

        xs = jnp.broadcast_to(n_s[pl.ds(idx, 1), :], (16, D)).astype(BF)
        hs = []
        for j in range(F // 128):
            gj = jnp.dot(xs, wg[j], preferred_element_type=F32)
            uj = jnp.dot(xs, wu[j], preferred_element_type=F32)
            hs.append((gj * jax.nn.sigmoid(gj) * uj).astype(BF))
        hid = jnp.concatenate(hs, axis=1)
        y = jnp.concatenate(
            [jnp.dot(hid, wd[j], preferred_element_type=F32) for j in range(D // 128)], axis=1)
        y = y * jax.nn.sigmoid(rmax[:, 0:1])

        @pl.when(last)
        def _():
            for i in range(NTB):
                out_copy(i).wait()

        rows = _rows(idx // 16, 16)
        x = x_s[rows, :].astype(F32)
        sel = lax.broadcasted_iota(I32, (16, D), 0) == idx % 16
        x_s[rows, :] = jnp.where(sel, x + y, x).astype(BF)

        @pl.when(last)
        def _():
            fix = pltpu.make_async_copy(x_s.at[rows], out_hbm.at[0, rows], o_sem.at[0])
            fix.start()
            fix.wait()

    x_copy(0).start()
    wqkv_copy(CHUNKS[0]).start()
    wqkv_copy(CHUNKS[1]).start()
    x_s[_rows(NTB, TB), :] = jnp.zeros((TB, D), BF)
    y_s[0] = jnp.zeros((TB, D), F32)
    best_s[...] = jnp.zeros((8, 128), F32)
    arg_s[...] = jnp.zeros((8, 128), I32)
    x_copy(0).wait()
    ln_rows(0, 0, TB)
    qkv_block(0, 1, True)

    def layer(l, carry):
        first = l == 0
        last = l == 1

        @pl.when(last)
        def _():
            ln_rows(0, 0, TB)

        def qkv_body(i, c):
            @pl.when(first & (i + 1 < NTB))
            def _():
                x_copy(i + 1).wait()
            qkv_block(i, (i + 1) % NTB, False)
            return c
        lax.fori_loop(1 - l, NTB, qkv_body, 0)

        @pl.when(first)
        def _():
            for c in ffn_copies():
                c.start()
            wo_copy.wait()

        scores(0, 0, 1, 0)
        attn_pair(0, (1, 2), 2)

        def attn_body(i, c):
            @pl.when(last & (i > 2))
            def _():
                out_copy(i - 3).start()
            attn_pair(i, (3, 3), jnp.minimum(2 * i + 2, NQB - 1))
            return c
        lax.fori_loop(1, NTB, attn_body, 0)

        out_proj(l // 2, NTB - 2)
        for c in range(TB // RC):
            router(NTB - 1, 0, c)

        @pl.when(last)
        def _():
            for i in range(NTB - 3, NTB):
                out_copy(i).start()

        ffn(first, last)
        return carry

    lax.fori_loop(0, 2, layer, 0)


@jax.jit
def pallas_interleave_layers__sliding_block__moe_arch_mod__prompt_kernel(
    A_x: jax.Array,
    A_wqkv: jax.Array,
    A_wo: jax.Array,
    B_x: jax.Array,
    B_w_r: jax.Array,
    B_w_gate: jax.Array,
    B_w_up: jax.Array,
    B_w_down: jax.Array,
):
    del B_x
    hbm = pl.BlockSpec(memory_space=pl.ANY)
    return pl.pallas_call(
        _kernel,
        in_specs=[hbm, hbm, hbm, pl.BlockSpec(memory_space=pltpu.VMEM), hbm, hbm, hbm],
        out_specs=hbm,
        out_shape=jax.ShapeDtypeStruct((1, S, D), BF),
        scratch_shapes=[
            pltpu.VMEM((S + TB, D), BF),
            pltpu.VMEM((S + TB, D), F32),
            pltpu.VMEM((2, TB // 2, D), I32),
            pltpu.VMEM((NNC, D, NC), BF),
            pltpu.VMEM((D, D), BF),
            pltpu.VMEM((F // 128, D, 128), BF),
            pltpu.VMEM((F // 128, D, 128), BF),
            pltpu.VMEM((D // 128, F, 128), BF),
            pltpu.VMEM((4 * NG, S // 2, 128), I32),
            pltpu.VMEM((4 * NG, S // 2, 128), I32),
            pltpu.VMEM((NQB, D // 2, QB), I32),
            pltpu.VMEM((TB // 2, D), I32),
            pltpu.VMEM((128, QB), F32),
            pltpu.VMEM((2, TB, D), F32),
            pltpu.VMEM((8, 128), F32),
            pltpu.VMEM((8, 128), I32),
            pltpu.VMEM((2, 4, 2 * QB, QB), F32),
            pltpu.VMEM((2, 4, 8, QB), F32),
            pltpu.SemaphoreType.DMA((NTB,)),
            pltpu.SemaphoreType.DMA((NNC + 2,)),
            pltpu.SemaphoreType.DMA((NTB,)),
        ],
        compiler_params=pltpu.CompilerParams(vmem_limit_bytes=100 * 1024 * 1024),
        name="mod_swa",
    )(A_x, A_wqkv, A_wo, B_w_r, B_w_gate, B_w_up, B_w_down)
```

```python
import math

import jax
import jax.numpy as jnp
from jax import lax
import jax.experimental.pallas as pl
import jax.experimental.pallas.tpu as pltpu

S = 2048
D = 1024
DH = 32
F = 3584
TB = 256
NTB = S // TB
QB = 128
NQB = S // QB
NG = D // 128
NC = 512
NNC = 3 * D // NC
CHUNKS = [4, 5, 2, 3, 0, 1]
RC = 32
SUB = 32
EPS = 1e-5
QSCALE = (DH ** -0.5) * math.log2(math.e)

BF = jnp.bfloat16
F32 = jnp.float32
I32 = jnp.int32
NT = (((1,), (1,)), ((), ()))


def _pack(v):
    return pltpu.bitcast(v.astype(BF), I32)


def _unpack(v):
    return pltpu.bitcast(v, BF)


def _layernorm(x):
    m = jnp.sum(x, axis=-1, keepdims=True) * (1.0 / D)
    xc = x - m
    v = jnp.sum(xc * xc, axis=-1, keepdims=True) * (1.0 / D)
    return xc * lax.rsqrt(v + EPS)


def _rows(i, n):
    return pl.ds(i * n if isinstance(i, int) else pl.multiple_of(i * n, n), n)


def _kernel(x_hbm, wqkv_hbm, wo_hbm, wr_ref, wg_hbm, wu_hbm, wd_hbm, out_hbm,
            x_s, n_s, xn, wqkv, wo, wg, wu, wd, q_s, q7_s, k_s, vt_s, o_s, ot_s, y_s, best_s, arg_s,
            s_s, m_s,
            x_sem, w_sem, o_sem):

    def x_copy(i):
        return pltpu.make_async_copy(x_hbm.at[0, _rows(i, TB)], x_s.at[_rows(i, TB)],
                                     x_sem.at[i])

    def out_copy(i):
        return pltpu.make_async_copy(x_s.at[_rows(i, TB)], out_hbm.at[0, _rows(i, TB)],
                                     o_sem.at[i])

    def wqkv_copy(j, half):
        rows = pl.ds(half * D // 2, D // 2)
        return pltpu.make_async_copy(
            wqkv_hbm.at[rows, pl.ds(j * NC, NC)], wqkv.at[j, rows], w_sem.at[j])

    wo_copy = pltpu.make_async_copy(wo_hbm, wo, w_sem.at[NNC])

    def ffn_copies():
        cs = []
        for j in range(F // 128):
            cs.append(pltpu.make_async_copy(
                wg_hbm.at[:, pl.ds(j * 128, 128)], wg.at[j], w_sem.at[NNC + 1]))
            cs.append(pltpu.make_async_copy(
                wu_hbm.at[:, pl.ds(j * 128, 128)], wu.at[j], w_sem.at[NNC + 1]))
        for j in range(D // 128):
            cs.append(pltpu.make_async_copy(
                wd_hbm.at[:, pl.ds(j * 128, 128)], wd.at[j], w_sem.at[NNC + 1]))
        return cs

    def ln_rows(i, r0, n):
        x = x_s[pl.ds(pl.multiple_of(i * TB + r0, n), n), :].astype(F32)
        xn[0, r0 // 2:(r0 + n) // 2, :] = _pack(_layernorm(x))

    def lane_group(n):
        return lax.broadcasted_iota(I32, (n, 128), 1) // DH

    def store_q(i, g, q):
        grp = lane_group(SUB // 2)
        rolled = [q] + [pltpu.roll(q, DH * t, 1) for t in range(1, 4)]
        for h in range(4):
            parts = []
            for c in range(TB // SUB):
                b = c % 4
                rows = slice(c * SUB // 2, (c + 1) * SUB // 2)
                parts.append(jnp.where(grp == b, rolled[(b - h) % 4][rows], 0))
            q_s[g * 4 + h, _rows(i, TB // 2), :] = jnp.concatenate(parts, axis=0)

    def store_k(i, g, k):
        grp = lane_group(TB // 2)
        even = grp % 2 == 0
        low = grp < 2
        pairs = [jnp.where(even, k, pltpu.roll(k, DH, 1)),
                 jnp.where(even, pltpu.roll(k, 3 * DH, 1), k)]
        for h in range(2):
            swapped = pltpu.roll(pairs[h], 2 * DH, 1)
            k_s[g * 4 + h, _rows(i, TB // 2), :] = jnp.where(low, pairs[h], swapped)
            k_s[g * 4 + h + 2, _rows(i, TB // 2), :] = jnp.where(low, swapped, pairs[h])

    def qkv_block(i, nxt, startup):
        if not startup:
            store_q((i + NTB - 1) % NTB, NG - 1, q7_s[...])
        for jj, j in enumerate(CHUNKS):
            if startup:
                wqkv_copy(j, 0).wait()
                wqkv_copy(j, 1).wait()
                if jj + 1 < NNC:
                    wqkv_copy(CHUNKS[jj + 1], 1).start()
                if jj + 2 < NNC:
                    wqkv_copy(CHUNKS[jj + 2], 0).start()
                elif jj + 2 == NNC:
                    x_copy(1).start()
                else:
                    x_copy(1).wait()
                    for b in range(2, NTB):
                        x_copy(b).start()
                    wo_copy.start()
            y = jnp.dot(_unpack(xn[min(jj, 1)]), wqkv[j], preferred_element_type=F32)
            if jj == 0:
                xn[1] = xn[0]
            kind, c0 = divmod(j * NC, D)
            for c in range(NC // 128):
                g = c0 // 128 + c
                yc = y[:, c * 128:(c + 1) * 128]
                if kind == 0 and g == NG - 1:
                    q7_s[...] = _pack(yc * QSCALE)
                elif kind == 0:
                    store_q(i, g, _pack(yc * QSCALE))
                elif kind == 1:
                    store_k(i, g, _pack(yc))
                else:
                    for t in range(TB // QB):
                        vt_s[i * (TB // QB) + t, g * 64:(g + 1) * 64, :] = _pack(
                            yc[t * QB:(t + 1) * QB, :].T)
            if startup:
                if jj == NNC - 1:
                    for c in range(8):
                        ln_rows(nxt, c * (TB // 8), TB // 8)
            elif 1 <= jj < 5:
                for c in range(2 * jj - 2, 2 * jj):
                    ln_rows(nxt, c * (TB // 8), TB // 8)

    def tri():
        kk = lax.broadcasted_iota(I32, (QB, QB), 0)
        qq = lax.broadcasted_iota(I32, (QB, QB), 1)
        return kk <= qq

    def scores(qb, g, nk, slot):
        kk = lax.broadcasted_iota(I32, (QB, QB), 0)
        qq = lax.broadcasted_iota(I32, (QB, QB), 1)
        grp = lane_group(SUB // 2)
        n = SUB // 2
        for h in range(4):
            hd = g * 4 + h
            tiles = [k_s[hd, _rows(qb - b, QB // 2), :] for b in range(nk)]
            if nk == 3:
                new, mid, old = tiles
                diag = jnp.where(grp >= 2,
                                 jnp.where(grp >= 3, old[3 * n:], old[2 * n:3 * n]),
                                 jnp.where(grp >= 1, old[n:2 * n], old[:n]))
                lhs = [diag, new[:n]] + [
                    jnp.where(grp >= c, new[c * n:(c + 1) * n], old[c * n:(c + 1) * n])
                    for c in range(1, 4)] + [mid]
            else:
                lhs = tiles
            st = lax.dot_general(_unpack(jnp.concatenate(lhs, axis=0)),
                                 _unpack(q_s[hd, _rows(qb, QB // 2), :]), NT,
                                 preferred_element_type=F32)
            if nk == 3:
                t = jnp.where((kk > qq) & (kk // SUB == qq // SUB),
                              jnp.concatenate([st[:SUB]] * 4, axis=0), st[SUB:SUB + QB])
                st = st[SUB:]
            else:
                t = jnp.where(kk <= qq, st[:QB], -1e30)
            s_s[slot, h, 0:QB, :] = t
            if nk >= 2:
                s_s[slot, h, QB:2 * QB, :] = st[QB:]
                t = jnp.maximum(t, st[QB:])
            m_s[slot, h] = jnp.max(t.reshape(QB // 8, 8, QB), axis=0)

    def softmax_pv(qb, g, nk, slot, odd):
        newest = tri()
        outs = []
        for h in range(4):
            m = jnp.max(m_s[slot, h], axis=0, keepdims=True)
            p0 = jnp.exp2(s_s[slot, h, 0:QB, :] - m)
            p1 = jnp.exp2(s_s[slot, h, QB:2 * QB, :] - m) if nk >= 2 else None
            if nk == 3:
                pt = [jnp.where(newest, p0, 0.0), jnp.where(newest, 0.0, p0)]
                backs = [0, 2]
            else:
                pt, backs = [p0], [0]
            if nk >= 2:
                pt, backs = pt + [p1], backs + [1]
            l = sum(jnp.sum(p.reshape(16, 8, QB), axis=0) for p in (p0, p1) if p is not None)
            l = jnp.sum(l, axis=0, keepdims=True)
            r0 = (g * 4 + h) * (DH // 2)
            vt = jnp.concatenate([vt_s[qb - b, r0:r0 + DH // 2, :] for b in backs], axis=1)
            ot = jnp.dot(_unpack(vt), jnp.concatenate(pt, axis=0).astype(BF),
                         preferred_element_type=F32)
            outs.append(ot * (1.0 / l))
        ot = jnp.concatenate(outs, axis=0)
        if odd and g + 1 == NG:
            ot_s[...] = ot
        else:
            o_s[_rows(odd, QB // 2), g * 128:(g + 1) * 128] = _pack(ot.T)

    def router(i, slot, c):
        wr = wr_ref[...].astype(F32).reshape(1, D)
        tok = lax.broadcasted_iota(I32, (8, 128), 0) + i * TB
        best, arg = best_s[...], arg_s[...]
        rows = _rows(i * (TB // RC) + c, RC)
        x1 = x_s[rows, :].astype(F32) + y_s[slot, c * RC:(c + 1) * RC, :]
        xn1 = _layernorm(x1)
        n_s[rows, :] = xn1
        r = jnp.broadcast_to(jnp.sum(xn1 * wr, axis=-1, keepdims=True), (RC, 128))
        x_s[rows, :] = (x1 + xn1).astype(BF)
        for t in range(RC // 8):
            rt = r[t * 8:(t + 1) * 8]
            arg = jnp.where(rt > best, tok + (c * RC + t * 8), arg)
            best = jnp.where(rt > best, rt, best)
        best_s[...] = jnp.where(i < NTB, best, -jnp.inf)
        arg_s[...] = arg

    def out_proj(slot, prev):
        o_s[QB // 2:, D - 128:] = _pack(ot_s[...].T)
        for j in range(D // 128):
            for c in range(j * TB // RC // 8, (j + 1) * TB // RC // 8):
                router(prev, 1 - slot, c)
            cols = slice(j * 128, (j + 1) * 128)
            y_s[slot, :, cols] = jnp.dot(_unpack(o_s[...]), wo[:, cols],
                                         preferred_element_type=F32)

    def out_tail(slot):
        o_s[QB // 2:, D - 128:] = _pack(ot_s[...].T)
        todo = [(NTB - 2, 1 - slot, c) for c in range(TB // RC)]
        for r0, r1, every in ((0, 192, 1), (192, 256, 2)):
            for j in range(D // 128):
                if j % every == 0:
                    router(*todo.pop(0))
                cols = slice(j * 128, (j + 1) * 128)
                y_s[slot, r0:r1, cols] = jnp.dot(_unpack(o_s[r0 // 2:r1 // 2, :]), wo[:, cols],
                                                 preferred_element_type=F32)
            todo += [(NTB - 1, slot, c) for c in range(r0 // RC, r1 // RC)]
        for t in todo:
            router(*t)

    def attn_first():
        store_q(NTB - 1, NG - 1, q7_s[...])
        for g in range(-1, NG):
            if g + 1 < NG:
                scores(0, g + 1, 1, 2 + (g + 1) % 2)
                scores(1, g + 1, 2, (g + 1) % 2)
            else:
                scores(2, 0, 3, 0)
            if g >= 0:
                softmax_pv(0, g, 1, 2 + g % 2, 0)
                softmax_pv(1, g, 2, g % 2, 1)

    def attn_pair(i, nks, nxt):
        for odd in range(2):
            qb = 2 * i + odd
            for g in range(NG):
                if g + 1 < NG:
                    scores(qb, g + 1, nks[odd], (g + 1) % 2)
                elif odd:
                    scores(nxt, 0, 3, 0)
                else:
                    scores(qb + 1, 0, nks[1], 0)
                if nks[0] == 3 and g == 0 and not odd:
                    out_proj(i % 2, jnp.where(i >= 2, i - 2, NTB))
                softmax_pv(qb, g, nks[odd], g % 2, odd)

    def ffn(first, last):
        best = best_s[...]
        rmax = jnp.max(best, axis=0, keepdims=True)
        idx = jnp.min(jnp.where(best == rmax, arg_s[...], S - 1))
        idx = jnp.clip(idx, 0, S - 1)

        @pl.when(first)
        def _():
            for c in ffn_copies():
                c.wait()

        xs = jnp.broadcast_to(n_s[pl.ds(idx, 1), :], (16, D)).astype(BF)
        hs = []
        for j in range(F // 128):
            gj = jnp.dot(xs, wg[j], preferred_element_type=F32)
            uj = jnp.dot(xs, wu[j], preferred_element_type=F32)
            hs.append((gj * jax.nn.sigmoid(gj) * uj).astype(BF))
            if j < 16:
                ln_rows(0, j * 16, 16)
        hid = jnp.concatenate(hs, axis=1)
        y = jnp.concatenate(
            [jnp.dot(hid, wd[j], preferred_element_type=F32) for j in range(D // 128)], axis=1)
        y = y * jax.nn.sigmoid(rmax[:, 0:1])

        @pl.when(last)
        def _():
            for i in range(NTB):
                out_copy(i).wait()

        rows = _rows(idx // 16, 16)
        x = x_s[rows, :].astype(F32)
        sel = lax.broadcasted_iota(I32, (16, D), 0) == idx % 16
        x_s[rows, :] = jnp.where(sel, x + y, x).astype(BF)

        @pl.when(first & (idx < TB))
        def _():
            xn[0, _rows(idx // 16, 8), :] = _pack(_layernorm(x_s[rows, :].astype(F32)))

        @pl.when(last)
        def _():
            fix = pltpu.make_async_copy(x_s.at[rows], out_hbm.at[0, rows], o_sem.at[0])
            fix.start()
            fix.wait()

    x_copy(0).start()
    wqkv_copy(CHUNKS[0], 0).start()
    x_s[_rows(NTB, TB), :] = jnp.zeros((TB, D), BF)
    y_s[0] = jnp.zeros((TB, D), F32)
    best_s[...] = jnp.zeros((8, 128), F32)
    arg_s[...] = jnp.zeros((8, 128), I32)
    x_copy(0).wait()
    wqkv_copy(CHUNKS[0], 1).start()
    wqkv_copy(CHUNKS[1], 0).start()
    for c in range(8):
        ln_rows(0, c * (TB // 8), TB // 8)
    qkv_block(0, 1, True)

    def layer(l, carry):
        first = l == 0
        last = l == 1

        def qkv_body(i, c):
            @pl.when(first & (i + 1 < NTB))
            def _():
                x_copy(i + 1).wait()
            qkv_block(i, (i + 1) % NTB, False)
            return c
        lax.fori_loop(1 - l, NTB, qkv_body, 0)

        @pl.when(first)
        def _():
            for c in ffn_copies():
                c.start()
            wo_copy.wait()

        attn_first()

        def attn_body(i, c):
            @pl.when(last & (i > 2))
            def _():
                out_copy(i - 3).start()
            attn_pair(i, (3, 3), jnp.minimum(2 * i + 2, NQB - 1))
            return c
        lax.fori_loop(1, NTB, attn_body, 0)

        out_tail(l // 2)

        @pl.when(last)
        def _():
            for i in range(NTB - 3, NTB):
                out_copy(i).start()

        ffn(first, last)
        return carry

    lax.fori_loop(0, 2, layer, 0)


@jax.jit
def pallas_interleave_layers__sliding_block__moe_arch_mod__prompt_kernel(
    A_x: jax.Array,
    A_wqkv: jax.Array,
    A_wo: jax.Array,
    B_x: jax.Array,
    B_w_r: jax.Array,
    B_w_gate: jax.Array,
    B_w_up: jax.Array,
    B_w_down: jax.Array,
):
    del B_x
    hbm = pl.BlockSpec(memory_space=pl.ANY)
    return pl.pallas_call(
        _kernel,
        in_specs=[hbm, hbm, hbm, pl.BlockSpec(memory_space=pltpu.VMEM), hbm, hbm, hbm],
        out_specs=hbm,
        out_shape=jax.ShapeDtypeStruct((1, S, D), BF),
        scratch_shapes=[
            pltpu.VMEM((S + TB, D), BF),
            pltpu.VMEM((S + TB, D), F32),
            pltpu.VMEM((2, TB // 2, D), I32),
            pltpu.VMEM((NNC, D, NC), BF),
            pltpu.VMEM((D, D), BF),
            pltpu.VMEM((F // 128, D, 128), BF),
            pltpu.VMEM((F // 128, D, 128), BF),
            pltpu.VMEM((D // 128, F, 128), BF),
            pltpu.VMEM((4 * NG, S // 2, 128), I32),
            pltpu.VMEM((TB // 2, 128), I32),
            pltpu.VMEM((4 * NG, S // 2, 128), I32),
            pltpu.VMEM((NQB, D // 2, QB), I32),
            pltpu.VMEM((TB // 2, D), I32),
            pltpu.VMEM((128, QB), F32),
            pltpu.VMEM((2, TB, D), F32),
            pltpu.VMEM((8, 128), F32),
            pltpu.VMEM((8, 128), I32),
            pltpu.VMEM((4, 4, 2 * QB, QB), F32),
            pltpu.VMEM((4, 4, 8, QB), F32),
            pltpu.SemaphoreType.DMA((NTB,)),
            pltpu.SemaphoreType.DMA((NNC + 2,)),
            pltpu.SemaphoreType.DMA((NTB,)),
        ],
        compiler_params=pltpu.CompilerParams(vmem_limit_bytes=100 * 1024 * 1024),
        name="mod_swa",
    )(A_x, A_wqkv, A_wo, B_w_r, B_w_gate, B_w_up, B_w_down)
```

```python
import math

import jax
import jax.numpy as jnp
from jax import lax
import jax.experimental.pallas as pl
import jax.experimental.pallas.tpu as pltpu

S = 2048
D = 1024
DH = 32
F = 3584
TB = 256
NTB = S // TB
QB = 128
NQB = S // QB
NG = D // 128
NC = 256
NNC = 3 * D // NC
CHUNKS = [8, 9, 10, 11, 4, 5, 6, 7, 0, 1, 2, 3]
RC = 32
SUB = 32
EPS = 1e-5
QSCALE = (DH ** -0.5) * math.log2(math.e)

BF = jnp.bfloat16
F32 = jnp.float32
I32 = jnp.int32
NT = (((1,), (1,)), ((), ()))


def _pack(v):
    return pltpu.bitcast(v.astype(BF), I32)


def _unpack(v):
    return pltpu.bitcast(v, BF)


def _layernorm(x):
    m = jnp.sum(x, axis=-1, keepdims=True) * (1.0 / D)
    xc = x - m
    v = jnp.sum(xc * xc, axis=-1, keepdims=True) * (1.0 / D)
    return xc * lax.rsqrt(v + EPS)


def _rows(i, n):
    return pl.ds(i * n if isinstance(i, int) else pl.multiple_of(i * n, n), n)


def _kernel(x_hbm, wqkv_hbm, wo_hbm, wr_ref, wg_hbm, wu_hbm, wd_hbm, out_hbm,
            x_s, n_s, xn, wqkv, wo, wg, wu, wd, q_s, q7_s, k_s, vt_s, o_s, ot_s, y_s, best_s, arg_s,
            s_s, m_s,
            x_sem, w_sem, o_sem):

    def x_copy(i):
        return pltpu.make_async_copy(x_hbm.at[0, _rows(i, TB)], x_s.at[_rows(i, TB)],
                                     x_sem.at[i])

    def out_copy(i):
        return pltpu.make_async_copy(x_s.at[_rows(i, TB)], out_hbm.at[0, _rows(i, TB)],
                                     o_sem.at[i])

    def wqkv_copy(jj):
        j = CHUNKS[jj] // 2
        rows = pl.ds(jj % 2 * D // 2, D // 2)
        return pltpu.make_async_copy(
            wqkv_hbm.at[rows, pl.ds(j * 2 * NC, 2 * NC)], wqkv.at[j, rows], w_sem.at[j])

    wo_copy = pltpu.make_async_copy(wo_hbm, wo, w_sem.at[NNC // 2])

    def ffn_copies():
        cs = []
        for j in range(F // 128):
            cs.append(pltpu.make_async_copy(
                wg_hbm.at[:, pl.ds(j * 128, 128)], wg.at[j], w_sem.at[NNC // 2 + 1]))
            cs.append(pltpu.make_async_copy(
                wu_hbm.at[:, pl.ds(j * 128, 128)], wu.at[j], w_sem.at[NNC // 2 + 1]))
        for j in range(D // 128):
            cs.append(pltpu.make_async_copy(
                wd_hbm.at[:, pl.ds(j * 128, 128)], wd.at[j], w_sem.at[NNC // 2 + 1]))
        return cs

    def ln_rows(i, r0, n):
        x = x_s[pl.ds(pl.multiple_of(i * TB + r0, n), n), :].astype(F32)
        xn[0, r0 // 2:(r0 + n) // 2, :] = _pack(_layernorm(x))

    def lane_group(n):
        return lax.broadcasted_iota(I32, (n, 128), 1) // DH

    def store_q(i, g, q):
        grp = lane_group(SUB // 2)
        rolled = [q] + [pltpu.roll(q, DH * t, 1) for t in range(1, 4)]
        for h in range(4):
            parts = []
            for c in range(TB // SUB):
                b = c % 4
                rows = slice(c * SUB // 2, (c + 1) * SUB // 2)
                parts.append(jnp.where(grp == b, rolled[(b - h) % 4][rows], 0))
            q_s[g * 4 + h, _rows(i, TB // 2), :] = jnp.concatenate(parts, axis=0)

    def store_k(i, g, k):
        grp = lane_group(TB // 2)
        even = grp % 2 == 0
        low = grp < 2
        pairs = [jnp.where(even, k, pltpu.roll(k, DH, 1)),
                 jnp.where(even, pltpu.roll(k, 3 * DH, 1), k)]
        for h in range(2):
            swapped = pltpu.roll(pairs[h], 2 * DH, 1)
            k_s[g * 4 + h, _rows(i, TB // 2), :] = jnp.where(low, pairs[h], swapped)
            k_s[g * 4 + h + 2, _rows(i, TB // 2), :] = jnp.where(low, swapped, pairs[h])

    def qkv_block(i, nxt, startup):
        if not startup:
            store_q((i + NTB - 1) % NTB, NG - 1, q7_s[...])
        for jj, j in enumerate(CHUNKS):
            if startup and jj % 2 == 0:
                wqkv_copy(jj).wait()
                wqkv_copy(jj + 1).wait()
                for u in range(jj + 3, min(jj + 5, NNC)):
                    wqkv_copy(u).start()
                if jj == NNC - 6:
                    x_copy(1).start()
                if jj == NNC - 2:
                    x_copy(1).wait()
                    for b in range(2, NTB):
                        x_copy(b).start()
                    wo_copy.start()
            y = jnp.dot(_unpack(xn[min(jj // 2, 1)]),
                        wqkv[j // 2, :, j % 2 * NC:(j % 2 + 1) * NC], preferred_element_type=F32)
            if jj == 1:
                xn[1] = xn[0]
            kind, c0 = divmod(j * NC, D)
            for c in range(NC // 128):
                g = c0 // 128 + c
                yc = y[:, c * 128:(c + 1) * 128]
                if kind == 0 and g == NG - 1:
                    q7_s[...] = _pack(yc * QSCALE)
                elif kind == 0:
                    store_q(i, g, _pack(yc * QSCALE))
                elif kind == 1:
                    store_k(i, g, _pack(yc))
                else:
                    for t in range(TB // QB):
                        vt_s[i * (TB // QB) + t, g * 64:(g + 1) * 64, :] = _pack(
                            yc[t * QB:(t + 1) * QB, :].T)
            if startup:
                if jj >= NNC - 2:
                    for c in range(4):
                        ln_rows(nxt, (jj - NNC + 2) * (TB // 2) + c * (TB // 8), TB // 8)
            elif 2 <= jj < 10:
                ln_rows(nxt, (jj - 2) * (TB // 8), TB // 8)

    def tri():
        kk = lax.broadcasted_iota(I32, (QB, QB), 0)
        qq = lax.broadcasted_iota(I32, (QB, QB), 1)
        return kk <= qq

    def scores(qb, g, nk, slot):
        kk = lax.broadcasted_iota(I32, (QB, QB), 0)
        qq = lax.broadcasted_iota(I32, (QB, QB), 1)
        grp = lane_group(SUB // 2)
        n = SUB // 2
        for h in range(4):
            hd = g * 4 + h
            tiles = [k_s[hd, _rows(qb - b, QB // 2), :] for b in range(nk)]
            if nk == 3:
                new, mid, old = tiles
                diag = jnp.where(grp >= 2,
                                 jnp.where(grp >= 3, old[3 * n:], old[2 * n:3 * n]),
                                 jnp.where(grp >= 1, old[n:2 * n], old[:n]))
                lhs = [diag, new[:n]] + [
                    jnp.where(grp >= c, new[c * n:(c + 1) * n], old[c * n:(c + 1) * n])
                    for c in range(1, 4)] + [mid]
            else:
                lhs = tiles
            st = lax.dot_general(_unpack(jnp.concatenate(lhs, axis=0)),
                                 _unpack(q_s[hd, _rows(qb, QB // 2), :]), NT,
                                 preferred_element_type=F32)
            if nk == 3:
                t = jnp.where((kk > qq) & (kk // SUB == qq // SUB),
                              jnp.concatenate([st[:SUB]] * 4, axis=0), st[SUB:SUB + QB])
                st = st[SUB:]
            else:
                t = jnp.where(kk <= qq, st[:QB], -1e30)
            s_s[slot, h, 0:QB, :] = t
            if nk >= 2:
                s_s[slot, h, QB:2 * QB, :] = st[QB:]
                t = jnp.maximum(t, st[QB:])
            m_s[slot, h] = jnp.max(t.reshape(QB // 8, 8, QB), axis=0)

    def softmax_pv(qb, g, nk, slot, odd):
        newest = tri()
        outs = []
        for h in range(4):
            m = jnp.max(m_s[slot, h], axis=0, keepdims=True)
            p0 = jnp.exp2(s_s[slot, h, 0:QB, :] - m)
            p1 = jnp.exp2(s_s[slot, h, QB:2 * QB, :] - m) if nk >= 2 else None
            if nk == 3:
                pt = [jnp.where(newest, p0, 0.0), jnp.where(newest, 0.0, p0)]
                backs = [0, 2]
            else:
                pt, backs = [p0], [0]
            if nk >= 2:
                pt, backs = pt + [p1], backs + [1]
            l = sum(jnp.sum(p.reshape(16, 8, QB), axis=0) for p in (p0, p1) if p is not None)
            l = jnp.sum(l, axis=0, keepdims=True)
            r0 = (g * 4 + h) * (DH // 2)
            vt = jnp.concatenate([vt_s[qb - b, r0:r0 + DH // 2, :] for b in backs], axis=1)
            ot = jnp.dot(_unpack(vt), jnp.concatenate(pt, axis=0).astype(BF),
                         preferred_element_type=F32)
            outs.append(ot * (1.0 / l))
        ot = jnp.concatenate(outs, axis=0)
        if odd and g + 1 == NG:
            ot_s[...] = ot
        else:
            o_s[_rows(odd, QB // 2), g * 128:(g + 1) * 128] = _pack(ot.T)

    def router(i, slot, c):
        wr = wr_ref[...].astype(F32).reshape(1, D)
        tok = lax.broadcasted_iota(I32, (8, 128), 0) + i * TB
        best, arg = best_s[...], arg_s[...]
        rows = _rows(i * (TB // RC) + c, RC)
        x1 = x_s[rows, :].astype(F32) + y_s[slot, c * RC:(c + 1) * RC, :]
        xn1 = _layernorm(x1)
        n_s[rows, :] = xn1
        r = jnp.broadcast_to(jnp.sum(xn1 * wr, axis=-1, keepdims=True), (RC, 128))
        x_s[rows, :] = (x1 + xn1).astype(BF)
        for t in range(RC // 8):
            rt = r[t * 8:(t + 1) * 8]
            arg = jnp.where(rt > best, tok + (c * RC + t * 8), arg)
            best = jnp.where(rt > best, rt, best)
        best_s[...] = jnp.where(i < NTB, best, -jnp.inf)
        arg_s[...] = arg

    def out_proj(slot, prev):
        o_s[QB // 2:, D - 128:] = _pack(ot_s[...].T)
        for j in range(D // 128):
            for c in range(j * TB // RC // 8, (j + 1) * TB // RC // 8):
                router(prev, 1 - slot, c)
            cols = slice(j * 128, (j + 1) * 128)
            y_s[slot, :, cols] = jnp.dot(_unpack(o_s[...]), wo[:, cols],
                                         preferred_element_type=F32)

    def out_tail(slot):
        o_s[QB // 2:, D - 128:] = _pack(ot_s[...].T)
        todo = [(NTB - 2, 1 - slot, c) for c in range(TB // RC)]
        for r0, r1, every in ((0, 192, 1), (192, 256, 2)):
            for j in range(D // 128):
                if j % every == 0:
                    router(*todo.pop(0))
                cols = slice(j * 128, (j + 1) * 128)
                y_s[slot, r0:r1, cols] = jnp.dot(_unpack(o_s[r0 // 2:r1 // 2, :]), wo[:, cols],
                                                 preferred_element_type=F32)
            todo += [(NTB - 1, slot, c) for c in range(r0 // RC, r1 // RC)]
        for t in todo:
            router(*t)

    def attn_first():
        store_q(NTB - 1, NG - 1, q7_s[...])
        for g in range(-1, NG):
            if g + 1 < NG:
                scores(0, g + 1, 1, 2 + (g + 1) % 2)
                scores(1, g + 1, 2, (g + 1) % 2)
            else:
                scores(2, 0, 3, 0)
            if g >= 0:
                softmax_pv(0, g, 1, 2 + g % 2, 0)
                softmax_pv(1, g, 2, g % 2, 1)

    def attn_pair(i, nks, nxt):
        for odd in range(2):
            qb = 2 * i + odd
            for g in range(NG):
                if g + 1 < NG:
                    scores(qb, g + 1, nks[odd], (g + 1) % 2)
                elif odd:
                    scores(nxt, 0, 3, 0)
                else:
                    scores(qb + 1, 0, nks[1], 0)
                if nks[0] == 3 and g == 0 and not odd:
                    out_proj(i % 2, jnp.where(i >= 2, i - 2, NTB))
                softmax_pv(qb, g, nks[odd], g % 2, odd)

    def ffn(first, last):
        best = best_s[...]
        rmax = jnp.max(best, axis=0, keepdims=True)
        idx = jnp.min(jnp.where(best == rmax, arg_s[...], S - 1))
        idx = jnp.clip(idx, 0, S - 1)

        @pl.when(first)
        def _():
            for c in ffn_copies():
                c.wait()

        xs = jnp.broadcast_to(n_s[pl.ds(idx, 1), :], (16, D)).astype(BF)
        hs = []
        for j in range(F // 128):
            gj = jnp.dot(xs, wg[j], preferred_element_type=F32)
            uj = jnp.dot(xs, wu[j], preferred_element_type=F32)
            hs.append((gj * jax.nn.sigmoid(gj) * uj).astype(BF))
            if j < 16:
                ln_rows(0, j * 16, 16)
        hid = jnp.concatenate(hs, axis=1)
        y = jnp.concatenate(
            [jnp.dot(hid, wd[j], preferred_element_type=F32) for j in range(D // 128)], axis=1)
        y = y * jax.nn.sigmoid(rmax[:, 0:1])

        @pl.when(last)
        def _():
            for i in range(NTB):
                out_copy(i).wait()

        rows = _rows(idx // 16, 16)
        x = x_s[rows, :].astype(F32)
        sel = lax.broadcasted_iota(I32, (16, D), 0) == idx % 16
        x_s[rows, :] = jnp.where(sel, x + y, x).astype(BF)

        @pl.when(first & (idx < TB))
        def _():
            xn[0, _rows(idx // 16, 8), :] = _pack(_layernorm(x_s[rows, :].astype(F32)))

        @pl.when(last)
        def _():
            fix = pltpu.make_async_copy(x_s.at[rows], out_hbm.at[0, rows], o_sem.at[0])
            fix.start()
            fix.wait()

    x_copy(0).start()
    wqkv_copy(0).start()
    wqkv_copy(1).start()
    x_s[_rows(NTB, TB), :] = jnp.zeros((TB, D), BF)
    y_s[0] = jnp.zeros((TB, D), F32)
    best_s[...] = jnp.zeros((8, 128), F32)
    arg_s[...] = jnp.zeros((8, 128), I32)
    x_copy(0).wait()
    for c in range(8):
        ln_rows(0, c * (TB // 8), TB // 8)
    wqkv_copy(2).start()
    qkv_block(0, 1, True)

    def layer(l, carry):
        first = l == 0
        last = l == 1

        def qkv_body(i, c):
            @pl.when(first & (i + 1 < NTB))
            def _():
                x_copy(i + 1).wait()
            qkv_block(i, (i + 1) % NTB, False)
            return c
        lax.fori_loop(1 - l, NTB, qkv_body, 0)

        @pl.when(first)
        def _():
            for c in ffn_copies():
                c.start()
            wo_copy.wait()

        attn_first()

        def attn_body(i, c):
            @pl.when(last & (i > 2))
            def _():
                out_copy(i - 3).start()
            attn_pair(i, (3, 3), jnp.minimum(2 * i + 2, NQB - 1))
            return c
        lax.fori_loop(1, NTB, attn_body, 0)

        out_tail(l // 2)

        @pl.when(last)
        def _():
            for i in range(NTB - 3, NTB):
                out_copy(i).start()

        ffn(first, last)
        return carry

    lax.fori_loop(0, 2, layer, 0)


@jax.jit
def pallas_interleave_layers__sliding_block__moe_arch_mod__prompt_kernel(
    A_x: jax.Array,
    A_wqkv: jax.Array,
    A_wo: jax.Array,
    B_x: jax.Array,
    B_w_r: jax.Array,
    B_w_gate: jax.Array,
    B_w_up: jax.Array,
    B_w_down: jax.Array,
):
    del B_x
    hbm = pl.BlockSpec(memory_space=pl.ANY)
    return pl.pallas_call(
        _kernel,
        in_specs=[hbm, hbm, hbm, pl.BlockSpec(memory_space=pltpu.VMEM), hbm, hbm, hbm],
        out_specs=hbm,
        out_shape=jax.ShapeDtypeStruct((1, S, D), BF),
        scratch_shapes=[
            pltpu.VMEM((S + TB, D), BF),
            pltpu.VMEM((S + TB, D), F32),
            pltpu.VMEM((2, TB // 2, D), I32),
            pltpu.VMEM((NNC // 2, D, 2 * NC), BF),
            pltpu.VMEM((D, D), BF),
            pltpu.VMEM((F // 128, D, 128), BF),
            pltpu.VMEM((F // 128, D, 128), BF),
            pltpu.VMEM((D // 128, F, 128), BF),
            pltpu.VMEM((4 * NG, S // 2, 128), I32),
            pltpu.VMEM((TB // 2, 128), I32),
            pltpu.VMEM((4 * NG, S // 2, 128), I32),
            pltpu.VMEM((NQB, D // 2, QB), I32),
            pltpu.VMEM((TB // 2, D), I32),
            pltpu.VMEM((128, QB), F32),
            pltpu.VMEM((2, TB, D), F32),
            pltpu.VMEM((8, 128), F32),
            pltpu.VMEM((8, 128), I32),
            pltpu.VMEM((4, 4, 2 * QB, QB), F32),
            pltpu.VMEM((4, 4, 8, QB), F32),
            pltpu.SemaphoreType.DMA((NTB,)),
            pltpu.SemaphoreType.DMA((NNC // 2 + 2,)),
            pltpu.SemaphoreType.DMA((NTB,)),
        ],
        compiler_params=pltpu.CompilerParams(vmem_limit_bytes=100 * 1024 * 1024),
        name="mod_swa",
    )(A_x, A_wqkv, A_wo, B_w_r, B_w_gate, B_w_up, B_w_down)
```

```python
import math

import jax
import jax.numpy as jnp
from jax import lax
import jax.experimental.pallas as pl
import jax.experimental.pallas.tpu as pltpu

S = 2048
D = 1024
DH = 32
F = 3584
TB = 256
NTB = S // TB
QB = 128
NQB = S // QB
NG = D // 128
NC = 256
NNC = 3 * D // NC
CHUNKS = [8, 9, 10, 11, 4, 5, 6, 7, 0, 1, 2, 3]
RC = 32
SUB = 32
EPS = 1e-5
QSCALE = (DH ** -0.5) * math.log2(math.e)

BF = jnp.bfloat16
F32 = jnp.float32
I32 = jnp.int32
NT = (((1,), (1,)), ((), ()))


def _pack(v):
    return pltpu.bitcast(v.astype(BF), I32)


def _unpack(v):
    return pltpu.bitcast(v, BF)


def _round(v):
    return v.astype(BF).astype(F32)


def _layernorm(x):
    m = jnp.sum(x, axis=-1, keepdims=True) * (1.0 / D)
    xc = x - m
    v = jnp.sum(xc * xc, axis=-1, keepdims=True) * (1.0 / D)
    sd = _round(jnp.sqrt(_round(_round(v) + EPS)))
    return _round(_round(x - _round(m)) * (1.0 / sd))


def _lhs_terms(top, bot):
    a11, a12, a21, a22 = top[:, :D // 2], top[:, D // 2:], bot[:, :D // 2], bot[:, D // 2:]
    return [a11, a11 + a12, a22, a21 + a22, a11 + a22, a12 - a22, a21 - a11]


def _rhs_term(t, b):
    first, sign, second = (((0, 1), -1, (1, 1)), ((1, 1), 0, None), ((1, 0), -1, (0, 0)),
                           ((0, 0), 0, None), ((0, 0), 1, (1, 1)), ((1, 0), 1, (1, 1)),
                           ((0, 0), 1, (0, 1)))[t]
    if sign == 0:
        return pltpu.bitcast(b(*first), I32)
    u, v = b(*first).astype(F32), b(*second).astype(F32)
    return _pack(u + v if sign > 0 else u - v)


def _strassen(product):
    m3, m5 = product(0), product(1)
    c12 = m3 + m5
    m4 = product(2)
    c11 = m4 - m5
    m2 = product(3)
    c21 = m2 + m4
    c22 = m3 - m2
    m1 = product(4)
    c11, c22 = c11 + m1, c22 + m1
    c11 = c11 + product(5)
    c22 = c22 + product(6)
    return [[c11, c12], [c21, c22]]


def _rows(i, n):
    return pl.ds(i * n if isinstance(i, int) else pl.multiple_of(i * n, n), n)


def _kernel(x_hbm, wqkv_hbm, wo_hbm, wr_ref, wg_hbm, wu_hbm, wd_hbm, out_hbm,
            x_s, n_s, xn0, xn, wqkv, wqkv7, wo, wo7, o7, wg, wu, wd, q_s, q7_s, k_s, vt_s, o_s, ot_s, y_s, best_s, arg_s,
            s_s, m_s,
            x_sem, w_sem, o_sem):

    def x_copy(i):
        return pltpu.make_async_copy(x_hbm.at[0, _rows(i, TB)], x_s.at[_rows(i, TB)],
                                     x_sem.at[i])

    def out_copy(i):
        return pltpu.make_async_copy(x_s.at[_rows(i, TB)], out_hbm.at[0, _rows(i, TB)],
                                     o_sem.at[i])

    def wqkv_copy(jj):
        j = CHUNKS[jj] // 2
        rows = pl.ds(jj % 2 * D // 2, D // 2)
        return pltpu.make_async_copy(
            wqkv_hbm.at[rows, pl.ds(j * 2 * NC, 2 * NC)], wqkv.at[j, rows], w_sem.at[j])

    def wo_copies(k):
        return [pltpu.make_async_copy(wo_hbm.at[_rows(k + 4 * h, D // 8)],
                                      wo.at[_rows(k + 4 * h, D // 8)], w_sem.at[NNC // 2 + 1 + k])
                for h in range(2)]

    def late_copies():
        return [x_copy(b) for b in range(3, NTB)] + sum((wo_copies(k) for k in range(1, 4)), [])

    def ffn_copies():
        cs = []
        for j in range(F // 128):
            cs.append(pltpu.make_async_copy(
                wg_hbm.at[:, pl.ds(j * 128, 128)], wg.at[j], w_sem.at[NNC // 2]))
            cs.append(pltpu.make_async_copy(
                wu_hbm.at[:, pl.ds(j * 128, 128)], wu.at[j], w_sem.at[NNC // 2]))
        for j in range(D // 128):
            cs.append(pltpu.make_async_copy(
                wd_hbm.at[:, pl.ds(j * 128, 128)], wd.at[j], w_sem.at[NNC // 2]))
        return cs

    def ln_terms(i, c):
        top, bot = [_layernorm(x_s[_rows(i * (TB // 16) + h * (TB // 32) + c, 16), :].astype(F32))
                    for h in range(2)]
        for t, a in enumerate(_lhs_terms(top, bot)):
            xn[0, t, _rows(c, 8), :] = _pack(a)

    def wo_terms(c):
        for t in range(7):
            wo7[t, _rows(c, 8), :] = _rhs_term(
                t, lambda i, j: wo[_rows(c + i * (D // 32), 16), _rows(j, D // 2)])

    def lane_group(n):
        return lax.broadcasted_iota(I32, (n, 128), 1) // DH

    def store_q(i, g, q):
        grp = lane_group(SUB // 2)
        rolled = [q] + [pltpu.roll(q, DH * t, 1) for t in range(1, 4)]
        for h in range(4):
            parts = []
            for c in range(TB // SUB):
                b = c % 4
                rows = slice(c * SUB // 2, (c + 1) * SUB // 2)
                parts.append(jnp.where(grp == b, rolled[(b - h) % 4][rows], 0))
            q_s[g * 4 + h, _rows(i, TB // 2), :] = jnp.concatenate(parts, axis=0)

    def store_k(i, g, k):
        grp = lane_group(TB // 2)
        even = grp % 2 == 0
        low = grp < 2
        pairs = [jnp.where(even, k, pltpu.roll(k, DH, 1)),
                 jnp.where(even, pltpu.roll(k, 3 * DH, 1), k)]
        for h in range(2):
            swapped = pltpu.roll(pairs[h], 2 * DH, 1)
            k_s[g * 4 + h, _rows(i, TB // 2), :] = jnp.where(low, pairs[h], swapped)
            k_s[g * 4 + h + 2, _rows(i, TB // 2), :] = jnp.where(low, swapped, pairs[h])

    def store_qkv(i, col, y):
        kind, g = divmod(col // 128, NG)
        if kind == 0 and g == NG - 1:
            q7_s[...] = _pack(y * QSCALE)
        elif kind == 0:
            store_q(i, g, _pack(y * QSCALE))
        elif kind == 1:
            store_k(i, g, _pack(y))
        else:
            for t in range(TB // QB):
                vt_s[i * (TB // QB) + t, g * 64:(g + 1) * 64, :] = _pack(y[t * QB:(t + 1) * QB].T)

    def qkv_block(i, nxt, startup=False):
        if not startup:
            store_q((i + NTB - 1) % NTB, NG - 1, q7_s[...])
        for jj, j in enumerate(CHUNKS):
            if startup and jj % 2 == 0:
                wqkv_copy(jj).wait()
                wqkv_copy(jj + 1).wait()
                for u in range(jj + 4, min(jj + 6, NNC)):
                    wqkv_copy(u).start()
                if jj == 2:
                    x_copy(1).start()
                if jj == 4:
                    x_copy(1).wait()
                if jj == NNC - 4:
                    x_copy(2).start()
                    for c in wo_copies(0):
                        c.start()

            def product(t):
                if startup:
                    w = _rhs_term(t, lambda r, c: wqkv[j // 2, _rows(r, D // 2),
                                                       _rows(2 * c + j % 2, 128)])
                    wqkv7[j, t] = w
                else:
                    w = wqkv7[j, t]
                return jnp.dot(_unpack(xn[min(jj // 2, 1), t]), _unpack(w),
                               preferred_element_type=F32)

            y = _strassen(product)
            if jj == 1:
                xn[1] = xn[0]
            for c in range(2):
                store_qkv(i, j // 2 * 2 * NC + c * NC + j % 2 * 128,
                          jnp.concatenate([y[0][c], y[1][c]], axis=0))
            if startup:
                if jj >= 4:
                    ln_terms(nxt, jj - 4)
            elif 2 <= jj < 10:
                ln_terms(nxt, jj - 2)
                wo_terms((i + 3) % 4 * 8 + jj - 2)

    def tri():
        kk = lax.broadcasted_iota(I32, (QB, QB), 0)
        qq = lax.broadcasted_iota(I32, (QB, QB), 1)
        return kk <= qq

    def scores(qb, g, nk, slot):
        kk = lax.broadcasted_iota(I32, (QB, QB), 0)
        qq = lax.broadcasted_iota(I32, (QB, QB), 1)
        grp = lane_group(SUB // 2)
        n = SUB // 2
        for h in range(4):
            hd = g * 4 + h
            tiles = [k_s[hd, _rows(qb - b, QB // 2), :] for b in range(nk)]
            if nk == 3:
                new, mid, old = tiles
                diag = jnp.where(grp >= 2,
                                 jnp.where(grp >= 3, old[3 * n:], old[2 * n:3 * n]),
                                 jnp.where(grp >= 1, old[n:2 * n], old[:n]))
                lhs = [diag, new[:n]] + [
                    jnp.where(grp >= c, new[c * n:(c + 1) * n], old[c * n:(c + 1) * n])
                    for c in range(1, 4)] + [mid]
            else:
                lhs = tiles
            st = lax.dot_general(_unpack(jnp.concatenate(lhs, axis=0)),
                                 _unpack(q_s[hd, _rows(qb, QB // 2), :]), NT,
                                 preferred_element_type=F32)
            if nk == 3:
                t = jnp.where((kk > qq) & (kk // SUB == qq // SUB),
                              jnp.concatenate([st[:SUB]] * 4, axis=0), st[SUB:SUB + QB])
                st = st[SUB:]
            else:
                t = jnp.where(kk <= qq, st[:QB], -1e30)
            s_s[slot, h, 0:QB, :] = t
            if nk >= 2:
                s_s[slot, h, QB:2 * QB, :] = st[QB:]
                t = jnp.maximum(t, st[QB:])
            m_s[slot, h] = jnp.max(t.reshape(QB // 8, 8, QB), axis=0)

    def softmax_pv(qb, g, nk, slot, odd):
        newest = tri()
        outs = []
        for h in range(4):
            m = jnp.max(m_s[slot, h], axis=0, keepdims=True)
            p0 = jnp.exp2(s_s[slot, h, 0:QB, :] - m)
            p1 = jnp.exp2(s_s[slot, h, QB:2 * QB, :] - m) if nk >= 2 else None
            if nk == 3:
                pt = [jnp.where(newest, p0, 0.0), jnp.where(newest, 0.0, p0)]
                backs = [0, 2]
            else:
                pt, backs = [p0], [0]
            if nk >= 2:
                pt, backs = pt + [p1], backs + [1]
            l = sum(jnp.sum(p.reshape(16, 8, QB), axis=0) for p in (p0, p1) if p is not None)
            l = jnp.sum(l, axis=0, keepdims=True)
            r0 = (g * 4 + h) * (DH // 2)
            vt = jnp.concatenate([vt_s[qb - b, r0:r0 + DH // 2, :] for b in backs], axis=1)
            ot = jnp.dot(_unpack(vt), jnp.concatenate(pt, axis=0).astype(BF),
                         preferred_element_type=F32)
            outs.append(ot * (1.0 / l))
        ot = jnp.concatenate(outs, axis=0)
        if odd and g + 1 == NG:
            ot_s[...] = ot
        else:
            o_s[_rows(odd, QB), g * 128:(g + 1) * 128] = ot.T

    def router(i, slot, c):
        wr = wr_ref[...].astype(F32).reshape(1, D)
        tok = lax.broadcasted_iota(I32, (8, 128), 0) + i * TB
        best, arg = best_s[...], arg_s[...]
        rows = _rows(i * (TB // RC) + c, RC)
        x1 = x_s[rows, :].astype(F32) + y_s[slot, c * RC:(c + 1) * RC, :]
        xn1 = _layernorm(x1)
        n_s[rows, :] = xn1
        r = jnp.broadcast_to(jnp.sum(xn1 * wr, axis=-1, keepdims=True), (RC, 128))
        x_s[rows, :] = (x1 + xn1).astype(BF)
        for t in range(RC // 8):
            rt = r[t * 8:(t + 1) * 8]
            arg = jnp.where(rt > best, tok + (c * RC + t * 8), arg)
            best = jnp.where(rt > best, rt, best)
        best_s[...] = jnp.where(i < NTB, best, -jnp.inf)
        arg_s[...] = arg

    def out_proj(slot, prev):
        o_s[QB:, D - 128:] = ot_s[...].T
        for t, a in enumerate(_lhs_terms(o_s[:QB, :], o_s[QB:, :])):
            o7[t] = _pack(a)
        for j in range(4):
            for c in range(j * TB // RC // 4, (j + 1) * TB // RC // 4):
                router(prev, 1 - slot, c)
            y = _strassen(lambda t: jnp.dot(
                _unpack(o7[t]), _unpack(wo7[t, :, j * 128:(j + 1) * 128]),
                preferred_element_type=F32))
            for r, c in ((0, 1), (1, 0), (0, 0), (1, 1)):
                y_s[slot, _rows(r, QB), _rows(c * 4 + j, 128)] = y[r][c]

    def out_tail(slot):
        o_s[QB:, D - 128:] = ot_s[...].T
        xn0[...] = _pack(o_s[...])
        todo = [(NTB - 2, 1 - slot, c) for c in range(TB // RC)]
        for r0, r1, every in ((0, 192, 1), (192, 256, 2)):
            for j in range(D // 128):
                if j % every == 0:
                    router(*todo.pop(0))
                cols = slice(j * 128, (j + 1) * 128)
                y_s[slot, r0:r1, cols] = jnp.dot(_unpack(xn0[r0 // 2:r1 // 2, :]), wo[:, cols],
                                                 preferred_element_type=F32)
            todo += [(NTB - 1, slot, c) for c in range(r0 // RC, r1 // RC)]
        for t in todo:
            router(*t)

    def attn_first():
        store_q(NTB - 1, NG - 1, q7_s[...])
        for g in range(-1, NG):
            if g + 1 < NG:
                scores(0, g + 1, 1, 2 + (g + 1) % 2)
                scores(1, g + 1, 2, (g + 1) % 2)
            else:
                scores(2, 0, 3, 0)
            if g >= 0:
                softmax_pv(0, g, 1, 2 + g % 2, 0)
                softmax_pv(1, g, 2, g % 2, 1)

    def attn_pair(i, nks, nxt):
        for odd in range(2):
            qb = 2 * i + odd
            for g in range(NG):
                if g + 1 < NG:
                    scores(qb, g + 1, nks[odd], (g + 1) % 2)
                elif odd:
                    scores(nxt, 0, 3, 0)
                else:
                    scores(qb + 1, 0, nks[1], 0)
                if nks[0] == 3 and g == 0 and not odd:
                    out_proj(i % 2, jnp.where(i >= 2, i - 2, NTB))
                softmax_pv(qb, g, nks[odd], g % 2, odd)

    def ffn(first, last):
        best = best_s[...]
        rmax = jnp.max(best, axis=0, keepdims=True)
        idx = jnp.min(jnp.where(best == rmax, arg_s[...], S - 1))
        idx = jnp.clip(idx, 0, S - 1)

        @pl.when(first)
        def _():
            for c in ffn_copies():
                c.wait()

        xs = jnp.broadcast_to(n_s[pl.ds(idx, 1), :], (16, D)).astype(BF)
        nf = F // 128 // 2

        def ffn_body(k, y):
            hs = []
            for j in range(nf):
                gj = jnp.dot(xs, wg[k * nf + j], preferred_element_type=F32)
                uj = jnp.dot(xs, wu[k * nf + j], preferred_element_type=F32)
                hs.append((gj * jax.nn.sigmoid(gj) * uj).astype(BF))
                if j % 4 == 0:
                    ln_terms(0, k * 4 + j // 4)
            hid = jnp.concatenate(hs, axis=1)
            return y + jnp.concatenate(
                [jnp.dot(hid, wd[j, _rows(k, F // 2), :], preferred_element_type=F32)
                 for j in range(D // 128)], axis=1)
        y = lax.fori_loop(0, 2, ffn_body, jnp.zeros((16, D), F32))
        y = y * jax.nn.sigmoid(rmax[:, 0:1])

        @pl.when(last)
        def _():
            for i in range(NTB):
                out_copy(i).wait()

        rows = _rows(idx // 16, 16)
        x = x_s[rows, :].astype(F32)
        sel = lax.broadcasted_iota(I32, (16, D), 0) == idx % 16
        x_s[rows, :] = jnp.where(sel, x + y, x).astype(BF)

        @pl.when(first & (idx < TB))
        def _():
            ln_terms(0, idx // 16 % 8)

        @pl.when(last)
        def _():
            fix = pltpu.make_async_copy(x_s.at[rows], out_hbm.at[0, rows], o_sem.at[0])
            fix.start()
            fix.wait()

    x_copy(0).start()
    wqkv_copy(0).start()
    wqkv_copy(1).start()
    x_s[_rows(NTB, TB), :] = jnp.zeros((TB, D), BF)
    y_s[0] = jnp.zeros((TB, D), F32)
    best_s[...] = jnp.zeros((8, 128), F32)
    arg_s[...] = jnp.zeros((8, 128), I32)
    x_copy(0).wait()
    wqkv_copy(2).start()

    def ln_body(k, c):
        for t in range(4):
            ln_terms(0, 4 * k + t)
        return c
    lax.fori_loop(0, 2, ln_body, 0)
    wqkv_copy(3).start()
    qkv_block(0, 1, True)

    def layer(l, carry):
        first = l == 0
        last = l == 1

        def qkv_body(i, c):
            @pl.when(first & (i == 1))
            def _():
                x_copy(2).wait()
                for cp in wo_copies(0):
                    cp.wait()
                for cp in late_copies():
                    cp.start()

            @pl.when(first & (i == 2))
            def _():
                for cp in late_copies():
                    cp.wait()
                for cp in ffn_copies():
                    cp.start()
            qkv_block(i, (i + 1) % NTB)
            return c
        lax.fori_loop(1 - l, NTB, qkv_body, 0)

        attn_first()

        def attn_body(i, c):
            @pl.when(last & (i > 2))
            def _():
                out_copy(i - 3).start()
            attn_pair(i, (3, 3), jnp.minimum(2 * i + 2, NQB - 1))
            return c
        lax.fori_loop(1, NTB, attn_body, 0)

        out_tail(l // 2)

        @pl.when(last)
        def _():
            for i in range(NTB - 3, NTB):
                out_copy(i).start()

        ffn(first, last)
        return carry

    lax.fori_loop(0, 2, layer, 0)


@jax.jit
def pallas_interleave_layers__sliding_block__moe_arch_mod__prompt_kernel(
    A_x: jax.Array,
    A_wqkv: jax.Array,
    A_wo: jax.Array,
    B_x: jax.Array,
    B_w_r: jax.Array,
    B_w_gate: jax.Array,
    B_w_up: jax.Array,
    B_w_down: jax.Array,
):
    del B_x
    hbm = pl.BlockSpec(memory_space=pl.ANY)
    return pl.pallas_call(
        _kernel,
        in_specs=[hbm, hbm, hbm, pl.BlockSpec(memory_space=pltpu.VMEM), hbm, hbm, hbm],
        out_specs=hbm,
        out_shape=jax.ShapeDtypeStruct((1, S, D), BF),
        scratch_shapes=[
            pltpu.VMEM((S + TB, D), BF),
            pltpu.VMEM((S + TB, D), F32),
            pltpu.VMEM((TB // 2, D), I32),
            pltpu.VMEM((2, 7, QB // 2, D // 2), I32),
            pltpu.VMEM((NNC // 2, D, 2 * NC), BF),
            pltpu.VMEM((NNC, 7, D // 4, 128), I32),
            pltpu.VMEM((D, D), BF),
            pltpu.VMEM((7, D // 4, D // 2), I32),
            pltpu.VMEM((7, QB // 2, D // 2), I32),
            pltpu.VMEM((F // 128, D, 128), BF),
            pltpu.VMEM((F // 128, D, 128), BF),
            pltpu.VMEM((D // 128, F, 128), BF),
            pltpu.VMEM((4 * NG, S // 2, 128), I32),
            pltpu.VMEM((TB // 2, 128), I32),
            pltpu.VMEM((4 * NG, S // 2, 128), I32),
            pltpu.VMEM((NQB, D // 2, QB), I32),
            pltpu.VMEM((TB, D), F32),
            pltpu.VMEM((128, QB), F32),
            pltpu.VMEM((2, TB, D), F32),
            pltpu.VMEM((8, 128), F32),
            pltpu.VMEM((8, 128), I32),
            pltpu.VMEM((4, 4, 2 * QB, QB), F32),
            pltpu.VMEM((4, 4, 8, QB), F32),
            pltpu.SemaphoreType.DMA((NTB,)),
            pltpu.SemaphoreType.DMA((NNC // 2 + 5,)),
            pltpu.SemaphoreType.DMA((NTB,)),
        ],
        compiler_params=pltpu.CompilerParams(vmem_limit_bytes=112 * 1024 * 1024),
        name="mod_swa",
    )(A_x, A_wqkv, A_wo, B_w_r, B_w_gate, B_w_up, B_w_down)
```

```python
import math

import jax
import jax.numpy as jnp
from jax import lax
import jax.experimental.pallas as pl
import jax.experimental.pallas.tpu as pltpu

S = 2048
D = 1024
DH = 32
F = 3584
TB = 256
NTB = S // TB
QB = 128
NQB = S // QB
NG = D // 128
NC = 256
NNC = 3 * D // NC
CHUNKS = [4, 5, 6, 7, 8, 9, 10, 11, 0, 1, 2, 3]
RC = 32
SUB = 32
EPS = 1e-5
QSCALE = (DH ** -0.5) * math.log2(math.e)

BF = jnp.bfloat16
F32 = jnp.float32
I32 = jnp.int32
NT = (((1,), (1,)), ((), ()))


def _pack(v):
    return pltpu.bitcast(v.astype(BF), I32)


def _unpack(v):
    return pltpu.bitcast(v, BF)


def _round(v):
    return v.astype(BF).astype(F32)


def _layernorm(x):
    m = jnp.sum(x, axis=-1, keepdims=True) * (1.0 / D)
    xc = x - m
    v = jnp.sum(xc * xc, axis=-1, keepdims=True) * (1.0 / D)
    sd = _round(jnp.sqrt(_round(_round(v) + EPS)))
    return xc * (1.0 / sd)


def _lhs_terms(top, bot):
    a11, a12, a21, a22 = top[:, :D // 2], top[:, D // 2:], bot[:, :D // 2], bot[:, D // 2:]
    return [a11, a11 + a12, a22, a21 + a22, a11 + a22, a12 - a22, a21 - a11]


def _rhs_term(t, b):
    first, sign, second = (((0, 1), -1, (1, 1)), ((1, 1), 0, None), ((1, 0), -1, (0, 0)),
                           ((0, 0), 0, None), ((0, 0), 1, (1, 1)), ((1, 0), 1, (1, 1)),
                           ((0, 0), 1, (0, 1)))[t]
    if sign == 0:
        return pltpu.bitcast(b(*first), I32)
    u, v = b(*first).astype(F32), b(*second).astype(F32)
    return _pack(u + v if sign > 0 else u - v)


def _strassen(product):
    m3, m5 = product(0), product(1)
    c12 = m3 + m5
    m4 = product(2)
    c11 = m4 - m5
    m2 = product(3)
    c21 = m2 + m4
    c22 = m3 - m2
    m1 = product(4)
    c11, c22 = c11 + m1, c22 + m1
    c11 = c11 + product(5)
    c22 = c22 + product(6)
    return [[c11, c12], [c21, c22]]


def _rows(i, n):
    return pl.ds(i * n if isinstance(i, int) else pl.multiple_of(i * n, n), n)


def _kernel(x_hbm, wqkv_hbm, wo_hbm, wr_ref, wg_hbm, wu_hbm, wd_hbm, out_hbm,
            x_s, n_s, xn0, xn, wqkv, wqkv7, wo, wo7, o7, wg, wu, wd, q_s, q7_s, k_s, vt_s, o_s, ot_s, y_s, best_s, arg_s,
            s_s, m_s,
            x_sem, w_sem, o_sem):

    def x_copy(i):
        return pltpu.make_async_copy(x_hbm.at[0, _rows(i, TB)], x_s.at[_rows(i, TB)],
                                     x_sem.at[i])

    def out_copy(i):
        return pltpu.make_async_copy(x_s.at[_rows(i, TB)], out_hbm.at[0, _rows(i, TB)],
                                     o_sem.at[i])

    def wqkv_copy(jj):
        j = CHUNKS[jj] // 2
        rows = pl.ds(jj % 2 * D // 2, D // 2)
        return pltpu.make_async_copy(
            wqkv_hbm.at[rows, pl.ds(j * 2 * NC, 2 * NC)], wqkv.at[j, rows], w_sem.at[j])

    def wo_copies(k):
        return [pltpu.make_async_copy(wo_hbm.at[_rows(k + 4 * h, D // 8)],
                                      wo.at[_rows(k + 4 * h, D // 8)], w_sem.at[NNC // 2 + 1 + k])
                for h in range(2)]

    def late_copies():
        return [x_copy(b) for b in range(3, NTB)] + sum((wo_copies(k) for k in range(1, 4)), [])

    def ffn_copies():
        cs = []
        for j in range(F // 128):
            cs.append(pltpu.make_async_copy(
                wg_hbm.at[:, pl.ds(j * 128, 128)], wg.at[j], w_sem.at[NNC // 2]))
            cs.append(pltpu.make_async_copy(
                wu_hbm.at[:, pl.ds(j * 128, 128)], wu.at[j], w_sem.at[NNC // 2]))
        for j in range(D // 128):
            cs.append(pltpu.make_async_copy(
                wd_hbm.at[:, pl.ds(j * 128, 128)], wd.at[j], w_sem.at[NNC // 2]))
        return cs

    def ln_terms(i, c, chain=True):
        top, bot = [_layernorm(x_s[_rows(i * (TB // 16) + h * (TB // 32) + c, 16), :].astype(F32))
                    for h in range(2)]
        for t, a in enumerate(_lhs_terms(top, bot)):
            xn[0, t, _rows(c, 8), :] = _pack(a)
        if chain:
            x_s[S + TB:, :128] = (top[:, :128] + bot[:, :128]).astype(BF)

    def wo_terms(c):
        for t in range(7):
            wo7[t, _rows(c, 8), :] = _rhs_term(
                t, lambda i, j: wo[_rows(c + i * (D // 32), 16), _rows(j, D // 2)])

    def lane_group(n):
        return lax.broadcasted_iota(I32, (n, 128), 1) // DH

    def store_q(i, g, q):
        grp = lane_group(SUB // 2)
        rolled = [q] + [pltpu.roll(q, DH * t, 1) for t in range(1, 4)]
        for h in range(4):
            parts = []
            for c in range(TB // SUB):
                b = c % 4
                rows = slice(c * SUB // 2, (c + 1) * SUB // 2)
                parts.append(jnp.where(grp == b, rolled[(b - h) % 4][rows], 0))
            q_s[g * 4 + h, _rows(i, TB // 2), :] = jnp.concatenate(parts, axis=0)

    def store_k(i, g, k):
        grp = lane_group(TB // 2)
        even = grp % 2 == 0
        low = grp < 2
        pairs = [jnp.where(even, k, pltpu.roll(k, DH, 1)),
                 jnp.where(even, pltpu.roll(k, 3 * DH, 1), k)]
        for h in range(2):
            swapped = pltpu.roll(pairs[h], 2 * DH, 1)
            k_s[g * 4 + h, _rows(i, TB // 2), :] = jnp.where(low, pairs[h], swapped)
            k_s[g * 4 + h + 2, _rows(i, TB // 2), :] = jnp.where(low, swapped, pairs[h])

    def store_qkv(i, col, y):
        kind, g = divmod(col // 128, NG)
        if kind == 0 and g == NG - 1:
            q7_s[...] = _pack(y * QSCALE)
        elif kind == 0:
            store_q(i, g, _pack(y * QSCALE))
        elif kind == 1:
            store_k(i, g, _pack(y))
        else:
            for t in range(TB // QB):
                vt_s[i * (TB // QB) + t, g * 64:(g + 1) * 64, :] = _pack(y[t * QB:(t + 1) * QB].T)

    def qkv_block(i, nxt, startup=False):
        if not startup:
            store_q((i + NTB - 1) % NTB, NG - 1, q7_s[...])
        for jj, j in enumerate(CHUNKS):
            if startup and jj % 2 == 0:
                wqkv_copy(jj).wait()
                wqkv_copy(jj + 1).wait()
                for u in range(jj + 4, min(jj + 6, NNC)):
                    wqkv_copy(u).start()
                if jj == 2:
                    x_copy(1).start()
                if jj == 4:
                    x_copy(1).wait()
                if jj == NNC - 4:
                    x_copy(2).start()
                    for c in wo_copies(0):
                        c.start()

            def product(t):
                if startup:
                    w = _rhs_term(t, lambda r, c: wqkv[j // 2, _rows(r, D // 2),
                                                       _rows(2 * c + j % 2, 128)])
                    wqkv7[j, t] = w
                else:
                    w = wqkv7[j, t]
                return jnp.dot(_unpack(xn[min(jj // 2, 1), t]), _unpack(w),
                               preferred_element_type=F32)

            y = _strassen(product)
            if jj == 1:
                xn[1] = xn[0]
            for c in range(2):
                store_qkv(i, j // 2 * 2 * NC + c * NC + j % 2 * 128,
                          jnp.concatenate([y[0][c], y[1][c]], axis=0))
            if startup:
                if jj >= 4:
                    ln_terms(nxt, jj - 4)
            elif 2 <= jj < 10:
                ln_terms(nxt, jj - 2)
                wo_terms((i + 3) % 4 * 8 + jj - 2)

    def tri():
        kk = lax.broadcasted_iota(I32, (QB, QB), 0)
        qq = lax.broadcasted_iota(I32, (QB, QB), 1)
        return kk <= qq

    def scores(qb, g, nk, slot):
        kk = lax.broadcasted_iota(I32, (QB, QB), 0)
        qq = lax.broadcasted_iota(I32, (QB, QB), 1)
        grp = lane_group(SUB // 2)
        n = SUB // 2
        for h in range(4):
            hd = g * 4 + h
            tiles = [k_s[hd, _rows(qb - b, QB // 2), :] for b in range(nk)]
            if nk == 3:
                new, mid, old = tiles
                diag = jnp.where(grp >= 2,
                                 jnp.where(grp >= 3, old[3 * n:], old[2 * n:3 * n]),
                                 jnp.where(grp >= 1, old[n:2 * n], old[:n]))
                lhs = [diag, new[:n]] + [
                    jnp.where(grp >= c, new[c * n:(c + 1) * n], old[c * n:(c + 1) * n])
                    for c in range(1, 4)] + [mid]
            else:
                lhs = tiles
            st = lax.dot_general(_unpack(jnp.concatenate(lhs, axis=0)),
                                 _unpack(q_s[hd, _rows(qb, QB // 2), :]), NT,
                                 preferred_element_type=F32)
            if nk == 3:
                t = jnp.where((kk > qq) & (kk // SUB == qq // SUB),
                              jnp.concatenate([st[:SUB]] * 4, axis=0), st[SUB:SUB + QB])
                st = st[SUB:]
            else:
                t = jnp.where(kk <= qq, st[:QB], -1e30)
            s_s[slot, h, 0:QB, :] = t
            if nk >= 2:
                s_s[slot, h, QB:2 * QB, :] = st[QB:]
                t = jnp.maximum(t, st[QB:])
            m_s[slot, h] = jnp.max(t.reshape(QB // 8, 8, QB), axis=0)

    def softmax_pv(qb, g, nk, slot, odd):
        newest = tri()
        outs = []
        for h in range(4):
            m = jnp.max(m_s[slot, h], axis=0, keepdims=True)
            p0 = jnp.exp2(s_s[slot, h, 0:QB, :] - m)
            p1 = jnp.exp2(s_s[slot, h, QB:2 * QB, :] - m) if nk >= 2 else None
            if nk == 3:
                pt = [jnp.where(newest, p0, 0.0), jnp.where(newest, 0.0, p0)]
                backs = [0, 2]
            else:
                pt, backs = [p0], [0]
            if nk >= 2:
                pt, backs = pt + [p1], backs + [1]
            l = sum(jnp.sum(p.reshape(16, 8, QB), axis=0) for p in (p0, p1) if p is not None)
            l = jnp.sum(l, axis=0, keepdims=True)
            r0 = (g * 4 + h) * (DH // 2)
            vt = jnp.concatenate([vt_s[qb - b, r0:r0 + DH // 2, :] for b in backs], axis=1)
            ot = jnp.dot(_unpack(vt), jnp.concatenate(pt, axis=0).astype(BF),
                         preferred_element_type=F32)
            outs.append(ot * (1.0 / l))
        ot = jnp.concatenate(outs, axis=0)
        if odd and g + 1 == NG:
            ot_s[...] = ot
        else:
            o_s[_rows(odd, QB), g * 128:(g + 1) * 128] = ot.T

    def router(i, slot, c):
        wr = wr_ref[...].astype(F32).reshape(1, D)
        tok = lax.broadcasted_iota(I32, (8, 128), 0) + i * TB
        best, arg = best_s[...], arg_s[...]
        rows = _rows(i * (TB // RC) + c, RC)
        x1 = x_s[rows, :].astype(F32) + y_s[slot, c * RC:(c + 1) * RC, :]
        xn1 = _layernorm(x1)
        n_s[rows, :] = xn1
        r = jnp.broadcast_to(jnp.sum(xn1 * wr, axis=-1, keepdims=True), (RC, 128))
        x_s[rows, :] = (x1 + xn1).astype(BF)
        for t in range(RC // 8):
            rt = r[t * 8:(t + 1) * 8]
            arg = jnp.where(rt > best, tok + (c * RC + t * 8), arg)
            best = jnp.where(rt > best, rt, best)
        best_s[...] = jnp.where(i < NTB, best, -jnp.inf)
        arg_s[...] = arg

    def out_proj(slot, prev):
        o_s[QB:, D - 128:] = ot_s[...].T
        for t, a in enumerate(_lhs_terms(o_s[:QB, :], o_s[QB:, :])):
            o7[t] = _pack(a)
        for j in range(4):
            for c in range(j * TB // RC // 4, (j + 1) * TB // RC // 4):
                router(prev, 1 - slot, c)
            y = _strassen(lambda t: jnp.dot(
                _unpack(o7[t]), _unpack(wo7[t, :, j * 128:(j + 1) * 128]),
                preferred_element_type=F32))
            for r, c in ((0, 1), (1, 0), (0, 0), (1, 1)):
                y_s[slot, _rows(r, QB), _rows(c * 4 + j, 128)] = y[r][c]

    def out_tail(slot):
        o_s[QB:, D - 128:] = ot_s[...].T
        xn0[...] = _pack(o_s[...])
        todo = [(NTB - 2, 1 - slot, c) for c in range(TB // RC)]
        for r0, r1, every in ((0, 192, 1), (192, 256, 2)):
            for j in range(D // 128):
                if j % every == 0:
                    router(*todo.pop(0))
                cols = slice(j * 128, (j + 1) * 128)
                y_s[slot, r0:r1, cols] = jnp.dot(_unpack(xn0[r0 // 2:r1 // 2, :]), wo[:, cols],
                                                 preferred_element_type=F32)
            todo += [(NTB - 1, slot, c) for c in range(r0 // RC, r1 // RC)]
        for t in todo:
            router(*t)

    def attn_first():
        store_q(NTB - 1, NG - 1, q7_s[...])
        for g in range(-1, NG):
            if g + 1 < NG:
                scores(0, g + 1, 1, 2 + (g + 1) % 2)
                scores(1, g + 1, 2, (g + 1) % 2)
            else:
                scores(2, 0, 3, 0)
            if g >= 0:
                softmax_pv(0, g, 1, 2 + g % 2, 0)
                softmax_pv(1, g, 2, g % 2, 1)

    def attn_pair(i, nks, nxt):
        for odd in range(2):
            qb = 2 * i + odd
            for g in range(NG):
                if g + 1 < NG:
                    scores(qb, g + 1, nks[odd], (g + 1) % 2)
                elif odd:
                    scores(nxt, 0, 3, 0)
                else:
                    scores(qb + 1, 0, nks[1], 0)
                if nks[0] == 3 and g == 0 and not odd:
                    out_proj(i % 2, jnp.where(i >= 2, i - 2, NTB))
                softmax_pv(qb, g, nks[odd], g % 2, odd)

    def ffn(l, first, last):
        best = best_s[...]
        rmax = jnp.max(best, axis=0, keepdims=True)
        idx = jnp.min(jnp.where(best == rmax, arg_s[...], S - 1))
        idx = jnp.clip(idx, 0, S - 1)

        @pl.when(first)
        def _():
            for c in ffn_copies():
                c.wait()

        xs = jnp.broadcast_to(n_s[pl.ds(idx, 1), :], (16, D)).astype(BF)
        hs = []
        for j in range(F // 128):
            gj = jnp.dot(xs, wg[j], preferred_element_type=F32)
            uj = jnp.dot(xs, wu[j], preferred_element_type=F32)
            hs.append((gj * jax.nn.sigmoid(gj) * uj).astype(BF))
            if j % 3 == 0 and j < 24:
                ln_terms(l // 2, j // 3)
        hid = jnp.concatenate(hs, axis=1)
        y = jnp.concatenate(
            [jnp.dot(hid, wd[j], preferred_element_type=F32) for j in range(D // 128)], axis=1)
        y = y * jax.nn.sigmoid(rmax[:, 0:1])

        @pl.when(last)
        def _():
            for i in range(NTB):
                out_copy(i).wait()

        rows = _rows(idx // 16, 16)
        x = x_s[rows, :].astype(F32)
        sel = lax.broadcasted_iota(I32, (16, D), 0) == idx % 16
        x_s[rows, :] = jnp.where(sel, x + y, x).astype(BF)

        @pl.when(first & (idx < TB))
        def _():
            ln_terms(0, idx // 16 % 8, False)

        @pl.when(last)
        def _():
            fix = pltpu.make_async_copy(x_s.at[rows], out_hbm.at[0, rows], o_sem.at[0])
            fix.start()
            fix.wait()

    x_copy(0).start()
    wqkv_copy(0).start()
    wqkv_copy(1).start()
    x_s[_rows(NTB, TB), :] = jnp.zeros((TB, D), BF)
    y_s[0] = jnp.zeros((TB, D), F32)
    best_s[...] = jnp.zeros((8, 128), F32)
    arg_s[...] = jnp.zeros((8, 128), I32)
    x_copy(0).wait()
    wqkv_copy(2).start()

    def ln_body(k, c):
        for t in range(4):
            ln_terms(0, 4 * k + t, False)
        return c
    lax.fori_loop(0, 2, ln_body, 0)
    wqkv_copy(3).start()
    qkv_block(0, 1, True)

    def layer(l, carry):
        first = l == 0
        last = l == 1

        def qkv_body(i, c):
            @pl.when(first & (i == 1))
            def _():
                x_copy(2).wait()
                for cp in wo_copies(0):
                    cp.wait()
                for cp in late_copies():
                    cp.start()

            @pl.when(first & (i == 2))
            def _():
                for cp in late_copies():
                    cp.wait()
                for cp in ffn_copies():
                    cp.start()
            qkv_block(i, (i + 1) % NTB)
            return c
        lax.fori_loop(1 - l, NTB, qkv_body, 0)

        attn_first()

        def attn_body(i, c):
            @pl.when(last & (i > 2))
            def _():
                out_copy(i - 3).start()
            attn_pair(i, (3, 3), jnp.minimum(2 * i + 2, NQB - 1))
            return c
        lax.fori_loop(1, NTB, attn_body, 0)

        out_tail(l // 2)

        @pl.when(last)
        def _():
            for i in range(NTB - 3, NTB):
                out_copy(i).start()

        ffn(l, first, last)
        return carry

    lax.fori_loop(0, 2, layer, 0)


@jax.jit
def pallas_interleave_layers__sliding_block__moe_arch_mod__prompt_kernel(
    A_x: jax.Array,
    A_wqkv: jax.Array,
    A_wo: jax.Array,
    B_x: jax.Array,
    B_w_r: jax.Array,
    B_w_gate: jax.Array,
    B_w_up: jax.Array,
    B_w_down: jax.Array,
):
    del B_x
    hbm = pl.BlockSpec(memory_space=pl.ANY)
    return pl.pallas_call(
        _kernel,
        in_specs=[hbm, hbm, hbm, pl.BlockSpec(memory_space=pltpu.VMEM), hbm, hbm, hbm],
        out_specs=hbm,
        out_shape=jax.ShapeDtypeStruct((1, S, D), BF),
        scratch_shapes=[
            pltpu.VMEM((S + TB + 16, D), BF),
            pltpu.VMEM((S + TB, D), F32),
            pltpu.VMEM((TB // 2, D), I32),
            pltpu.VMEM((2, 7, QB // 2, D // 2), I32),
            pltpu.VMEM((NNC // 2, D, 2 * NC), BF),
            pltpu.VMEM((NNC, 7, D // 4, 128), I32),
            pltpu.VMEM((D, D), BF),
            pltpu.VMEM((7, D // 4, D // 2), I32),
            pltpu.VMEM((7, QB // 2, D // 2), I32),
            pltpu.VMEM((F // 128, D, 128), BF),
            pltpu.VMEM((F // 128, D, 128), BF),
            pltpu.VMEM((D // 128, F, 128), BF),
            pltpu.VMEM((4 * NG, S // 2, 128), I32),
            pltpu.VMEM((TB // 2, 128), I32),
            pltpu.VMEM((4 * NG, S // 2, 128), I32),
            pltpu.VMEM((NQB, D // 2, QB), I32),
            pltpu.VMEM((TB, D), F32),
            pltpu.VMEM((128, QB), F32),
            pltpu.VMEM((2, TB, D), F32),
            pltpu.VMEM((8, 128), F32),
            pltpu.VMEM((8, 128), I32),
            pltpu.VMEM((4, 4, 2 * QB, QB), F32),
            pltpu.VMEM((4, 4, 8, QB), F32),
            pltpu.SemaphoreType.DMA((NTB,)),
            pltpu.SemaphoreType.DMA((NNC // 2 + 5,)),
            pltpu.SemaphoreType.DMA((NTB,)),
        ],
        compiler_params=pltpu.CompilerParams(vmem_limit_bytes=112 * 1024 * 1024),
        name="mod_swa",
    )(A_x, A_wqkv, A_wo, B_w_r, B_w_gate, B_w_up, B_w_down)
```

```python
import math

import jax
import jax.numpy as jnp
from jax import lax
import jax.experimental.pallas as pl
import jax.experimental.pallas.tpu as pltpu

S = 2048
D = 1024
DH = 32
F = 3584
TB = 256
NTB = S // TB
QB = 128
NQB = S // QB
NG = D // 128
NC = 256
NNC = 3 * D // NC
CHUNKS = [4, 5, 6, 7, 8, 9, 10, 11, 0, 1, 2, 3]
RC = 32
SUB = 32
EPS = 1e-5
QSCALE = (DH ** -0.5) * math.log2(math.e)

BF = jnp.bfloat16
F32 = jnp.float32
I32 = jnp.int32
NT = (((1,), (1,)), ((), ()))


def _pack(v):
    return pltpu.bitcast(v.astype(BF), I32)


def _unpack(v):
    return pltpu.bitcast(v, BF)


def _round(v):
    return v.astype(BF).astype(F32)


def _layernorm(x):
    m = jnp.sum(x, axis=-1, keepdims=True) * (1.0 / D)
    xc = x - m
    v = jnp.sum(xc * xc, axis=-1, keepdims=True) * (1.0 / D)
    sd = _round(jnp.sqrt(_round(_round(v) + EPS)))
    return xc * (1.0 / sd)


def _lhs_terms(top, bot):
    a11, a12, a21, a22 = top[:, :D // 2], top[:, D // 2:], bot[:, :D // 2], bot[:, D // 2:]
    return [a11, a11 + a12, a22, a21 + a22, a11 + a22, a12 - a22, a21 - a11]


def _rhs_term(t, b):
    first, sign, second = (((0, 1), -1, (1, 1)), ((1, 1), 0, None), ((1, 0), -1, (0, 0)),
                           ((0, 0), 0, None), ((0, 0), 1, (1, 1)), ((1, 0), 1, (1, 1)),
                           ((0, 0), 1, (0, 1)))[t]
    if sign == 0:
        return pltpu.bitcast(b(*first), I32)
    u, v = b(*first).astype(F32), b(*second).astype(F32)
    return _pack(u + v if sign > 0 else u - v)


STRASSEN_USES = (((0, 1, 1), (1, 1, 1)), ((0, 1, 1), (0, 0, -1)), ((0, 0, 1), (1, 0, 1)),
                 ((1, 0, 1), (1, 1, -1)), ((0, 0, 1), (1, 1, 1)), ((0, 0, 1),), ((1, 1, 1),))


def _strassen(product):
    m3, m5 = product(0), product(1)
    c12 = m3 + m5
    m4 = product(2)
    c11 = m4 - m5
    m2 = product(3)
    c21 = m2 + m4
    c22 = m3 - m2
    m1 = product(4)
    c11, c22 = c11 + m1, c22 + m1
    c11 = c11 + product(5)
    c22 = c22 + product(6)
    return [[c11, c12], [c21, c22]]


def _rows(i, n):
    return pl.ds(i * n if isinstance(i, int) else pl.multiple_of(i * n, n), n)


def _kernel(x_hbm, wqkv_hbm, wo_hbm, wr_ref, wg_hbm, wu_hbm, wd_hbm, out_hbm,
            x_s, n_s, xn0, xn, wqkv, wqkv7, wo, wo7, wg, wu, wd, q_s, q7_s, k_s, vt_s, o_s, ot_s, y_s, best_s, arg_s,
            s_s, m_s,
            x_sem, w_sem, o_sem):

    def x_copy(i):
        return pltpu.make_async_copy(x_hbm.at[0, _rows(i, TB)], x_s.at[_rows(i, TB)],
                                     x_sem.at[i])

    def out_copy(i):
        return pltpu.make_async_copy(x_s.at[_rows(i, TB)], out_hbm.at[0, _rows(i, TB)],
                                     o_sem.at[i])

    def wqkv_copy(jj):
        j = CHUNKS[jj] // 2
        rows = pl.ds(jj % 2 * D // 2, D // 2)
        return pltpu.make_async_copy(
            wqkv_hbm.at[rows, pl.ds(j * 2 * NC, 2 * NC)], wqkv.at[j, rows], w_sem.at[j])

    def wo_copies(k):
        return [pltpu.make_async_copy(wo_hbm.at[_rows(k + 4 * h, D // 8)],
                                      wo.at[_rows(k + 4 * h, D // 8)], w_sem.at[NNC // 2 + 1 + k])
                for h in range(2)]

    def late_copies():
        return [x_copy(b) for b in range(3, NTB)] + sum((wo_copies(k) for k in range(1, 4)), [])

    def ffn_copies():
        cs = []
        for j in range(F // 128):
            cs.append(pltpu.make_async_copy(
                wg_hbm.at[:, pl.ds(j * 128, 128)], wg.at[j], w_sem.at[NNC // 2]))
            cs.append(pltpu.make_async_copy(
                wu_hbm.at[:, pl.ds(j * 128, 128)], wu.at[j], w_sem.at[NNC // 2]))
        for j in range(D // 128):
            cs.append(pltpu.make_async_copy(
                wd_hbm.at[:, pl.ds(j * 128, 128)], wd.at[j], w_sem.at[NNC // 2]))
        return cs

    def ln_terms(i, c, chain=True):
        top, bot = [_layernorm(x_s[_rows(i * (TB // 16) + h * (TB // 32) + c, 16), :].astype(F32))
                    for h in range(2)]
        for t, a in enumerate(_lhs_terms(top, bot)):
            xn[0, t, _rows(c, 8), :] = _pack(a)
        if chain:
            x_s[S + TB:, :128] = (top[:, :128] + bot[:, :128]).astype(BF)

    def wo_terms(c):
        for t in range(7):
            wo7[t, _rows(c, 8), :] = _rhs_term(
                t, lambda i, j: wo[_rows(c + i * (D // 32), 16), _rows(j, D // 2)])

    def lane_group(n):
        return lax.broadcasted_iota(I32, (n, 128), 1) // DH

    def store_q(i, g, q):
        grp = lane_group(SUB // 2)
        rolled = [q] + [pltpu.roll(q, DH * t, 1) for t in range(1, 4)]
        for h in range(4):
            parts = []
            for c in range(TB // SUB):
                b = c % 4
                rows = slice(c * SUB // 2, (c + 1) * SUB // 2)
                parts.append(jnp.where(grp == b, rolled[(b - h) % 4][rows], 0))
            q_s[g * 4 + h, _rows(i, TB // 2), :] = jnp.concatenate(parts, axis=0)

    def store_k(i, g, k):
        grp = lane_group(TB // 2)
        even = grp % 2 == 0
        low = grp < 2
        pairs = [jnp.where(even, k, pltpu.roll(k, DH, 1)),
                 jnp.where(even, pltpu.roll(k, 3 * DH, 1), k)]
        for h in range(2):
            swapped = pltpu.roll(pairs[h], 2 * DH, 1)
            k_s[g * 4 + h, _rows(i, TB // 2), :] = jnp.where(low, pairs[h], swapped)
            k_s[g * 4 + h + 2, _rows(i, TB // 2), :] = jnp.where(low, swapped, pairs[h])

    def store_qkv(i, col, y):
        kind, g = divmod(col // 128, NG)
        if kind == 0 and g == NG - 1:
            q7_s[...] = _pack(y * QSCALE)
        elif kind == 0:
            store_q(i, g, _pack(y * QSCALE))
        elif kind == 1:
            store_k(i, g, _pack(y))
        else:
            for t in range(TB // QB):
                vt_s[i * (TB // QB) + t, g * 64:(g + 1) * 64, :] = _pack(y[t * QB:(t + 1) * QB].T)

    def qkv_block(i, nxt, startup=False):
        if not startup:
            store_q((i + NTB - 1) % NTB, NG - 1, q7_s[...])
        for jj, j in enumerate(CHUNKS):
            if startup and jj % 2 == 0:
                wqkv_copy(jj).wait()
                wqkv_copy(jj + 1).wait()
                for u in range(jj + 4, min(jj + 6, NNC)):
                    wqkv_copy(u).start()
                if jj == 2:
                    x_copy(1).start()
                if jj == 4:
                    x_copy(1).wait()
                if jj == NNC - 4:
                    x_copy(2).start()
                    for c in wo_copies(0):
                        c.start()

            def product(t):
                if startup:
                    w = _rhs_term(t, lambda r, c: wqkv[j // 2, _rows(r, D // 2),
                                                       _rows(2 * c + j % 2, 128)])
                    wqkv7[j, t] = w
                else:
                    w = wqkv7[j, t]
                return jnp.dot(_unpack(xn[min(jj // 2, 1), t]), _unpack(w),
                               preferred_element_type=F32)

            y = _strassen(product)
            if jj == 1:
                xn[1] = xn[0]
            for c in range(2):
                store_qkv(i, j // 2 * 2 * NC + c * NC + j % 2 * 128,
                          jnp.concatenate([y[0][c], y[1][c]], axis=0))
            if startup:
                if jj >= 4:
                    ln_terms(nxt, jj - 4)
            elif 2 <= jj < 10:
                ln_terms(nxt, jj - 2)
                wo_terms((i + 3) % 4 * 8 + jj - 2)

    def tri():
        kk = lax.broadcasted_iota(I32, (QB, QB), 0)
        qq = lax.broadcasted_iota(I32, (QB, QB), 1)
        return kk <= qq

    def scores(qb, g, nk, slot):
        kk = lax.broadcasted_iota(I32, (QB, QB), 0)
        qq = lax.broadcasted_iota(I32, (QB, QB), 1)
        grp = lane_group(SUB // 2)
        n = SUB // 2
        for h in range(4):
            hd = g * 4 + h
            tiles = [k_s[hd, _rows(qb - b, QB // 2), :] for b in range(nk)]
            if nk == 3:
                new, mid, old = tiles
                diag = jnp.where(grp >= 2,
                                 jnp.where(grp >= 3, old[3 * n:], old[2 * n:3 * n]),
                                 jnp.where(grp >= 1, old[n:2 * n], old[:n]))
                lhs = [diag, new[:n]] + [
                    jnp.where(grp >= c, new[c * n:(c + 1) * n], old[c * n:(c + 1) * n])
                    for c in range(1, 4)] + [mid]
            else:
                lhs = tiles
            st = lax.dot_general(_unpack(jnp.concatenate(lhs, axis=0)),
                                 _unpack(q_s[hd, _rows(qb, QB // 2), :]), NT,
                                 preferred_element_type=F32)
            if nk == 3:
                t = jnp.where((kk > qq) & (kk // SUB == qq // SUB),
                              jnp.concatenate([st[:SUB]] * 4, axis=0), st[SUB:SUB + QB])
                st = st[SUB:]
            else:
                t = jnp.where(kk <= qq, st[:QB], -1e30)
            s_s[slot, h, 0:QB, :] = t
            if nk >= 2:
                s_s[slot, h, QB:2 * QB, :] = st[QB:]
                t = jnp.maximum(t, st[QB:])
            m_s[slot, h] = jnp.max(t.reshape(QB // 8, 8, QB), axis=0)

    def softmax_pv(qb, g, nk, slot, odd):
        newest = tri()
        outs = []
        for h in range(4):
            m = jnp.max(m_s[slot, h], axis=0, keepdims=True)
            p0 = jnp.exp2(s_s[slot, h, 0:QB, :] - m)
            p1 = jnp.exp2(s_s[slot, h, QB:2 * QB, :] - m) if nk >= 2 else None
            if nk == 3:
                pt = [jnp.where(newest, p0, 0.0), jnp.where(newest, 0.0, p0)]
                backs = [0, 2]
            else:
                pt, backs = [p0], [0]
            if nk >= 2:
                pt, backs = pt + [p1], backs + [1]
            l = sum(jnp.sum(p.reshape(16, 8, QB), axis=0) for p in (p0, p1) if p is not None)
            l = jnp.sum(l, axis=0, keepdims=True)
            r0 = (g * 4 + h) * (DH // 2)
            vt = jnp.concatenate([vt_s[qb - b, r0:r0 + DH // 2, :] for b in backs], axis=1)
            ot = jnp.dot(_unpack(vt), jnp.concatenate(pt, axis=0).astype(BF),
                         preferred_element_type=F32)
            outs.append(ot * (1.0 / l))
        ot = jnp.concatenate(outs, axis=0)
        if odd and g + 1 == NG:
            ot_s[...] = ot
        else:
            o_s[_rows(odd, QB), g * 128:(g + 1) * 128] = ot.T

    def router(i, slot, c):
        wr = wr_ref[...].astype(F32).reshape(1, D)
        tok = lax.broadcasted_iota(I32, (8, 128), 0) + i * TB
        best, arg = best_s[...], arg_s[...]
        rows = _rows(i * (TB // RC) + c, RC)
        x1 = x_s[rows, :].astype(F32) + y_s[slot, c * RC:(c + 1) * RC, :]
        xn1 = _layernorm(x1)
        n_s[rows, :] = xn1
        r = jnp.broadcast_to(jnp.sum(xn1 * wr, axis=-1, keepdims=True), (RC, 128))
        x_s[rows, :] = (x1 + xn1).astype(BF)
        for t in range(RC // 8):
            rt = r[t * 8:(t + 1) * 8]
            arg = jnp.where(rt > best, tok + (c * RC + t * 8), arg)
            best = jnp.where(rt > best, rt, best)
        best_s[...] = jnp.where(i < NTB, best, -jnp.inf)
        arg_s[...] = arg

    def out_proj(slot, prev):
        o_s[QB:, D - 128:] = ot_s[...].T
        router(prev, 1 - slot, 0)
        seen = set()
        for t, uses in enumerate(STRASSEN_USES):
            a = _lhs_terms(o_s[:QB, :], o_s[QB:, :])[t]
            m = jnp.dot(a.astype(BF), _unpack(wo7[t]), preferred_element_type=F32)
            for r, c, sign in uses:
                at = (slot, _rows(r, QB), _rows(c, D // 2))
                if (r, c) in seen:
                    y_s[at] = y_s[at] + m if sign > 0 else y_s[at] - m
                else:
                    y_s[at] = m if sign > 0 else -m
                seen.add((r, c))
            router(prev, 1 - slot, t + 1)

    def out_tail(slot):
        o_s[QB:, D - 128:] = ot_s[...].T
        xn0[...] = _pack(o_s[...])
        todo = [(NTB - 2, 1 - slot, c) for c in range(TB // RC)]
        for r0, r1, every in ((0, 192, 1), (192, 256, 2)):
            for j in range(D // 128):
                if j % every == 0:
                    router(*todo.pop(0))
                cols = slice(j * 128, (j + 1) * 128)
                y_s[slot, r0:r1, cols] = jnp.dot(_unpack(xn0[r0 // 2:r1 // 2, :]), wo[:, cols],
                                                 preferred_element_type=F32)
            todo += [(NTB - 1, slot, c) for c in range(r0 // RC, r1 // RC)]
        for t in todo:
            router(*t)

    def attn_first():
        store_q(NTB - 1, NG - 1, q7_s[...])
        for g in range(-1, NG):
            if g + 1 < NG:
                scores(0, g + 1, 1, 2 + (g + 1) % 2)
                scores(1, g + 1, 2, (g + 1) % 2)
            else:
                scores(2, 0, 3, 0)
            if g >= 0:
                softmax_pv(0, g, 1, 2 + g % 2, 0)
                softmax_pv(1, g, 2, g % 2, 1)

    def attn_pair(i, nxt):
        for odd in range(2):
            qb = 2 * i + odd
            for g in range(NG):
                if g + 1 < NG:
                    scores(qb, g + 1, 3, (g + 1) % 2)
                else:
                    scores(nxt if odd else qb + 1, 0, 3, 0)
                if g == 0 and not odd:
                    out_proj(i % 2, jnp.where(i >= 2, i - 2, NTB))
                softmax_pv(qb, g, 3, g % 2, odd)

    def ffn(l, first, last):
        best = best_s[...]
        rmax = jnp.max(best, axis=0, keepdims=True)
        idx = jnp.min(jnp.where(best == rmax, arg_s[...], S - 1))
        idx = jnp.clip(idx, 0, S - 1)

        @pl.when(first)
        def _():
            for c in ffn_copies():
                c.wait()

        xs = jnp.broadcast_to(n_s[pl.ds(idx, 1), :], (16, D)).astype(BF)
        hs = []
        for j in range(F // 128):
            gj = jnp.dot(xs, wg[j], preferred_element_type=F32)
            uj = jnp.dot(xs, wu[j], preferred_element_type=F32)
            hs.append((gj * jax.nn.sigmoid(gj) * uj).astype(BF))
            if j % 3 == 0 and j < 24:
                ln_terms(l // 2, j // 3)
        hid = jnp.concatenate(hs, axis=1)
        y = jnp.concatenate(
            [jnp.dot(hid, wd[j], preferred_element_type=F32) for j in range(D // 128)], axis=1)
        y = y * jax.nn.sigmoid(rmax[:, 0:1])

        @pl.when(last)
        def _():
            for i in range(NTB):
                out_copy(i).wait()

        rows = _rows(idx // 16, 16)
        x = x_s[rows, :].astype(F32)
        sel = lax.broadcasted_iota(I32, (16, D), 0) == idx % 16
        x_s[rows, :] = jnp.where(sel, x + y, x).astype(BF)

        @pl.when(first & (idx < TB))
        def _():
            ln_terms(0, idx // 16 % 8, False)

        @pl.when(last)
        def _():
            fix = pltpu.make_async_copy(x_s.at[rows], out_hbm.at[0, rows], o_sem.at[0])
            fix.start()
            fix.wait()

    x_copy(0).start()
    wqkv_copy(0).start()
    wqkv_copy(1).start()
    x_s[_rows(NTB, TB), :] = jnp.zeros((TB, D), BF)
    y_s[0] = jnp.zeros((TB, D), F32)
    best_s[...] = jnp.zeros((8, 128), F32)
    arg_s[...] = jnp.zeros((8, 128), I32)
    x_copy(0).wait()
    wqkv_copy(2).start()

    def ln_body(k, c):
        for t in range(4):
            ln_terms(0, 4 * k + t, False)
        return c
    lax.fori_loop(0, 2, ln_body, 0)
    wqkv_copy(3).start()
    qkv_block(0, 1, True)

    def layer(l, carry):
        first = l == 0
        last = l == 1

        def qkv_body(i, c):
            @pl.when(first & (i == 1))
            def _():
                x_copy(2).wait()
                for cp in wo_copies(0):
                    cp.wait()
                for cp in late_copies():
                    cp.start()

            @pl.when(first & (i == 2))
            def _():
                for cp in late_copies():
                    cp.wait()
                for cp in ffn_copies():
                    cp.start()
            qkv_block(i, (i + 1) % NTB)
            return c
        lax.fori_loop(1 - l, NTB, qkv_body, 0)

        attn_first()

        def attn_body(i, c):
            @pl.when(last & (i > 2))
            def _():
                out_copy(i - 3).start()
            attn_pair(i, jnp.minimum(2 * i + 2, NQB - 1))
            return c
        lax.fori_loop(1, NTB, attn_body, 0)

        out_tail(l // 2)

        @pl.when(last)
        def _():
            for i in range(NTB - 3, NTB):
                out_copy(i).start()

        ffn(l, first, last)
        return carry

    lax.fori_loop(0, 2, layer, 0)


@jax.jit
def pallas_interleave_layers__sliding_block__moe_arch_mod__prompt_kernel(
    A_x: jax.Array,
    A_wqkv: jax.Array,
    A_wo: jax.Array,
    B_x: jax.Array,
    B_w_r: jax.Array,
    B_w_gate: jax.Array,
    B_w_up: jax.Array,
    B_w_down: jax.Array,
):
    del B_x
    hbm = pl.BlockSpec(memory_space=pl.ANY)
    return pl.pallas_call(
        _kernel,
        in_specs=[hbm, hbm, hbm, pl.BlockSpec(memory_space=pltpu.VMEM), hbm, hbm, hbm],
        out_specs=hbm,
        out_shape=jax.ShapeDtypeStruct((1, S, D), BF),
        scratch_shapes=[
            pltpu.VMEM((S + TB + 16, D), BF),
            pltpu.VMEM((S + TB, D), F32),
            pltpu.VMEM((TB // 2, D), I32),
            pltpu.VMEM((2, 7, QB // 2, D // 2), I32),
            pltpu.VMEM((NNC // 2, D, 2 * NC), BF),
            pltpu.VMEM((NNC, 7, D // 4, 128), I32),
            pltpu.VMEM((D, D), BF),
            pltpu.VMEM((7, D // 4, D // 2), I32),
            pltpu.VMEM((F // 128, D, 128), BF),
            pltpu.VMEM((F // 128, D, 128), BF),
            pltpu.VMEM((D // 128, F, 128), BF),
            pltpu.VMEM((4 * NG, S // 2, 128), I32),
            pltpu.VMEM((TB // 2, 128), I32),
            pltpu.VMEM((4 * NG, S // 2, 128), I32),
            pltpu.VMEM((NQB, D // 2, QB), I32),
            pltpu.VMEM((TB, D), F32),
            pltpu.VMEM((128, QB), F32),
            pltpu.VMEM((2, TB, D), F32),
            pltpu.VMEM((8, 128), F32),
            pltpu.VMEM((8, 128), I32),
            pltpu.VMEM((4, 4, 2 * QB, QB), F32),
            pltpu.VMEM((4, 4, 8, QB), F32),
            pltpu.SemaphoreType.DMA((NTB,)),
            pltpu.SemaphoreType.DMA((NNC // 2 + 5,)),
            pltpu.SemaphoreType.DMA((NTB,)),
        ],
        compiler_params=pltpu.CompilerParams(vmem_limit_bytes=112 * 1024 * 1024),
        name="mod_swa",
    )(A_x, A_wqkv, A_wo, B_w_r, B_w_gate, B_w_up, B_w_down)
```

```python
import math

import jax
import jax.numpy as jnp
from jax import lax
import jax.experimental.pallas as pl
import jax.experimental.pallas.tpu as pltpu

S = 2048
D = 1024
DH = 32
F = 3584
TB = 256
NTB = S // TB
QB = 128
NQB = S // QB
NG = D // 128
NC = 256
NNC = 3 * D // NC
CHUNKS = [4, 5, 6, 7, 8, 9, 10, 11, 0, 1, 2, 3]
RC = 32
SUB = 32
EPS = 1e-5
QSCALE = (DH ** -0.5) * math.log2(math.e)

BF = jnp.bfloat16
F32 = jnp.float32
I32 = jnp.int32
NT = (((1,), (1,)), ((), ()))


def _pack(v):
    return pltpu.bitcast(v.astype(BF), I32)


def _unpack(v):
    return pltpu.bitcast(v, BF)


def _round(v):
    return v.astype(BF).astype(F32)


def _layernorm(x):
    m = jnp.sum(x, axis=-1, keepdims=True) * (1.0 / D)
    xc = x - m
    v = jnp.sum(xc * xc, axis=-1, keepdims=True) * (1.0 / D)
    sd = _round(jnp.sqrt(_round(_round(v) + EPS)))
    return xc * (1.0 / sd)


def _lhs_terms(top, bot):
    a11, a12, a21, a22 = top[:, :D // 2], top[:, D // 2:], bot[:, :D // 2], bot[:, D // 2:]
    return [a11, a11 + a12, a22, a21 + a22, a11 + a22, a12 - a22, a21 - a11]


def _rhs_term(t, b):
    first, sign, second = (((0, 1), -1, (1, 1)), ((1, 1), 0, None), ((1, 0), -1, (0, 0)),
                           ((0, 0), 0, None), ((0, 0), 1, (1, 1)), ((1, 0), 1, (1, 1)),
                           ((0, 0), 1, (0, 1)))[t]
    if sign == 0:
        return pltpu.bitcast(b(*first), I32)
    u, v = b(*first).astype(F32), b(*second).astype(F32)
    return _pack(u + v if sign > 0 else u - v)


STRASSEN_USES = (((0, 1, 1), (1, 1, 1)), ((0, 1, 1), (0, 0, -1)), ((0, 0, 1), (1, 0, 1)),
                 ((1, 0, 1), (1, 1, -1)), ((0, 0, 1), (1, 1, 1)), ((0, 0, 1),), ((1, 1, 1),))


def _strassen(product):
    m3, m5 = product(0), product(1)
    c12 = m3 + m5
    m4 = product(2)
    c11 = m4 - m5
    m2 = product(3)
    c21 = m2 + m4
    c22 = m3 - m2
    m1 = product(4)
    c11, c22 = c11 + m1, c22 + m1
    c11 = c11 + product(5)
    c22 = c22 + product(6)
    return [[c11, c12], [c21, c22]]


def _rows(i, n):
    return pl.ds(i * n if isinstance(i, int) else pl.multiple_of(i * n, n), n)


def _kernel(x_hbm, wqkv_hbm, wo_hbm, wr_ref, wg_hbm, wu_hbm, wd_hbm, out_hbm,
            x_s, n_s, xn0, xn, wqkv, wqkv7, wo, wo7, wg, wu, wd, q_s, q7_s, k_s, vt_s, o_s, ot_s, y_s, best_s, arg_s,
            s_s, m_s,
            x_sem, w_sem, o_sem):

    def x_copy(i):
        return pltpu.make_async_copy(x_hbm.at[0, _rows(i, TB)], x_s.at[_rows(i, TB)],
                                     x_sem.at[i])

    def out_copy(i):
        return pltpu.make_async_copy(x_s.at[_rows(i, TB)], out_hbm.at[0, _rows(i, TB)],
                                     o_sem.at[i])

    def wqkv_copy(jj):
        j = CHUNKS[jj] // 2
        rows = pl.ds(jj % 2 * D // 2, D // 2)
        return pltpu.make_async_copy(
            wqkv_hbm.at[rows, pl.ds(j * 2 * NC, 2 * NC)], wqkv.at[j, rows], w_sem.at[j])

    def wo_copies(k):
        return [pltpu.make_async_copy(wo_hbm.at[_rows(k + 4 * h, D // 8)],
                                      wo.at[_rows(k + 4 * h, D // 8)], w_sem.at[NNC // 2 + 1 + k])
                for h in range(2)]

    def late_copies():
        return [x_copy(b) for b in range(3, NTB)] + sum((wo_copies(k) for k in range(1, 4)), [])

    def ffn_copies():
        cs = []
        for j in range(F // 128):
            cs.append(pltpu.make_async_copy(
                wg_hbm.at[:, pl.ds(j * 128, 128)], wg.at[j], w_sem.at[NNC // 2]))
            cs.append(pltpu.make_async_copy(
                wu_hbm.at[:, pl.ds(j * 128, 128)], wu.at[j], w_sem.at[NNC // 2]))
        for j in range(D // 128):
            cs.append(pltpu.make_async_copy(
                wd_hbm.at[:, pl.ds(j * 128, 128)], wd.at[j], w_sem.at[NNC // 2]))
        return cs

    def ln_terms(i, c, chain=True):
        top, bot = [_layernorm(x_s[_rows(i * (TB // 16) + h * (TB // 32) + c, 16), :].astype(F32))
                    for h in range(2)]
        for t, a in enumerate(_lhs_terms(top, bot)):
            xn[0, t, _rows(c, 8), :] = _pack(a)
        if chain:
            x_s[S + TB:, :128] = (top[:, :128] + bot[:, :128]).astype(BF)

    def wo_terms(c):
        for t in range(7):
            wo7[t, _rows(c, 8), :] = _rhs_term(
                t, lambda i, j: wo[_rows(c + i * (D // 32), 16), _rows(j, D // 2)])

    def lane_group(n):
        return lax.broadcasted_iota(I32, (n, 128), 1) // DH

    def store_q(i, g, q):
        grp = lane_group(SUB // 2)
        rolled = [q] + [pltpu.roll(q, DH * t, 1) for t in range(1, 4)]
        for h in range(4):
            parts = []
            for c in range(TB // SUB):
                b = c % 4
                rows = slice(c * SUB // 2, (c + 1) * SUB // 2)
                parts.append(jnp.where(grp == b, rolled[(b - h) % 4][rows], 0))
            q_s[g * 4 + h, _rows(i, TB // 2), :] = jnp.concatenate(parts, axis=0)

    def store_k(i, g, k):
        grp = lane_group(TB // 2)
        even = grp % 2 == 0
        low = grp < 2
        pairs = [jnp.where(even, k, pltpu.roll(k, DH, 1)),
                 jnp.where(even, pltpu.roll(k, 3 * DH, 1), k)]
        for h in range(2):
            swapped = pltpu.roll(pairs[h], 2 * DH, 1)
            k_s[g * 4 + h, _rows(i, TB // 2), :] = jnp.where(low, pairs[h], swapped)
            k_s[g * 4 + h + 2, _rows(i, TB // 2), :] = jnp.where(low, swapped, pairs[h])

    def store_qkv(i, col, y):
        kind, g = divmod(col // 128, NG)
        if kind == 0 and g == NG - 1:
            q7_s[...] = _pack(y * QSCALE)
        elif kind == 0:
            store_q(i, g, _pack(y * QSCALE))
        elif kind == 1:
            store_k(i, g, _pack(y))
        else:
            for t in range(TB // QB):
                vt_s[i * (TB // QB) + t, g * 64:(g + 1) * 64, :] = _pack(y[t * QB:(t + 1) * QB].T)

    def qkv_block(i, nxt, startup=False):
        if not startup:
            store_q((i + NTB - 1) % NTB, NG - 1, q7_s[...])
        for jj, j in enumerate(CHUNKS):
            if startup and jj % 2 == 0:
                wqkv_copy(jj).wait()
                wqkv_copy(jj + 1).wait()
                for u in range(jj + 4, min(jj + 6, NNC)):
                    wqkv_copy(u).start()
                if jj == 2:
                    x_copy(1).start()
                if jj == 4:
                    x_copy(1).wait()
                if jj == NNC - 4:
                    x_copy(2).start()
                    for c in wo_copies(0):
                        c.start()

            def product(t):
                if startup:
                    w = _rhs_term(t, lambda r, c: wqkv[j // 2, _rows(r, D // 2),
                                                       _rows(2 * c + j % 2, 128)])
                    wqkv7[j, t] = w
                else:
                    w = wqkv7[j, t]
                return jnp.dot(_unpack(xn[min(jj // 2, 1), t]), _unpack(w),
                               preferred_element_type=F32)

            y = _strassen(product)
            if jj == 1:
                xn[1] = xn[0]
            for c in range(2):
                store_qkv(i, j // 2 * 2 * NC + c * NC + j % 2 * 128,
                          jnp.concatenate([y[0][c], y[1][c]], axis=0))
            if startup:
                if jj >= 4:
                    ln_terms(nxt, jj - 4)
            elif 2 <= jj < 10:
                ln_terms(nxt, jj - 2)
                wo_terms((i + 3) % 4 * 8 + jj - 2)

    def tri():
        kk = lax.broadcasted_iota(I32, (QB, QB), 0)
        qq = lax.broadcasted_iota(I32, (QB, QB), 1)
        return kk <= qq

    def scores(qb, g, nk, slot):
        kk = lax.broadcasted_iota(I32, (QB, QB), 0)
        qq = lax.broadcasted_iota(I32, (QB, QB), 1)
        grp = lane_group(SUB // 2)
        n = SUB // 2
        for h in range(4):
            hd = g * 4 + h
            tiles = [k_s[hd, _rows(qb - b, QB // 2), :] for b in range(nk)]
            if nk == 3:
                new, mid, old = tiles
                diag = jnp.where(grp >= 2,
                                 jnp.where(grp >= 3, old[3 * n:], old[2 * n:3 * n]),
                                 jnp.where(grp >= 1, old[n:2 * n], old[:n]))
                lhs = [diag, new[:n]] + [
                    jnp.where(grp >= c, new[c * n:(c + 1) * n], old[c * n:(c + 1) * n])
                    for c in range(1, 4)] + [mid]
            else:
                lhs = tiles
            st = lax.dot_general(_unpack(jnp.concatenate(lhs, axis=0)),
                                 _unpack(q_s[hd, _rows(qb, QB // 2), :]), NT,
                                 preferred_element_type=F32)
            if nk == 3:
                t = jnp.where((kk > qq) & (kk // SUB == qq // SUB),
                              jnp.concatenate([st[:SUB]] * 4, axis=0), st[SUB:SUB + QB])
                st = st[SUB:]
            else:
                t = jnp.where(kk <= qq, st[:QB], -1e30)
            s_s[slot, h, 0:QB, :] = t
            if nk >= 2:
                s_s[slot, h, QB:2 * QB, :] = st[QB:]
                t = jnp.maximum(t, st[QB:])
            m_s[slot, h] = jnp.max(t.reshape(QB // 8, 8, QB), axis=0)

    def softmax_pv(qb, g, nk, slot, odd):
        newest = tri()
        outs = []
        for h in range(4):
            m = jnp.max(m_s[slot, h], axis=0, keepdims=True)
            p0 = jnp.exp2(s_s[slot, h, 0:QB, :] - m)
            p1 = jnp.exp2(s_s[slot, h, QB:2 * QB, :] - m) if nk >= 2 else None
            if nk == 3:
                pt = [jnp.where(newest, p0, 0.0), jnp.where(newest, 0.0, p0)]
                backs = [0, 2]
            else:
                pt, backs = [p0], [0]
            if nk >= 2:
                pt, backs = pt + [p1], backs + [1]
            l = sum(jnp.sum(p.reshape(16, 8, QB), axis=0) for p in (p0, p1) if p is not None)
            l = jnp.sum(l, axis=0, keepdims=True)
            r0 = (g * 4 + h) * (DH // 2)
            vt = jnp.concatenate([vt_s[qb - b, r0:r0 + DH // 2, :] for b in backs], axis=1)
            ot = jnp.dot(_unpack(vt), jnp.concatenate(pt, axis=0).astype(BF),
                         preferred_element_type=F32)
            outs.append(ot * (1.0 / l))
        ot = jnp.concatenate(outs, axis=0)
        if odd and g + 1 == NG:
            ot_s[...] = ot
        else:
            o_s[_rows(odd, QB), g * 128:(g + 1) * 128] = ot.T

    def router(i, slot, c):
        wr = wr_ref[...].astype(F32).reshape(1, D)
        tok = lax.broadcasted_iota(I32, (8, 128), 0) + i * TB
        best, arg = best_s[...], arg_s[...]
        rows = _rows(i * (TB // RC) + c, RC)
        x1 = x_s[rows, :].astype(F32) + y_s[slot, c * RC:(c + 1) * RC, :]
        xn1 = _layernorm(x1)
        n_s[rows, :] = xn1
        r = jnp.broadcast_to(jnp.sum(xn1 * wr, axis=-1, keepdims=True), (RC, 128))
        x_s[rows, :] = (x1 + xn1).astype(BF)
        for t in range(RC // 8):
            rt = r[t * 8:(t + 1) * 8]
            arg = jnp.where(rt > best, tok + (c * RC + t * 8), arg)
            best = jnp.where(rt > best, rt, best)
        best_s[...] = jnp.where(i < NTB, best, -jnp.inf)
        arg_s[...] = arg

    def out_proj(slot, prev):
        o_s[QB:, D - 128:] = ot_s[...].T
        router(prev, 1 - slot, 0)
        seen = set()
        for t, uses in enumerate(STRASSEN_USES):
            a = _lhs_terms(o_s[:QB, :], o_s[QB:, :])[t]
            m = jnp.dot(a.astype(BF), _unpack(wo7[t]), preferred_element_type=F32)
            for r, c, sign in uses:
                at = (slot, _rows(r, QB), _rows(c, D // 2))
                if (r, c) in seen:
                    y_s[at] = y_s[at] + m if sign > 0 else y_s[at] - m
                else:
                    y_s[at] = m if sign > 0 else -m
                seen.add((r, c))
            router(prev, 1 - slot, t + 1)

    def out_tail(slot):
        o_s[QB:, D - 128:] = ot_s[...].T
        xn0[...] = _pack(o_s[...])
        todo = [(NTB - 2, 1 - slot, c) for c in range(TB // RC)]
        for r0, r1, every in ((0, 192, 1), (192, 256, 2)):
            for j in range(D // 128):
                if j % every == 0:
                    router(*todo.pop(0))
                cols = slice(j * 128, (j + 1) * 128)
                y_s[slot, r0:r1, cols] = jnp.dot(_unpack(xn0[r0 // 2:r1 // 2, :]), wo[:, cols],
                                                 preferred_element_type=F32)
            todo += [(NTB - 1, slot, c) for c in range(r0 // RC, r1 // RC)]
        for t in todo:
            router(*t)

    def attn_first():
        store_q(NTB - 1, NG - 1, q7_s[...])
        for g in range(-1, NG):
            if g + 1 < NG:
                scores(0, g + 1, 1, 2 + (g + 1) % 2)
                scores(1, g + 1, 2, (g + 1) % 2)
            else:
                scores(2, 0, 3, 0)
            if g >= 0:
                softmax_pv(0, g, 1, 2 + g % 2, 0)
                softmax_pv(1, g, 2, g % 2, 1)

    def attn_pair(i, nxt):
        for odd in range(2):
            qb = 2 * i + odd
            for g in range(NG):
                if g + 1 < NG:
                    scores(qb, g + 1, 3, (g + 1) % 2)
                else:
                    scores(nxt if odd else qb + 1, 0, 3, 0)
                if g == 0 and not odd:
                    out_proj(i % 2, jnp.where(i >= 2, i - 2, NTB))
                softmax_pv(qb, g, 3, g % 2, odd)

    def ffn(l, first, last):
        best = best_s[...]
        rmax = jnp.max(best, axis=0, keepdims=True)
        idx = jnp.min(jnp.where(best == rmax, arg_s[...], S - 1))
        idx = jnp.clip(idx, 0, S - 1)

        @pl.when(first)
        def _():
            for c in ffn_copies():
                c.wait()

        xs = jnp.broadcast_to(n_s[pl.ds(idx, 1), :], (16, D)).astype(BF)
        hs = []
        for j in range(F // 128):
            gj = jnp.dot(xs, wg[j], preferred_element_type=F32)
            uj = jnp.dot(xs, wu[j], preferred_element_type=F32)
            hj = gj[:8] * jax.nn.sigmoid(gj[:8]) * uj[:8]
            hs.append(jnp.concatenate([hj, hj], axis=0).astype(BF))
            if j % 3 == 0 and j < 24:
                ln_terms(l // 2, j // 3)
        hid = jnp.concatenate(hs, axis=1)
        y = jnp.concatenate(
            [jnp.dot(hid, wd[j], preferred_element_type=F32) for j in range(D // 128)], axis=1)
        y = y * jax.nn.sigmoid(rmax[:, 0:1])

        @pl.when(last)
        def _():
            for i in range(NTB):
                out_copy(i).wait()

        rows = _rows(idx // 16, 16)
        x = x_s[rows, :].astype(F32)
        sel = lax.broadcasted_iota(I32, (16, D), 0) == idx % 16
        x_s[rows, :] = jnp.where(sel, x + y, x).astype(BF)

        @pl.when(first & (idx < TB))
        def _():
            ln_terms(0, idx // 16 % 8, False)

        @pl.when(last)
        def _():
            fix = pltpu.make_async_copy(x_s.at[rows], out_hbm.at[0, rows], o_sem.at[0])
            fix.start()
            fix.wait()

    x_copy(0).start()
    wqkv_copy(0).start()
    wqkv_copy(1).start()
    x_s[_rows(NTB, TB), :] = jnp.zeros((TB, D), BF)
    y_s[0] = jnp.zeros((TB, D), F32)
    best_s[...] = jnp.zeros((8, 128), F32)
    arg_s[...] = jnp.zeros((8, 128), I32)
    x_copy(0).wait()
    wqkv_copy(2).start()

    def ln_body(k, c):
        for t in range(4):
            ln_terms(0, 4 * k + t, False)
        return c
    lax.fori_loop(0, 2, ln_body, 0)
    wqkv_copy(3).start()
    qkv_block(0, 1, True)

    def layer(l, carry):
        first = l == 0
        last = l == 1

        def qkv_body(i, c):
            @pl.when(first & (i == 1))
            def _():
                x_copy(2).wait()
                for cp in wo_copies(0):
                    cp.wait()
                for cp in late_copies():
                    cp.start()

            @pl.when(first & (i == 2))
            def _():
                for cp in late_copies():
                    cp.wait()
                for cp in ffn_copies():
                    cp.start()
            qkv_block(i, (i + 1) % NTB)
            return c
        lax.fori_loop(1 - l, NTB, qkv_body, 0)

        attn_first()

        def attn_body(i, c):
            attn_pair(i, jnp.minimum(2 * i + 2, NQB - 1))
            return c
        lax.fori_loop(1, NTB, attn_body, 0)

        @pl.when(last)
        def _():
            for i in range(NTB - 2):
                out_copy(i).start()
        out_tail(l // 2)

        @pl.when(last)
        def _():
            for i in range(NTB - 2, NTB):
                out_copy(i).start()

        ffn(l, first, last)
        return carry

    lax.fori_loop(0, 2, layer, 0)


@jax.jit
def pallas_interleave_layers__sliding_block__moe_arch_mod__prompt_kernel(
    A_x: jax.Array,
    A_wqkv: jax.Array,
    A_wo: jax.Array,
    B_x: jax.Array,
    B_w_r: jax.Array,
    B_w_gate: jax.Array,
    B_w_up: jax.Array,
    B_w_down: jax.Array,
):
    del B_x
    hbm = pl.BlockSpec(memory_space=pl.ANY)
    return pl.pallas_call(
        _kernel,
        in_specs=[hbm, hbm, hbm, pl.BlockSpec(memory_space=pltpu.VMEM), hbm, hbm, hbm],
        out_specs=hbm,
        out_shape=jax.ShapeDtypeStruct((1, S, D), BF),
        scratch_shapes=[
            pltpu.VMEM((S + TB + 16, D), BF),
            pltpu.VMEM((S + TB, D), F32),
            pltpu.VMEM((TB // 2, D), I32),
            pltpu.VMEM((2, 7, QB // 2, D // 2), I32),
            pltpu.VMEM((NNC // 2, D, 2 * NC), BF),
            pltpu.VMEM((NNC, 7, D // 4, 128), I32),
            pltpu.VMEM((D, D), BF),
            pltpu.VMEM((7, D // 4, D // 2), I32),
            pltpu.VMEM((F // 128, D, 128), BF),
            pltpu.VMEM((F // 128, D, 128), BF),
            pltpu.VMEM((D // 128, F, 128), BF),
            pltpu.VMEM((4 * NG, S // 2, 128), I32),
            pltpu.VMEM((TB // 2, 128), I32),
            pltpu.VMEM((4 * NG, S // 2, 128), I32),
            pltpu.VMEM((NQB, D // 2, QB), I32),
            pltpu.VMEM((TB, D), F32),
            pltpu.VMEM((128, QB), F32),
            pltpu.VMEM((2, TB, D), F32),
            pltpu.VMEM((8, 128), F32),
            pltpu.VMEM((8, 128), I32),
            pltpu.VMEM((4, 4, 2 * QB, QB), F32),
            pltpu.VMEM((4, 4, 8, QB), F32),
            pltpu.SemaphoreType.DMA((NTB,)),
            pltpu.SemaphoreType.DMA((NNC // 2 + 5,)),
            pltpu.SemaphoreType.DMA((NTB,)),
        ],
        compiler_params=pltpu.CompilerParams(vmem_limit_bytes=112 * 1024 * 1024),
        name="mod_swa",
    )(A_x, A_wqkv, A_wo, B_w_r, B_w_gate, B_w_up, B_w_down)
```
